```python
import os as _os
_os.environ.setdefault("JAX_PLATFORMS", "cpu")
import jax
import jax.numpy as jnp

def _softmax(x, axis=-1):
    return jax.nn.softmax(x, axis=axis)
def _gelu(x):
    return jax.nn.gelu(x, approximate=True)
def _silu(x):
    return jax.nn.silu(x)
def _sigmoid(x):
    return jax.nn.sigmoid(x)
def _layernorm(x, axis=-1, eps=1e-5):
    m = jnp.mean(x, axis=axis, keepdims=True)
    v = jnp.var(x, axis=axis, keepdims=True)
    return (x - m) / jnp.sqrt(v + eps)
def _scatter_add(tgt, idx, src, axis=0):
    return tgt.at[idx].add(src)
def _segment_sum(src, seg, n):
    return jax.ops.segment_sum(src, seg, n)
class _Rng:
    def __init__(self, key):
        self._k = key
    def _next(self):
        self._k, sub = jax.random.split(self._k)
        return sub
    def normal(self, shape):
        return jax.random.normal(self._next(), shape, dtype=jnp.bfloat16)
    def randint(self, lo, hi, shape):
        return jax.random.randint(self._next(), shape, lo, hi, dtype=jnp.int32)
    def uniform(self, shape, lo=0.0, hi=1.0):
        return jax.random.uniform(self._next(), shape, jnp.bfloat16, lo, hi)
    def permutation(self, n):
        return jax.random.permutation(self._next(), n)


kernel_name = 'sequential_preLN__softmax_full_mha__dense_activation_gelu__prompt'

def setup_inputs():
    _rng = _Rng(jax.random.key(int.from_bytes(__import__("os").urandom(4), "little")))
    _w = (lambda a: (lambda t: t.astype(jnp.bfloat16) if jnp.issubdtype(t.dtype, jnp.floating) else t)(jnp.asarray(a)))
    def _A_setup():
        B, S, D = 1, 2048, 512
        return {
            "x": _w((lambda *s: _rng.normal(s) * 0.05)(B, S, D)),
            "wqkv": _w((lambda *s: _rng.normal(s) * 0.05)(D, 3 * D)),
            "wo": _w((lambda *s: _rng.normal(s) * 0.05)(D, D)),
        }
    _A_in = _A_setup()

    def _B_setup():
        B, S, D, F = 1, 2048, 512, 1792
        return {
            "x": _w((lambda *s: _rng.normal(s) * 0.05)(B, S, D)),
            "w1": _w((lambda *s: _rng.normal(s) * 0.4)(D, F) * (D ** -0.5)),
            "b1": _w((lambda *s: _rng.normal(s) * 0.4)(F) * 0.01),
            "w2": _w((lambda *s: _rng.normal(s) * 0.4)(F, D) * (F ** -0.5)),
            "b2": _w((lambda *s: _rng.normal(s) * 0.05)(D) * 0.01),
        }
    _B_in = _B_setup()

    return {
        "A_x": _A_in["x"],
        "A_wqkv": _A_in["wqkv"],
        "A_wo": _A_in["wo"],
        "B_x": _B_in["x"],
        "B_w1": _B_in["w1"],
        "B_b1": _B_in["b1"],
        "B_w2": _B_in["w2"],
        "B_b2": _B_in["b2"],
    }

def reference(A_x, A_wqkv, A_wo, B_x, B_w1, B_b1, B_w2, B_b2):
    def _A_ref(x, wqkv, wo):
        B, S, D = x.shape
        H = 32; Dh = D // H
        qkv = (lambda x, *d: x.transpose(*d))((x @ wqkv).reshape(B, S, 3, H, Dh), 2, 0, 3, 1, 4)
        q, k, v = qkv[0], qkv[1], qkv[2]
        scale = Dh ** -0.5
        scores = jnp.einsum("bhqd,bhkd->bhqk", q, k) * scale
        p = _softmax(scores, axis=-1)
        o = jnp.einsum("bhqk,bhkd->bhqd", p, v)
        return (lambda x, *d: x.transpose(*d))(o, 0, 2, 1, 3).reshape(B, S, D) @ wo

    def _B_ref(x, w1, b1, w2, b2):
        h = jnp.einsum("bsd,df->bsf", x, w1) + b1
        h = _gelu(h)
        return jnp.einsum("bsf,fd->bsd", h, w2) + b2

    x = A_x
    h = x + _A_ref(_layernorm(x, axis=-1), A_wqkv, A_wo)
    h2 = h + _B_ref(_layernorm(h, axis=-1), B_w1, B_b1, B_w2, B_b2)
    return h2
```

```python
import jax
import jax.numpy as jnp
import numpy as np
import jax.experimental.pallas as pl
import jax.experimental.pallas.tpu as pltpu

S, D, F, H, DH = 2048, 512, 1792, 32, 16
TQ = 512
CK = 128
NC = S // CK
R1 = 256
R3 = 256
FC = 256
QT_MODE = 0
EPS = 1e-5
bf16, f32, u32 = jnp.bfloat16, jnp.float32, jnp.uint32
Q_SCALE = float(DH ** -0.5 * np.log2(np.e))


def _ln(x):
    m = jnp.mean(x, axis=-1, keepdims=True)
    xc = x - m
    v = jnp.mean(xc * xc, axis=-1, keepdims=True)
    return xc * jax.lax.rsqrt(v + EPS)


def _gelu(x):
    c = float(np.sqrt(2.0 / np.pi))
    return (0.5 * x) * (1.0 + jnp.tanh(x * (c + (c * 0.044715) * (x * x))))


def _kernel(x_hbm, wqkv_hbm, wo_hbm, w1_hbm, b1_ref, w2_hbm, b2_ref, out_hbm,
            x_v, wqkv_v, wo_v, w1_v, w2_v, k_p, qt_p, vt_p, ot_v, s_a, s_b, g_v, out_v,
            in_sem, out_sem):
    n1, n3 = S // R1, S // R3

    def x_copy(i):
        rows = pl.ds(i * R1, R1)
        return pltpu.make_async_copy(x_hbm.at[rows], x_v.at[rows], in_sem.at[i])
    w_copies = [
        pltpu.make_async_copy(src, dst, in_sem.at[n1 + i])
        for i, (src, dst) in enumerate(((wqkv_hbm, wqkv_v), (wo_hbm, wo_v), (w1_hbm, w1_v), (w2_hbm, w2_v)))
    ]
    x_copy(0).start()
    w_copies[0].start()
    for i in range(1, n1):
        x_copy(i).start()
    for c in w_copies[1:]:
        c.start()

    w_copies[0].wait()

    def qkv_step(i, carry):
        x_copy(i).wait()
        r0 = pl.multiple_of(i * R1, R1)
        xn = _ln(x_v[pl.ds(r0, R1), :].astype(f32)).astype(bf16)
        q = jnp.dot(xn, wqkv_v[:, 0:D], preferred_element_type=f32) * Q_SCALE
        k = jnp.dot(xn, wqkv_v[:, D:2 * D], preferred_element_type=f32)
        v = jnp.dot(xn, wqkv_v[:, 2 * D:3 * D], preferred_element_type=f32)
        kp = pltpu.bitcast(k.astype(bf16), u32)
        for g in range(D // 128):
            k_p[g, pl.ds(pl.multiple_of(i * (R1 // 2), R1 // 2), R1 // 2), :] = kp[:, g * 128:(g + 1) * 128]
        if QT_MODE == 0:
            qt = q.T.astype(bf16); vt = v.T.astype(bf16)
        else:
            qt = q.astype(bf16).T; vt = v.astype(bf16).T
        qt_p[:, pl.ds(r0, R1)] = pltpu.bitcast(qt, u32)
        vt_p[:, pl.ds(r0, R1)] = pltpu.bitcast(vt, u32)
        return carry
    jax.lax.fori_loop(0, n1, qkv_step, 0)

    bufs = (s_a, s_b)

    def a_chunk(t, j, c, m):
        qb, g = t // 4, t % 4
        q = pltpu.bitcast(qt_p[pl.ds(pl.multiple_of(g * 64 + j * 8, 8), 8), pl.ds(pl.multiple_of(qb * TQ, TQ), TQ)], bf16)
        parts = []
        if j > 0:
            parts.append(jnp.zeros((16 * j, TQ), bf16))
        parts.append(q)
        if j < 7:
            parts.append(jnp.zeros((16 * (7 - j), TQ), bf16))
        kk = pltpu.bitcast(k_p[g, pl.ds(c * CK // 2, CK // 2), :], bf16)
        st = jnp.dot(kk, jnp.concatenate(parts, axis=0), preferred_element_type=f32)
        bufs[j % 2][pl.ds(c * CK, CK), :] = st
        for r in range(CK // 8):
            row = st[r * 8:(r + 1) * 8]
            m = row if m is None else jnp.maximum(m, row)
        return m

    def b_chunk(t, j, c, m, l, acc):
        g = t % 4
        p = jnp.exp2(bufs[j % 2][pl.ds(c * CK, CK), :] - jnp.tile(m, (CK // 8, 1)))
        for r in reversed(range(CK // 8)):
            row = p[r * 8:(r + 1) * 8]
            l = row if l is None else l + row
        lb = pltpu.bitcast(l, u32)
        z = lb[:, 0:128]
        for n in range(1, TQ // 128):
            z = z | lb[:, n * 128:(n + 1) * 128]
        vb = vt_p[pl.ds(pl.multiple_of(g * 64 + j * 8, 8), 8), pl.ds(c * CK, CK)] | (z >> 31)
        o = jnp.dot(pltpu.bitcast(vb, bf16), p.astype(bf16), preferred_element_type=f32)
        acc = o if acc is None else acc + o
        return l, acc

    def fin_m(m):
        return jnp.broadcast_to(jnp.max(m, axis=0, keepdims=True), (8, TQ))

    def fin_b(t, j, l, acc):
        qb, g = t // 4, t % 4
        o = acc * (1.0 / jnp.sum(l, axis=0, keepdims=True))
        ot_v[pl.ds(pl.multiple_of(g * 128 + j * 16, 16), 16), pl.ds(pl.multiple_of(qb * TQ, TQ), TQ)] = o

    NT = (S // TQ) * 4
    m = None
    for c in range(NC):
        m = a_chunk(0, 0, c, m)
    m_cur = fin_m(m)

    def body(t, m_cur):
        t_next = jnp.minimum(t + 1, NT - 1)
        for j in range(8):
            m = l = acc = None
            for c in range(NC):
                if j < 7:
                    m = a_chunk(t, j + 1, c, m)
                else:
                    m = a_chunk(t_next, 0, c, m)
                l, acc = b_chunk(t, j, c, m_cur, l, acc)
            fin_b(t, j, l, acc)
            m_cur = fin_m(m)
        return m_cur
    jax.lax.fori_loop(0, NT, body, m_cur)

    for c in w_copies[1:]:
        c.wait()
    b1 = b1_ref[...].astype(f32).reshape(1, F)
    b2 = b2_ref[...].astype(f32).reshape(1, D)

    def out_copy(i):
        rows = pl.ds(pl.multiple_of(i * R3, R3), R3)
        return pltpu.make_async_copy(out_v.at[rows], out_hbm.at[rows], out_sem.at[i])

    def ffn_step(i, carry):
        r0 = pl.multiple_of(i * R3, R3)
        o = ot_v[:, pl.ds(r0, R3)].T.astype(bf16)
        h = x_v[pl.ds(r0, R3), :].astype(f32) + jnp.dot(o, wo_v[...], preferred_element_type=f32)
        hn = _ln(h).astype(bf16)
        for f0 in range(0, F, FC):
            a = jnp.dot(hn, w1_v[:, f0:f0 + FC], preferred_element_type=f32) + b1[:, f0:f0 + FC]
            g_v[:, f0:f0 + FC] = _gelu(a).astype(bf16)
        y = jnp.dot(g_v[...], w2_v[...], preferred_element_type=f32)
        out_v[pl.ds(r0, R3), :] = (h + y + b2).astype(out_v.dtype)
        out_copy(i).start()
        return carry
    jax.lax.fori_loop(0, n3, ffn_step, 0)
    for i in range(n3):
        out_copy(i).wait()


@jax.jit
def pallas_sequential_preLN__softmax_full_mha__dense_activation_gelu__prompt_kernel(
        A_x, A_wqkv, A_wo, B_x, B_w1, B_b1, B_w2, B_b2):
    del B_x
    any_spec = pl.BlockSpec(memory_space=pl.ANY)
    vmem_spec = pl.BlockSpec(memory_space=pltpu.VMEM)
    out = pl.pallas_call(
        _kernel,
        out_shape=jax.ShapeDtypeStruct((S, D), A_x.dtype),
        in_specs=[any_spec, any_spec, any_spec, any_spec, vmem_spec, any_spec, vmem_spec],
        out_specs=any_spec,
        scratch_shapes=[
            pltpu.VMEM((S, D), bf16), pltpu.VMEM((D, 3 * D), bf16), pltpu.VMEM((D, D), bf16),
            pltpu.VMEM((D, F), bf16), pltpu.VMEM((F, D), bf16),
            pltpu.VMEM((D // 128, S // 2, 128), u32), pltpu.VMEM((D // 2, S), u32), pltpu.VMEM((D // 2, S), u32),
            pltpu.VMEM((D, S), f32), pltpu.VMEM((S, TQ), f32), pltpu.VMEM((S, TQ), f32),
            pltpu.VMEM((R3, F), bf16), pltpu.VMEM((S, D), bf16),
            pltpu.SemaphoreType.DMA((S // R1 + 4,)), pltpu.SemaphoreType.DMA((S // R3,)),
        ],
        compiler_params=pltpu.CompilerParams(vmem_limit_bytes=100 * 1024 * 1024),
    )(A_x.reshape(S, D), A_wqkv, A_wo, B_w1, B_b1, B_w2, B_b2)
    return out.reshape(A_x.shape)
```

```python
import jax
import jax.numpy as jnp
import numpy as np
import jax.experimental.pallas as pl
import jax.experimental.pallas.tpu as pltpu

S, D, F, H, DH = 2048, 512, 1792, 32, 16
TQ = 512
NQ = TQ // 128
NB = S // TQ
CK = 128
NC = S // CK
PAT = [16]
NV = [PAT[c % len(PAT)] for c in range(NC)]
NT = [(CK - v) // 16 for v in NV]
V0 = [sum(NV[:c]) for c in range(NC + 1)]
T0 = [sum(NT[:c]) for c in range(NC + 1)]
HU = 4
OFF = 2
TSH = 2
KSP = 2
R1 = 256
R3 = 128
U1 = 1
FC = 256
ONLY = 0
FORCE_SAFE = 0
DMAP = 0
RCP = 1
TS = 128
EPS = 1e-5
L_MIN, L_MAX, A_MAX = 2.0 ** -40, 2.0 ** 40, 2.0 ** 120
bf16, f32, u32, i32 = jnp.bfloat16, jnp.float32, jnp.uint32, jnp.int32
Q_SCALE = float(DH ** -0.5 * np.log2(np.e))


def _mo(x, n):
    return x if isinstance(x, int) else pl.multiple_of(x, n)


def _mm(a, b):
    return jax.lax.dot_general(a, b, (((1,), (0,)), ((), ())), preferred_element_type=f32)


def _take(x, idx, axis):
    return jnp.take_along_axis(x, idx, axis=axis, mode="promise_in_bounds")


def _ln(x):
    m = jnp.mean(x, axis=-1, keepdims=True)
    xc = x - m
    v = jnp.mean(xc * xc, axis=-1, keepdims=True)
    return xc * jax.lax.rsqrt(v + EPS)


def _gelu(x):
    c = float(np.sqrt(2.0 / np.pi))
    return (0.5 * x) * (1.0 + jnp.tanh(x * (c + (c * 0.044715) * (x * x))))


def _kernel(x_hbm, wqkv_hbm, wo_hbm, w1_hbm, b1_ref, w2_hbm, b2_ref, out_hbm,
            x_v, wqkv_v, wo_v, w1_v, w2_v, xn_v, k_p, ko_v, qt_v, vt_p, ot_v, l_v,
            km, kx, kb, qw, qb, vw, z_v, o_v, h_v, hn_v, g_v, out_v, in_sem, out_sem):
    n1, n3 = S // R1, S // R3

    XA = 512

    def part(src, dst, rows, cols, i):
        return pltpu.make_async_copy(src.at[rows, cols], dst.at[rows, cols], in_sem.at[i])
    every = slice(None)
    cp_x = [part(x_hbm, x_v, pl.ds(r0, n), every, i) for i, (r0, n) in enumerate(((0, XA), (XA, XA), (2 * XA, S - 2 * XA)))]
    cp_q, cp_k, cp_v = [part(wqkv_hbm, wqkv_v, every, pl.ds(i * D, D), 3 + i) for i in range(3)]
    cp_w = [part(src, dst, every, every, 6 + i) for i, (src, dst) in enumerate(((wo_hbm, wo_v), (w1_hbm, w1_v), (w2_hbm, w2_v)))]
    for c in (cp_x[0], cp_k, cp_q, cp_x[1], cp_v, cp_x[2], *cp_w):
        c.start()

    def ln1(r0, r1):
        for r in range(r0, r1, R1):
            rows = pl.ds(r, R1)
            xn_v[rows, :] = _ln(x_v[rows, :].astype(f32)).astype(bf16)

    def proj_q(r0, r1):
        for r in range(r0, r1, R1):
            q = _mm(xn_v[pl.ds(r, R1), :], wqkv_v[:, 0:D]) * Q_SCALE
            qt_v[:, pl.ds(r, R1)] = q.T

    def proj_k(r0, r1):
        for r in range(r0, r1, R1):
            k = _mm(xn_v[pl.ds(r, R1), :], wqkv_v[:, D:2 * D])
            kp = pltpu.bitcast(k.astype(bf16), u32)
            for g in range(D // 128):
                lanes = slice(g * 128, (g + 1) * 128)
                k_p[g, pl.ds(r // 2, R1 // 2), :] = kp[:, lanes]
                for c in range(r // CK, (r + R1) // CK):
                    ko_v[g, pl.ds(V0[c], NV[c]), :] = k[(c + 1) * CK - NV[c] - r:(c + 1) * CK - r, lanes]

    def proj_v(r0, r1):
        for r in range(r0, r1, R1):
            v = _mm(xn_v[pl.ds(r, R1), :], wqkv_v[:, 2 * D:3 * D])
            vt_p[:, pl.ds(r, R1)] = pltpu.bitcast(v.T.astype(bf16), u32)

    lane = jax.lax.broadcasted_iota(i32, (8, 128), 1)

    def stage_mxu_keys(h, u, c, after=lambda x: x):
        idx = after((lane + (h % 8) * DH) & 127)
        kp = k_p[h // 8, pl.ds(c * CK // 2, NT[c] * 8), :]
        km[u, pl.ds(T0[c] * 8, NT[c] * 8), :] = _take(kp, jnp.tile(idx, (NT[c], 1)), axis=1)
        if c == 0:
            idx = (idx + (128 - DH)) & 127
            moved = _take(kp[(NT[c] - OFF) * 8:], jnp.tile(idx, (OFF, 1)), axis=1)
            ln = jnp.tile(lane, (OFF, 1))
            kx[u] = jnp.where((ln >= DH) & (ln < 2 * DH), moved, 0)

    def stage_values(h, u):
        vw[u] = vt_p[pl.ds(_mo(h * (DH // 2), DH // 2), DH // 2), :]

    def stage_vpu_keys(h, u, d, after=lambda x: x):
        idx = after(jnp.full((8, 128), (h % 8) * DH + d, i32))
        kb[u, d] = _take(ko_v[h // 8], jnp.tile(idx, (V0[NC] // 8, 1)), axis=1)

    def stage_query(h, u, b, d, after=lambda x: x):
        q = qt_v[pl.ds(_mo(h * DH + d // 8 * 8, 8), 8), pl.ds(b * TQ, TQ)]
        idx = after(jnp.full((8, 128), d % 8, i32))
        for n in range(NQ):
            qb[u, b, d, :, pl.ds(n * 128, 128)] = _take(q[:, n * 128:(n + 1) * 128], idx, axis=0)
        if d % 8 == 0:
            qw[u, b, pl.ds(d, 8), :] = q

    z_v[...] = jnp.zeros((8, 128), f32)
    with jax.named_scope("wait0"):
        cp_x[0].wait()
        ln1(0, XA)
        cp_k.wait()
    with jax.named_scope("phase1"):
        on = ONLY in (0, 1)
        if on:
            proj_k(0, XA)
        cp_q.wait()
        cp_x[1].wait()
        if on:
            ln1(XA, 2 * XA)
            proj_q(0, XA)
            proj_k(XA, 2 * XA)
        cp_v.wait()
        cp_x[2].wait()
        if on:
            ln1(2 * XA, S)
            proj_q(XA, 2 * XA)
            proj_k(2 * XA, S)
            proj_q(2 * XA, S)
        for u in range(HU):
            if u < HU - 1:
                for c in range(NC):
                    stage_mxu_keys(u, u, c)
                for d in range(DH):
                    stage_vpu_keys(u, u, d)
            for b in range(NB):
                for d in range(DH):
                    stage_query(u, u, b, d)
        if on:
            proj_v(0, S)
        for u in range(HU - 1):
            stage_values(u, u)

    def fast_step(it, carry):
        lo, hi, big = carry
        items = [(u, b, c) for u in range(HU) for b in range(NB) for c in range(NC)]
        tiles = [(n, t) for n, (u, b, c) in enumerate(items) for t in range(NT[c])]
        first = [n // NC * T0[NC] + T0[c] for n, (u, b, c) in enumerate(items)] + [len(tiles)]
        outs = [(n, q, r) for n, (u, b, c) in enumerate(items) for r in reversed(range(NV[c] // 8)) for q in range(NQ)]
        ties = {}
        for o, key in enumerate(outs):
            ties.setdefault((o * len(tiles)) // len(outs) + TSH, []).append(key)
        head = lambda u: it * HU + u
        later = lambda u: jnp.minimum(it + 1, H // HU - 1) * HU + u
        zero = z_v[...]
        always = zero >= 0.0
        sv, st = {}, {}

        def vpu_scores(n, q, r):
            if (n, q, r) not in sv:
                u, b, c = items[n]
                acc = None
                for d in range(DH):
                    t = kb[u, d, pl.ds(V0[c] + r * 8, 8), :] * qb[u, b, d, :, pl.ds(q * 128, 128)]
                    acc = t if acc is None else acc + t
                sv[n, q, r] = acc
            return sv[n, q, r]

        def key_tile(g, moved=False):
            n, t = tiles[g]
            u, b, c = items[n]
            if moved:
                kt = kx[u, pl.ds((OFF - 1 - t) * 8, 8), :]
            else:
                kt = km[u, pl.ds((T0[c + 1] - 1 - t) * 8, 8), :]
            for key in ties.get(g, ()):
                kt = jnp.where(always, kt, pltpu.bitcast(vpu_scores(*key), u32))
            return kt

        def mxu_scores(g0, g1):
            u0, b0, _ = items[tiles[g0][0]]
            u1, b1, _ = items[tiles[g1 - 1][0]]
            if (u0, b0) != (u1, b1):
                e = g1 // T0[NC] * T0[NC]
                lhs = [jnp.where(lane < DH, key_tile(g), 0) for g in range(g0, e)]
                lhs += [key_tile(g, True) for g in range(e, g1)]
                w = [qw[u0, b0], qw[u1, b1]]
            else:
                lhs = [key_tile(g) for g in range(g0, g1)]
                w = [qw[u0, b0]]
            w = jnp.concatenate(w + [jnp.zeros((128 - DH * len(w), TQ), f32)], axis=0)
            s = _mm(pltpu.bitcast(jnp.concatenate(lhs, axis=0), bf16), w)
            for g in range(g0, g1):
                st[g] = s[(g - g0) * 16:(g - g0 + 1) * 16]

        def weigh(n, l, acc):
            u, b, c = items[n]
            rows = [st.pop(first[n + 1] - 1 - t) for t in range(NT[c])]
            rows += [jnp.concatenate([vpu_scores(n, q, r) for q in range(NQ)], axis=1) for r in range(NV[c] // 8)]
            p = jnp.exp2(jnp.concatenate(rows, axis=0))
            for r in reversed(range(CK // 8)):
                row = p[r * 8:(r + 1) * 8]
                l = row if l is None else l + row
            o = _mm(pltpu.bitcast(vw[u, :, pl.ds(c * CK, CK)], bf16), p)
            return l, (o if acc is None else acc + o)

        bound = lambda m: len(tiles) if m >= len(items) else first[m] + OFF
        l = acc = None
        for m in range(len(items) + 1):
            g0, g1 = bound(m) if m else 0, bound(m + 1)
            if g0 < g1:
                mxu_scores(g0, g1)
            if m == 0:
                continue
            u, b, c = items[m - 1]
            if c == 0:
                l = acc = None
            l, acc = weigh(m - 1, l, acc)

            def after(x, l0=l[:, 0:128]):
                return jnp.where(always, x, pltpu.bitcast(l0, i32))
            step, sub = divmod(b * NC + c, KSP)
            if step < NC:
                h_fill = later(u - 1) if u > 0 else head(HU - 1)
                if sub == 0:
                    stage_vpu_keys(h_fill, (u - 1) % HU, step, after)
                if sub == KSP - 1:
                    stage_mxu_keys(h_fill, (u - 1) % HU, step, after)
                    if step == 0:
                        stage_values(h_fill, (u - 1) % HU)
            blk = u * NB + b
            if blk > 0:
                stage_query(later((blk - 1) // NB), (blk - 1) // NB, (blk - 1) % NB, c, after)
            if c == NC - 1:
                ot_v[pl.ds(_mo(head(u) * DH, DH), DH), pl.ds(b * TQ, TQ)] = acc
                l_v[head(u), :, pl.ds(b * TQ, TQ)] = l
                for q in range(NQ):
                    cols = slice(q * 128, (q + 1) * 128)
                    lo = jnp.minimum(lo, l[:, cols])
                    hi = jnp.maximum(hi, l[:, cols])
                    big = jnp.maximum(big, jnp.maximum(jnp.abs(acc[0:8, cols]), jnp.abs(acc[8:16, cols])))
        for d in range(DH):
            stage_query(later(HU - 1), HU - 1, NB - 1, d, after)
        return lo, hi, big

    one = jnp.ones((8, 128), f32)
    with jax.named_scope("phase2"):
        lo, hi, big = one, one, one
        if ONLY in (0, 2):
            lo, hi, big = jax.lax.fori_loop(0, H // HU, fast_step, (lo, hi, big))
    safe = (lo >= L_MIN) & (hi <= L_MAX) & (big <= A_MAX)

    @pl.when(jnp.max(jnp.where(safe, float(FORCE_SAFE), 1.0)) > 0.0)
    def _():
        def safe_step(i, carry):
            h, b = i // (S // TS), i % (S // TS)
            cols = pl.ds(_mo(b * TS, TS), TS)
            q = qt_v[pl.ds(_mo(h * DH, DH), DH), cols]
            row_head = jax.lax.broadcasted_iota(i32, (128, TS), 0) // DH
            qm = jnp.where(row_head == h % 8, jnp.tile(q, (8, 1)), 0.0)
            s = _mm(pltpu.bitcast(k_p[h // 8], bf16), qm)
            p = jnp.exp2(s - jnp.max(s, axis=0, keepdims=True))
            v = pltpu.bitcast(vt_p[pl.ds(_mo(h * (DH // 2), DH // 2), DH // 2), :], bf16)
            ot_v[pl.ds(_mo(h * DH, DH), DH), cols] = _mm(v, p)
            l_v[h, :, cols] = jnp.sum(p.reshape(S // 8, 8, TS), axis=0)
            return carry
        jax.lax.fori_loop(0, H * (S // TS), safe_step, 0)

    for c in cp_w:
        c.wait()
    b1 = b1_ref[...].astype(f32).reshape(1, F)
    b2 = b2_ref[...].astype(f32).reshape(1, D)

    def out_copy(i):
        rows = pl.ds(i * R3, R3)
        return pltpu.make_async_copy(out_v.at[rows], out_hbm.at[rows], out_sem.at[i])

    def normalize(i):
        rows = pl.ds(i * R3, R3)
        for g in range(D // 128):
            ot = []
            for h in range(g * 8, g * 8 + 8):
                lsum = jnp.sum(l_v[h, :, rows], axis=0, keepdims=True)
                if RCP:
                    inv = pl.reciprocal(lsum, approx=True)
                    inv = inv * (2.0 - lsum * inv)
                else:
                    inv = 1.0 / lsum
                ot.append(ot_v[pl.ds(h * DH, DH), rows] * inv)
            o_v[rows, pl.ds(g * 128, 128)] = jnp.concatenate(ot, axis=0).T.astype(bf16)

    def out_proj(i):
        rows = pl.ds(i * R3, R3)
        hid = x_v[rows, :].astype(f32) + _mm(o_v[rows, :], wo_v[...])
        h_v[rows, :] = hid
        hn_v[rows, :] = _ln(hid).astype(bf16)

    def ffn_up(i):
        hn = hn_v[pl.ds(i * R3, R3), :]
        for f0 in range(0, F, FC):
            a = _mm(hn, w1_v[:, f0:f0 + FC]) + b1[:, f0:f0 + FC]
            g_v[i % 2, :, f0:f0 + FC] = _gelu(a).astype(bf16)

    def ffn_down(i):
        rows = pl.ds(i * R3, R3)
        y = _mm(g_v[i % 2], w2_v[...])
        out_v[rows, :] = (h_v[rows, :] + y + b2).astype(out_v.dtype)

    with jax.named_scope("phase3"):
        if ONLY in (0, 3):
            normalize(0)
            out_proj(0)
            normalize(1)
            out_proj(1)
            normalize(2)
            for i in range(n3):
                ffn_up(i)
                if i + 2 < n3:
                    out_proj(i + 2)
                if i + 3 < n3:
                    normalize(i + 3)
                if DMAP == 1 and i > 0:
                    out_copy(i - 1).start()
                ffn_down(i)
                if DMAP == 0:
                    out_copy(i).start()
            if DMAP == 1:
                out_copy(n3 - 1).start()
            if DMAP == 2:
                for i in range(n3):
                    out_copy(i).start()
        else:
            for i in range(n3):
                out_copy(i).start()
    with jax.named_scope("tail"):
        for i in range(n3):
            out_copy(i).wait()


@jax.jit
def pallas_sequential_preLN__softmax_full_mha__dense_activation_gelu__prompt_kernel(
        A_x, A_wqkv, A_wo, B_x, B_w1, B_b1, B_w2, B_b2):
    del B_x
    any_spec = pl.BlockSpec(memory_space=pl.ANY)
    vmem_spec = pl.BlockSpec(memory_space=pltpu.VMEM)
    vm = pltpu.VMEM
    out = pl.pallas_call(
        _kernel,
        out_shape=jax.ShapeDtypeStruct((S, D), A_x.dtype),
        in_specs=[any_spec, any_spec, any_spec, any_spec, vmem_spec, any_spec, vmem_spec],
        out_specs=any_spec,
        scratch_shapes=[
            vm((S, D), bf16), vm((D, 3 * D), bf16), vm((D, D), bf16), vm((D, F), bf16), vm((F, D), bf16),
            vm((S, D), bf16),
            vm((D // 128, S // 2, 128), u32), vm((D // 128, V0[NC], 128), f32),
            vm((D, S), f32), vm((D // 2, S), u32), vm((D, S), f32), vm((H, 8, S), f32),
            vm((HU, T0[NC] * 8, 128), u32), vm((HU, OFF * 8, 128), u32), vm((HU, DH, V0[NC], 128), f32),
            vm((HU, NB, DH, TQ), f32), vm((HU, NB, DH, 8, TQ), f32), vm((HU, DH // 2, S), u32),
            vm((8, 128), f32),
            vm((S, D), bf16), vm((S, D), f32), vm((S, D), bf16), vm((2, R3, F), bf16), vm((S, D), bf16),
            pltpu.SemaphoreType.DMA((9,)), pltpu.SemaphoreType.DMA((S // R3,)),
        ],
        compiler_params=pltpu.CompilerParams(vmem_limit_bytes=100 * 1024 * 1024),
    )(A_x.reshape(S, D), A_wqkv, A_wo, B_w1, B_b1, B_w2, B_b2)
    return out.reshape(A_x.shape)
```

```python
import functools
import jax
import jax.numpy as jnp
import numpy as np
import jax.experimental.pallas as pl
import jax.experimental.pallas.tpu as pltpu

S, D, F, H, DH = 2048, 512, 1792, 32, 16
TQ = 512
NQ = TQ // 128
NB = S // TQ
CK = 128
NC = S // CK
PAT = [16]
NV = [PAT[c % len(PAT)] for c in range(NC)]
NT = [(CK - v) // 16 for v in NV]
V0 = [sum(NV[:c]) for c in range(NC + 1)]
T0 = [sum(NT[:c]) for c in range(NC + 1)]
HU = 4
OFF = 2
TSH = 2
KSP = 2
R1 = 256
R3 = 128
U1 = 1
FC = 256
ONLY = 0
FORCE_SAFE = 0
DMAP = 0
RCP = 1
MIX = 3
ORD = [range(7), (1, 3, 2, 4, 0, 5, 6), (0, 1, 3, 2, 4, 5, 6), (4, 2, 3, 1, 0, 6, 5)][0]
WO7 = 1
PR = 16
XF = 1
WP = 0
TORD = 0
NTM = 2
VB = 1
KQ = 1
TS = 128
EPS = 1e-5
L_MIN, L_MAX, A_MAX = 2.0 ** -40, 2.0 ** 40, 2.0 ** 120
bf16, f32, u32, i32 = jnp.bfloat16, jnp.float32, jnp.uint32, jnp.int32
Q_SCALE = float(DH ** -0.5 * np.log2(np.e))


def _mo(x, n):
    return x if isinstance(x, int) else pl.multiple_of(x, n)


def _mm(a, b):
    return jax.lax.dot_general(a, b, (((1,), (0,)), ((), ())), preferred_element_type=f32)


def _mm_nt(a, b):
    return jax.lax.dot_general(a, b, (((1,), (1,)), ((), ())), preferred_element_type=f32)


def _take(x, idx, axis):
    return jnp.take_along_axis(x, idx, axis=axis, mode="promise_in_bounds")


def _pack(x):
    return x


def _lhs7(a11, a12, a21, a22):
    return (a11 + a22, a21 + a22, a11, a22, a11 + a12, a21 - a11, a12 - a22)


def _rhs7(b11, b12, b21, b22):
    return (b11 + b22, b11, b12 - b22, b21 - b11, b22, b11 + b12, b21 + b22)


def _join7(m):
    return (m[0] + m[3] - m[4] + m[6], m[2] + m[4], m[1] + m[3], m[0] - m[1] + m[2] + m[5])


def _ln(x):
    m = jnp.mean(x, axis=-1, keepdims=True)
    xc = x - m
    v = jnp.mean(xc * xc, axis=-1, keepdims=True)
    return xc * jax.lax.rsqrt(v + EPS)


def _gelu(x):
    c = float(np.sqrt(2.0 / np.pi))
    return (0.5 * x) * (1.0 + jnp.tanh(x * (c + (c * 0.044715) * (x * x))))


def _kernel(x_hbm, wqkv_hbm, wo_hbm, w1_hbm, b1_ref, w2_hbm, b2_ref, out_hbm,
            x_v, wqkv_v, wo_v, w1_v, w2_v, wp, wt_v, xn_v, k_p, ko_v, qt_v, vt_p, ot_v, l_v,
            km, kx, kb, qw, qb, vw, z_v, wo7, w17, w27, o7, hn7, g7, h_v, out_v, in_sem, out_sem):
    n1, n3 = S // R1, S // R3

    XA = 512

    def part(src, dst, rows, cols, i):
        return pltpu.make_async_copy(src.at[rows, cols], dst.at[rows, cols], in_sem.at[i])
    every = slice(None)
    cp_x = [part(x_hbm, x_v, pl.ds(r0, n), every, i) for i, (r0, n) in enumerate(((0, XA), (XA, XA), (2 * XA, S - 2 * XA)))]
    cp_q, cp_k, cp_v = [part(wqkv_hbm, wqkv_v, every, pl.ds(i * D, D), 3 + i) for i in range(3)]
    cp_w = [part(src, dst, every, every, 6 + i) for i, (src, dst) in enumerate(((wo_hbm, wo_v), (w1_hbm, w1_v), (w2_hbm, w2_v)))]
    for c in (cp_x[0], cp_k, cp_q, cp_x[1], cp_v, cp_x[2], *cp_w):
        c.start()

    def ln1(r0, r1):
        for r in range(r0, r1, R1):
            rows = pl.ds(r, R1)
            xn_v[rows, :] = _ln(x_v[rows, :].astype(f32)).astype(xn_v.dtype)

    def repack(j):
        if WP:
            wp[j] = pltpu.bitcast(wqkv_v[:, pl.ds(j * D, D)], u32)
        if j != 1 and NTM & (j // 2 + 1):
            wt_v[j // 2] = wqkv_v[:, pl.ds(j * D, D)].T

    weight = lambda j: pltpu.bitcast(wp[j], bf16) if WP else wqkv_v[:, pl.ds(j * D, D)]

    def proj_q(r0, r1):
        qs = []
        for r in range(r0, r1, R1):
            if NTM & 1:
                qt = _mm_nt(wt_v[0], xn_v[pl.ds(r, R1), :]) * Q_SCALE
                qt_v[:, pl.ds(r, R1)] = qt
                qs.append(jnp.concatenate([qt[i * R1:(i + 1) * R1] for i in range(D // R1)], axis=1))
                continue
            q = _mm(xn_v[pl.ds(r, R1), :], weight(0)) * Q_SCALE
            qt_v[:, pl.ds(r, R1)] = q.T
            qs.append(q)
        return qs

    def spread(results, n):
        per = 4 * (R1 // 8)
        picks = [divmod(i * len(results) * per // n, per) for i in range(n)]
        return [None if results[b] is None else
                results[b][p % (R1 // 8) * 8:p % (R1 // 8) * 8 + 8, p // (R1 // 8) * 128:(p // (R1 // 8) + 1) * 128]
                for b, p in picks]

    def proj_k(r0, r1):
        for r in range(r0, r1, R1):
            k = _mm(xn_v[pl.ds(r, R1), :], weight(1))
            kp = pltpu.bitcast(k.astype(bf16), u32)
            for g in range(D // 128):
                lanes = slice(g * 128, (g + 1) * 128)
                k_p[g, pl.ds(r // 2, R1 // 2), :] = kp[:, lanes]
                for c in range(r // CK, (r + R1) // CK):
                    ko_v[g, pl.ds(V0[c], NV[c]), :] = k[(c + 1) * CK - NV[c] - r:(c + 1) * CK - r, lanes]

    def proj_v(r0, r1):
        vs = []
        for r in range(r0, r1, R1):
            if NTM & 2:
                vt = _mm_nt(wt_v[1], xn_v[pl.ds(r, R1), :])
                vt_p[:, pl.ds(r, R1)] = pltpu.bitcast(vt.astype(bf16), u32)
                vs.append(jnp.concatenate([vt[i * R1:(i + 1) * R1] for i in range(D // R1)], axis=1))
                continue
            v = _mm(xn_v[pl.ds(r, R1), :], weight(2))
            vt = v.astype(bf16).T if VB else v.T.astype(bf16)
            vt_p[:, pl.ds(r, R1)] = pltpu.bitcast(vt, u32)
            vs.append(v)
        return vs

    def tie(x, src):
        if src is None:
            return x
        reps = (x.shape[0] // 8, x.shape[1] // 128)
        src = src[0:8, 0:128]
        src = src if x.dtype == src.dtype else pltpu.bitcast(src, x.dtype)
        return jnp.where(jnp.tile(z_v[...], reps) >= 0.0, x, jnp.tile(src, reps))

    lane = jax.lax.broadcasted_iota(i32, (8, 128), 1)

    def stage_mxu_keys(h, u, c, after=lambda x: x):
        idx = after((lane + (h % 8) * DH) & 127)
        kp = k_p[h // 8, pl.ds(c * CK // 2, NT[c] * 8), :]
        km[u, pl.ds(T0[c] * 8, NT[c] * 8), :] = _take(kp, jnp.tile(idx, (NT[c], 1)), axis=1)
        if c == 0:
            idx = (idx + (128 - DH)) & 127
            moved = _take(kp[(NT[c] - OFF) * 8:], jnp.tile(idx, (OFF, 1)), axis=1)
            ln = jnp.tile(lane, (OFF, 1))
            kx[u] = jnp.where((ln >= DH) & (ln < 2 * DH), moved, 0)

    def stage_values(h, u):
        vw[u] = vt_p[pl.ds(_mo(h * (DH // 2), DH // 2), DH // 2), :]

    def stage_vpu_keys(h, u, d, after=lambda x: x):
        idx = after(jnp.full((8, 128), (h % 8) * DH + d, i32))
        kb[u, d] = _take(ko_v[h // 8], jnp.tile(idx, (V0[NC] // 8, 1)), axis=1)

    def stage_query(h, u, b, d, after=lambda x: x):
        q = qt_v[pl.ds(_mo(h * DH + d // 8 * 8, 8), 8), pl.ds(b * TQ, TQ)]
        idx = after(jnp.full((8, 128), d % 8, i32))
        for n in range(NQ):
            qb[u, b, d, :, pl.ds(n * 128, 128)] = _take(q[:, n * 128:(n + 1) * 128], idx, axis=0)
        if d % 8 == 0:
            qw[u, b, pl.ds(d, 8), :] = q

    z_v[...] = jnp.zeros((8, 128), f32)
    with jax.named_scope("wait0"):
        cp_x[0].wait()
        ln1(0, XA)
        cp_k.wait()
    with jax.named_scope("phase1"):
        on = ONLY in (0, 1, 4)
        repack(1)
        if on:
            proj_k(0, XA)
        cp_q.wait()
        cp_x[1].wait()
        repack(0)
        if on:
            ln1(XA, 2 * XA)
            proj_q(0, XA)
            proj_k(XA, 2 * XA)
        cp_v.wait()
        cp_x[2].wait()
        repack(2)
        if on:
            ln1(2 * XA, S)
            proj_q(XA, 2 * XA)
            proj_v(0, XA)
            proj_k(2 * XA, S)

        def stage_keys(heads, results):
            marks = iter(spread(results, len(heads) * (NC + DH)))
            for u in heads:
                for c in range(NC):
                    stage_mxu_keys(u, u, c, functools.partial(tie, src=next(marks)))
                for d in range(DH):
                    stage_vpu_keys(u, u, d, functools.partial(tie, src=next(marks)))
        for c in cp_w:
            c.wait()
        pieces = [(src, dst, r, c) for src, dst in ((wo_v, wo7), (w1_v, w17), (w2_v, w27))
                  for r in range(0, src.shape[0] // 2, PR) for c in range(0, src.shape[1] // 2, 128)]
        qs = proj_q(2 * XA, S) if on else [None]
        vs = proj_v(XA, S) if on else [None] * 2
        stage_keys(range(KQ), qs)
        stage_keys(range(KQ, HU - 1), vs[:-1])
        marks = iter(spread(vs[:-1], HU * NB * DH))
        for u in range(HU):
            for b in range(NB):
                for d in range(DH):
                    stage_query(u, u, b, d, functools.partial(tie, src=next(marks)))
        for (src, dst, r, c), wait_for in zip(pieces, spread(qs + vs[:-1], len(pieces))):
            kh, nh = src.shape[0] // 2, src.shape[1] // 2
            quad = []
            for i in range(2):
                for j in range(2):
                    w = pltpu.bitcast(src[pl.ds(r + i * kh, PR), pl.ds(j * nh + c, 128)], u32)
                    quad.append(pltpu.bitcast(tie(w, wait_for), bf16).astype(f32))
            for i, op in enumerate(_rhs7(*quad)):
                dst[i, pl.ds(r // 2, PR // 2), pl.ds(c, 128)] = pltpu.bitcast(op.astype(bf16), u32)
        for u in range(HU - 1):
            stage_values(u, u)

    def fast_step(it, carry):
        lo, hi, big = carry
        items = [(u, b, c) for u in range(HU) for b in range(NB) for c in range(NC)]
        tiles = [(n, t) for n, (u, b, c) in enumerate(items) for t in range(NT[c])]
        first = [n // NC * T0[NC] + T0[c] for n, (u, b, c) in enumerate(items)] + [len(tiles)]
        outs = [(n, q, r) for n, (u, b, c) in enumerate(items) for r in reversed(range(NV[c] // 8)) for q in range(NQ)]
        ties = {}
        for o, key in enumerate(outs):
            ties.setdefault((o * len(tiles)) // len(outs) + TSH, []).append(key)
        head = lambda u: it * HU + u
        later = lambda u: jnp.minimum(it + 1, H // HU - 1) * HU + u
        zero = z_v[...]
        always = zero >= 0.0
        sv, st = {}, {}

        def vpu_scores(n, q, r):
            if (n, q, r) not in sv:
                u, b, c = items[n]
                acc = None
                for d in range(DH):
                    t = kb[u, d, pl.ds(V0[c] + r * 8, 8), :] * qb[u, b, d, :, pl.ds(q * 128, 128)]
                    acc = t if acc is None else acc + t
                sv[n, q, r] = acc
            return sv[n, q, r]

        def key_tile(g, moved=False):
            n, t = tiles[g]
            u, b, c = items[n]
            if moved:
                kt = kx[u, pl.ds((OFF - 1 - t) * 8, 8), :]
            else:
                kt = km[u, pl.ds((T0[c + 1] - 1 - t) * 8, 8), :]
            for key in ties.get(g, ()):
                kt = jnp.where(always, kt, pltpu.bitcast(vpu_scores(*key), u32))
            return kt

        def mxu_scores(g0, g1):
            u0, b0, _ = items[tiles[g0][0]]
            u1, b1, _ = items[tiles[g1 - 1][0]]
            if (u0, b0) != (u1, b1):
                e = g1 // T0[NC] * T0[NC]
                lhs = [jnp.where(lane < DH, key_tile(g), 0) for g in range(g0, e)]
                lhs += [key_tile(g, True) for g in range(e, g1)]
                w = [qw[u0, b0], qw[u1, b1]]
            else:
                lhs = [key_tile(g) for g in range(g0, g1)]
                w = [qw[u0, b0]]
            w = jnp.concatenate(w + [jnp.zeros((128 - DH * len(w), TQ), f32)], axis=0)
            s = _mm(pltpu.bitcast(jnp.concatenate(lhs, axis=0), bf16), w)
            for g in range(g0, g1):
                st[g] = s[(g - g0) * 16:(g - g0 + 1) * 16]

        def weigh(n, l, acc):
            u, b, c = items[n]
            rows = [st.pop(first[n + 1] - 1 - t) for t in range(NT[c])]
            rows += [jnp.concatenate([vpu_scores(n, q, r) for q in range(NQ)], axis=1) for r in range(NV[c] // 8)]
            p = jnp.exp2(jnp.concatenate(rows, axis=0))
            for r in reversed(range(CK // 8)):
                row = p[r * 8:(r + 1) * 8]
                l = row if l is None else l + row
            o = _mm(pltpu.bitcast(vw[u, :, pl.ds(c * CK, CK)], bf16), p)
            return l, (o if acc is None else acc + o)

        bound = lambda m: len(tiles) if m >= len(items) else first[m] + OFF
        l = acc = None
        for m in range(len(items) + 1):
            g0, g1 = bound(m) if m else 0, bound(m + 1)
            if g0 < g1:
                mxu_scores(g0, g1)
            if m == 0:
                continue
            u, b, c = items[m - 1]
            if c == 0:
                l = acc = None
            l, acc = weigh(m - 1, l, acc)

            def after(x, l0=l[:, 0:128]):
                return jnp.where(always, x, pltpu.bitcast(l0, i32))
            step, sub = divmod(b * NC + c, KSP)
            if step < NC:
                h_fill = later(u - 1) if u > 0 else head(HU - 1)
                if sub == 0:
                    stage_vpu_keys(h_fill, (u - 1) % HU, step, after)
                if sub == KSP - 1:
                    stage_mxu_keys(h_fill, (u - 1) % HU, step, after)
                    if step == 0:
                        stage_values(h_fill, (u - 1) % HU)
            blk = u * NB + b
            if blk > 0:
                stage_query(later((blk - 1) // NB), (blk - 1) // NB, (blk - 1) % NB, c, after)
            if c == NC - 1:
                ot_v[pl.ds(_mo(head(u) * DH, DH), DH), pl.ds(b * TQ, TQ)] = acc
                l_v[head(u), :, pl.ds(b * TQ, TQ)] = l
                for q in range(NQ):
                    cols = slice(q * 128, (q + 1) * 128)
                    lo = jnp.minimum(lo, l[:, cols])
                    hi = jnp.maximum(hi, l[:, cols])
                    big = jnp.maximum(big, jnp.maximum(jnp.abs(acc[0:8, cols]), jnp.abs(acc[8:16, cols])))
        for d in range(DH):
            stage_query(later(HU - 1), HU - 1, NB - 1, d, after)
        return lo, hi, big

    one = jnp.ones((8, 128), f32)
    with jax.named_scope("phase2"):
        lo, hi, big = one, one, one
        if ONLY in (0, 2):
            lo, hi, big = jax.lax.fori_loop(0, H // HU, fast_step, (lo, hi, big))
        else:
            def dummy(i, c):
                z_v[...] = jnp.abs(z_v[...])
                l_v[i] = l_v[i] + 1.0
                if ONLY == 4:
                    for ref in (wo7, w17, w27, km, kb, qb, qw, vw, kx, ko_v, k_p):
                        idx = (i,) + (0,) * (len(ref.shape) - 3) + (slice(0, 8), slice(0, 128))
                        z_v[...] = z_v[...] + ref[idx].astype(f32)
                    z_v[...] = z_v[...] + vt_p[pl.ds(_mo(i * 8, 8), 8), 0:128].astype(f32) + qt_v[pl.ds(_mo(i * 8, 8), 8), 0:128]
                return c
            jax.lax.fori_loop(0, 2, dummy, 0)
    safe = (lo >= L_MIN) & (hi <= L_MAX) & (big <= A_MAX)

    @pl.when(jnp.max(jnp.where(safe, float(FORCE_SAFE), 1.0)) > 0.0)
    def _():
        def safe_step(i, carry):
            h, b = i // (S // TS), i % (S // TS)
            cols = pl.ds(_mo(b * TS, TS), TS)
            q = qt_v[pl.ds(_mo(h * DH, DH), DH), cols]
            row_head = jax.lax.broadcasted_iota(i32, (128, TS), 0) // DH
            qm = jnp.where(row_head == h % 8, jnp.tile(q, (8, 1)), 0.0)
            s = _mm(pltpu.bitcast(k_p[h // 8], bf16), qm)
            p = jnp.exp2(s - jnp.max(s, axis=0, keepdims=True))
            v = pltpu.bitcast(vt_p[pl.ds(_mo(h * (DH // 2), DH // 2), DH // 2), :], bf16)
            ot_v[pl.ds(_mo(h * DH, DH), DH), cols] = _mm(v, p)
            l_v[h, :, cols] = jnp.sum(p.reshape(S // 8, 8, TS), axis=0)
            return carry
        jax.lax.fori_loop(0, H * (S // TS), safe_step, 0)

    b1 = b1_ref[...].astype(f32).reshape(1, F)
    b2 = b2_ref[...].astype(f32).reshape(1, D)
    RH, DQ, FH = R3 // 2, D // 2, F // 2

    def out_copy(i):
        rows = pl.ds(i * R3, R3)
        return pltpu.make_async_copy(out_v.at[rows], out_hbm.at[rows], out_sem.at[i])

    def quadrants(i):
        return [(pl.ds(i * R3 + r * RH, RH), pl.ds(c * DQ, DQ)) for r in range(2) for c in range(2)]

    def normalize(i, srcs=(None,)):
        rows = pl.ds(i * R3, R3)
        ot = []
        for h in range(H):
            lsum = jnp.sum(tie(l_v[h, :, rows], srcs[h * len(srcs) // H]), axis=0, keepdims=True)
            inv = pl.reciprocal(lsum, approx=True)
            ot.append(ot_v[pl.ds(h * DH, DH), rows] * (inv * (2.0 - lsum * inv)))
        o = jnp.concatenate(ot, axis=0).T
        if WO7:
            for j, op in enumerate(_lhs7(o[:RH, :DQ], o[:RH, DQ:], o[RH:, :DQ], o[RH:, DQ:])):
                o7[i % 4, j] = op
        else:
            for j, op in enumerate((o[:RH, :DQ], o[:RH, DQ:], o[RH:, :DQ], o[RH:, DQ:])):
                o7[i % 4, j] = op

    def out_proj(i):
        if WO7:
            ys = _join7([_mm(o7[i % 4, j], pltpu.bitcast(wo7[j], bf16)) for j in range(7)])
        else:
            o = jnp.concatenate([jnp.concatenate([o7[i % 4, 2 * r], o7[i % 4, 2 * r + 1]], axis=1) for r in range(2)], axis=0)
            y = _mm(o, wo_v[...])
            ys = (y[:RH, :DQ], y[:RH, DQ:], y[RH:, :DQ], y[RH:, DQ:])
        for q, y in zip(quadrants(i), ys):
            h_v[q] = x_v[q].astype(f32) + y

    def ln2(i, srcs=(None,)):
        step = RH // len(srcs)
        for n, src in enumerate(srcs):
            halves = []
            for r in range(2):
                hid = h_v[pl.ds(i * R3 + r * RH + n * step, step), :]
                hid = jnp.concatenate([tie(hid[:, 0:128], src), hid[:, 128:]], axis=1)
                halves.append(_ln(hid))
            top, bot = halves
            for j, op in enumerate(_lhs7(top[:, :DQ], top[:, DQ:], bot[:, :DQ], bot[:, DQ:])):
                hn7[i % 4, j, pl.ds(n * step, step), :] = op

    def ffn_up(i, f0):
        w = min(FC, FH - f0)
        ms = {j: _mm(hn7[i % 4, j], pltpu.bitcast(w17[j, :, pl.ds(f0, w)], bf16)) for j in ORD}
        bias = [b1[:, f0:f0 + w], b1[:, FH + f0:FH + f0 + w]] * 2
        act = [_gelu(a + bb) for a, bb in zip(_join7(ms), bias)]
        for j, op in enumerate(_lhs7(*act)):
            g7[i % 2, j, :, pl.ds(f0, w)] = _pack(op)

    def ffn_down(i, j):
        return _mm(g7[i % 2, j], pltpu.bitcast(w27[j], bf16))

    def finish(i, ms):
        for q, y, bb in zip(quadrants(i), _join7(ms), [b2[:, :DQ], b2[:, DQ:]] * 2):
            out_v[q] = (h_v[q] + y + bb).astype(out_v.dtype)
        out_copy(i).start()

    with jax.named_scope("phase3"):
        if ONLY in (0, 3):
            normalize(0)
            out_proj(0)
            normalize(1)
            out_proj(1)
            ln2(0)
            for i in range(n3):
                for f0 in range(0, FH, FC):
                    ffn_up(i, f0)
                if 0 < i < n3 - 1:
                    out_proj(i + 1)
                ms = [ffn_down(i, j) for j in range(7)]
                if i + 1 < n3:
                    ln2(i + 1, [None, ms[0], ms[1], ms[2]] if MIX & 1 else [ms[0], ms[1], ms[2], ms[3]])
                if i + 2 < n3:
                    normalize(i + 2, [ms[3], ms[4], ms[5], ms[6]] if MIX & 2 else [ms[2], ms[3], ms[4], ms[5]])
                finish(i, ms)
        else:
            for i in range(n3):
                out_copy(i).start()
    with jax.named_scope("tail"):
        for i in range(n3):
            out_copy(i).wait()


@jax.jit
def pallas_sequential_preLN__softmax_full_mha__dense_activation_gelu__prompt_kernel(
        A_x, A_wqkv, A_wo, B_x, B_w1, B_b1, B_w2, B_b2):
    del B_x
    any_spec = pl.BlockSpec(memory_space=pl.ANY)
    vmem_spec = pl.BlockSpec(memory_space=pltpu.VMEM)
    vm = pltpu.VMEM
    out = pl.pallas_call(
        _kernel,
        out_shape=jax.ShapeDtypeStruct((S, D), A_x.dtype),
        in_specs=[any_spec, any_spec, any_spec, any_spec, vmem_spec, any_spec, vmem_spec],
        out_specs=any_spec,
        scratch_shapes=[
            vm((S, D), bf16), vm((D, 3 * D), bf16), vm((D, D), bf16), vm((D, F), bf16), vm((F, D), bf16),
            vm((3, D // 2, D), u32), vm((2, D, D), bf16), vm((S, D), f32 if XF else bf16),
            vm((D // 128, S // 2, 128), u32), vm((D // 128, V0[NC], 128), f32),
            vm((D, S), f32), vm((D // 2, S), u32), vm((D, S), f32), vm((H, 8, S), f32),
            vm((HU, T0[NC] * 8, 128), u32), vm((HU, OFF * 8, 128), u32), vm((HU, DH, V0[NC], 128), f32),
            vm((HU, NB, DH, TQ), f32), vm((HU, NB, DH, 8, TQ), f32), vm((HU, DH // 2, S), u32),
            vm((8, 128), f32),
            vm((7, D // 4, D // 2), u32), vm((7, D // 4, F // 2), u32), vm((7, F // 4, D // 2), u32),
            vm((4, 7, R3 // 2, D // 2), f32), vm((4, 7, R3 // 2, D // 2), f32), vm((2, 7, R3 // 2, F // 2), f32),
            vm((S, D), f32), vm((S, D), bf16),
            pltpu.SemaphoreType.DMA((9,)), pltpu.SemaphoreType.DMA((S // R3,)),
        ],
        compiler_params=pltpu.CompilerParams(vmem_limit_bytes=100 * 1024 * 1024),
    )(A_x.reshape(S, D), A_wqkv, A_wo, B_w1, B_b1, B_w2, B_b2)
    return out.reshape(A_x.shape)
```

```python
import functools
import jax
import jax.numpy as jnp
import numpy as np
import jax.experimental.pallas as pl
import jax.experimental.pallas.tpu as pltpu

S, D, F, H, DH = 2048, 512, 1792, 32, 16
TQ = 512
NQ = TQ // 128
NB = S // TQ
CK = 128
NC = S // CK
PAT = [16,16,16,16,16,16,16,32]
NV = [PAT[c % len(PAT)] for c in range(NC)]
NT = [(CK - v) // 16 for v in NV]
V0 = [sum(NV[:c]) for c in range(NC + 1)]
T0 = [sum(NT[:c]) for c in range(NC + 1)]
HU = 4
OFF = 2
TSH = 9
KSP = 2
R1 = 256
R3 = 128
U1 = 1
FC = 256
ONLY = 0
FORCE_SAFE = 0
DMAP = 0
RCP = 1
MIX = 3
ORD = [range(7), (1, 3, 2, 4, 0, 5, 6), (0, 1, 3, 2, 4, 5, 6), (4, 2, 3, 1, 0, 6, 5)][0]
WO7 = 1
PR = 16
XF = 1
WP = 0
TORD = 0
NTM = 2
VB = 1
KQ = 1
KP = 16
MP = 16
KSPAN = 32
MID = 7
QA = 0
DYN = 1
ALIVE = 0
CHK = 2
LSPAN = 16
LOFF = 44
DBG = 0
VEXP = 1
VPOS = 1
MOFF = [v if VPOS else 0 for v in NV]
VOFF = [0 if VPOS else CK - v for v in NV]
TS = 128
EPS = 1e-5
L_MIN, L_MAX, A_MAX = 2.0 ** -40, 2.0 ** 40, 2.0 ** 80
bf16, f32, u32, i32 = jnp.bfloat16, jnp.float32, jnp.uint32, jnp.int32
Q_SCALE = float(DH ** -0.5 * np.log2(np.e))


def _mo(x, n):
    return x if isinstance(x, int) else pl.multiple_of(x, n)


def _mm(a, b):
    return jax.lax.dot_general(a, b, (((1,), (0,)), ((), ())), preferred_element_type=f32)


def _mm_nt(a, b):
    return jax.lax.dot_general(a, b, (((1,), (1,)), ((), ())), preferred_element_type=f32)


def _take(x, idx, axis):
    return jnp.take_along_axis(x, idx, axis=axis, mode="promise_in_bounds", wrap_negative_indices=False)


def _pack(x):
    return x


def _lhs7(a11, a12, a21, a22):
    return (a11 + a22, a21 + a22, a11, a22, a11 + a12, a21 - a11, a12 - a22)


def _rhs7(b11, b12, b21, b22):
    return (b11 + b22, b11, b12 - b22, b21 - b11, b22, b11 + b12, b21 + b22)


def _join7(m):
    return (m[0] + m[3] - m[4] + m[6], m[2] + m[4], m[1] + m[3], m[0] - m[1] + m[2] + m[5])


def _ln(x):
    m = jnp.mean(x, axis=-1, keepdims=True)
    xc = x - m
    v = jnp.mean(xc * xc, axis=-1, keepdims=True)
    return xc * jax.lax.rsqrt(v + EPS)


def _gelu(x):
    c = float(np.sqrt(2.0 / np.pi))
    return (0.5 * x) * (1.0 + jnp.tanh(x * (c + (c * 0.044715) * (x * x))))


def _kernel(x_hbm, wqkv_hbm, wo_hbm, w1_hbm, b1_ref, w2_hbm, b2_ref, out_hbm,
            x_v, wqkv_v, wo_v, w1_v, w2_v, wp, wt_v, xn_v, k_p, ko_v, qt_v, vt_p, ot_v, l_v,
            qw, qb, p0_v, pc_v, z_v, wo7, w17, w27, o7, hn7, g7, h_v, out_v, in_sem, out_sem, *slots):
    km, kx, kb, vw = (slots[i * HU:(i + 1) * HU] for i in range(4))
    n1, n3 = S // R1, S // R3

    XA = 512

    def part(src, dst, rows, cols, i):
        return pltpu.make_async_copy(src.at[rows, cols], dst.at[rows, cols], in_sem.at[i])
    every = slice(None)
    cp_x = [part(x_hbm, x_v, pl.ds(r0, n), every, i) for i, (r0, n) in enumerate(((0, XA), (XA, XA), (2 * XA, S - 2 * XA)))]
    cp_q, cp_k, cp_v = [part(wqkv_hbm, wqkv_v, every, pl.ds(i * D, D), 3 + i) for i in range(3)]
    cp_w = [part(src, dst, every, every, 6 + i) for i, (src, dst) in enumerate(((wo_hbm, wo_v), (w1_hbm, w1_v), (w2_hbm, w2_v)))]
    for c in (cp_x[0], cp_k, cp_q, cp_x[1], cp_v, cp_x[2], *cp_w):
        c.start()

    def ln1(r0, r1):
        for r in range(r0, r1, R1):
            rows = pl.ds(r, R1)
            xn_v[rows, :] = _ln(x_v[rows, :].astype(f32)).astype(xn_v.dtype)

    def repack(j):
        if WP:
            wp[j] = pltpu.bitcast(wqkv_v[:, pl.ds(j * D, D)], u32)
        if j != 1 and NTM & (j // 2 + 1):
            wt_v[j // 2] = wqkv_v[:, pl.ds(j * D, D)].T

    weight = lambda j: pltpu.bitcast(wp[j], bf16) if WP else wqkv_v[:, pl.ds(j * D, D)]

    def proj_q(r0, r1):
        qs = []
        for r in range(r0, r1, R1):
            if NTM & 1:
                qt = _mm_nt(wt_v[0], xn_v[pl.ds(r, R1), :]) * Q_SCALE
                qt_v[:, pl.ds(r, R1)] = qt
                qs.append(jnp.concatenate([qt[i * R1:(i + 1) * R1] for i in range(D // R1)], axis=1))
                continue
            q = _mm(xn_v[pl.ds(r, R1), :], weight(0)) * Q_SCALE
            qt_v[:, pl.ds(r, R1)] = q.T
            qs.append(q)
        return qs

    def spread(results, n):
        per = 4 * (R1 // 8)
        picks = [divmod(i * len(results) * per // n, per) for i in range(n)]
        return [None if results[b] is None else
                results[b][p % (R1 // 8) * 8:p % (R1 // 8) * 8 + 8, p // (R1 // 8) * 128:(p // (R1 // 8) + 1) * 128]
                for b, p in picks]

    def proj_k(r0, r1):
        for r in range(r0, r1, R1):
            k = _mm(xn_v[pl.ds(r, R1), :], weight(1))
            kp = pltpu.bitcast(k.astype(bf16), u32)
            for g in range(D // 128):
                lanes = slice(g * 128, (g + 1) * 128)
                k_p[g, pl.ds(r // 2, R1 // 2), :] = kp[:, lanes]
                for c in range(r // CK, (r + R1) // CK):
                    ko_v[g, pl.ds(V0[c], NV[c]), :] = k[c * CK + VOFF[c] - r:c * CK + VOFF[c] + NV[c] - r, lanes]

    peaks = [jnp.zeros((8, 128), f32)] * 2

    def v_peak(v):
        for n in range(v.shape[1] // 128):
            for r in range(0, v.shape[0], 8):
                peaks[n % 2] = jnp.maximum(peaks[n % 2], jnp.abs(v[r:r + 8, n * 128:(n + 1) * 128]))

    def proj_v(r0, r1):
        vs = []
        for r in range(r0, r1, R1):
            if NTM & 2:
                vt = _mm_nt(wt_v[1], xn_v[pl.ds(r, R1), :])
                vt_p[:, pl.ds(r, R1)] = pltpu.bitcast(vt.astype(bf16), u32)
                v_peak(vt)
                vs.append(jnp.concatenate([vt[i * R1:(i + 1) * R1] for i in range(D // R1)], axis=1))
                continue
            v = _mm(xn_v[pl.ds(r, R1), :], weight(2))
            vt = v.astype(bf16).T if VB else v.T.astype(bf16)
            vt_p[:, pl.ds(r, R1)] = pltpu.bitcast(vt, u32)
            v_peak(v)
            vs.append(v)
        return vs

    def tie(x, src):
        if src is None:
            return x
        reps = (x.shape[0] // 8, x.shape[1] // 128)
        src = src[0:8, 0:128]
        src = src if x.dtype == src.dtype else pltpu.bitcast(src, x.dtype)
        return jnp.where(jnp.tile(z_v[...], reps) >= 0.0, x, jnp.tile(src, reps))

    lane = jax.lax.broadcasted_iota(i32, (8, 128), 1)

    key_tiles = [(c, t) for c in range(NC) for t in range(NT[c])]

    def stage_mxu_keys(h, u, part, parts, after=lambda x: x, zero=0):
        mine = range(part * len(key_tiles) // parts, (part + 1) * len(key_tiles) // parts)
        idx = after((lane + (h % 8) * DH) & 127)
        for g in mine:
            c, t = key_tiles[g]
            kp = k_p[h // 8, pl.ds((c * CK + MOFF[c]) // 2 + t * 8, 8), :]
            km[u][pl.ds(_mo((g + zero) * 8, 8), 8), :] = _take(kp, idx, axis=1)
            if c == 0 and t >= NT[0] - OFF:
                moved = _take(kp, (idx + (128 - DH)) & 127, axis=1)
                kx[u][pl.ds(_mo((t - NT[0] + OFF + zero) * 8, 8), 8), :] = jnp.where((lane >= DH) & (lane < 2 * DH), moved, 0)

    def stage_values(h, u, zero=0):
        vw[u][zero] = vt_p[pl.ds(_mo(h * (DH // 2), DH // 2), DH // 2), :]

    def stage_vpu_keys(h, u, part, parts, after=lambda x: x, zero=0):
        d, sub = divmod(part, parts // DH)
        n = V0[NC] // 8
        r0, r1 = sub * n // (parts // DH), (sub + 1) * n // (parts // DH)
        idx = after(jnp.full((8, 128), (h % 8) * DH + d, i32))
        rows = pl.ds(r0 * 8, (r1 - r0) * 8)
        kb[u][d + zero, rows, :] = _take(ko_v[h // 8, rows, :], jnp.tile(idx, (r1 - r0, 1)), axis=1)

    def stage_query(h, u, b, d, after=lambda x: x):
        q = qt_v[pl.ds(_mo(h * DH + d // 8 * 8, 8), 8), pl.ds(b * TQ, TQ)]
        idx = after(jnp.full((8, 128), d % 8, i32))
        for n in range(NQ):
            qb[u, b, d, :, pl.ds(n * 128, 128)] = _take(q[:, n * 128:(n + 1) * 128], idx, axis=0)
        if d % 8 == 0:
            qw[u, b, pl.ds(d, 8), :] = q

    z_v[...] = jnp.zeros((8, 128), f32)
    with jax.named_scope("wait0"):
        cp_x[0].wait()
        ln1(0, XA)
        cp_k.wait()
    with jax.named_scope("phase1"):
        on = ONLY in (0, 1, 4)
        repack(1)
        if on:
            proj_k(0, XA)
        cp_q.wait()
        cp_x[1].wait()
        repack(0)
        if on:
            ln1(XA, 2 * XA)
            proj_q(0, XA)
            proj_k(XA, 2 * XA)
        cp_v.wait()
        cp_x[2].wait()
        repack(2)
        if on:
            ln1(2 * XA, S)
            proj_q(XA, 2 * XA)
            proj_v(0, XA)
            proj_k(2 * XA, S)

        def stage_keys(heads, results):
            marks = iter(spread(results, len(heads) * (NC + DH)))
            for u in heads:
                for c in range(NC):
                    stage_mxu_keys(u, u, c, NC, functools.partial(tie, src=next(marks)))
                for d in range(DH):
                    stage_vpu_keys(u, u, d, DH, functools.partial(tie, src=next(marks)))
        for c in cp_w:
            c.wait()
        pieces = [(src, dst, r, c) for src, dst in ((wo_v, wo7), (w1_v, w17), (w2_v, w27))
                  for r in range(0, src.shape[0] // 2, PR) for c in range(0, src.shape[1] // 2, 128)]
        qs = proj_q(2 * XA, S) if on else [None]
        vs = proj_v(XA, S) if on else [None] * 2
        stage_keys(range(KQ), qs)
        stage_keys(range(KQ, HU - 1), vs[:-1])
        marks = iter(spread(vs[:-1], HU * NB * DH))
        for u in range(HU):
            for b in range(NB):
                for d in range(DH):
                    stage_query(u, u, b, d, functools.partial(tie, src=next(marks)))
        for (src, dst, r, c), wait_for in zip(pieces, spread(qs + vs[:-1], len(pieces))):
            kh, nh = src.shape[0] // 2, src.shape[1] // 2
            quad = []
            for i in range(2):
                for j in range(2):
                    w = pltpu.bitcast(src[pl.ds(r + i * kh, PR), pl.ds(j * nh + c, 128)], u32)
                    quad.append(pltpu.bitcast(tie(w, wait_for), bf16).astype(f32))
            for i, op in enumerate(_rhs7(*quad)):
                dst[i, pl.ds(r // 2, PR // 2), pl.ds(c, 128)] = pltpu.bitcast(op.astype(bf16), u32)
        for u in range(HU - 1):
            stage_values(u, u)

    def query_weights(*blocks):
        w = [qw[u, b] for u, b in blocks]
        return jnp.concatenate(w + [jnp.zeros((128 - DH * len(w), TQ), f32)], axis=0)

    def finish_step(it, acc, v):
        h = it * HU + HU - 1
        acc = acc + _mm(pltpu.bitcast(v, bf16), pc_v[...])
        ot_v[pl.ds(_mo(h * DH, DH), DH), pl.ds((NB - 1) * TQ, TQ)] = acc

    def fast_step(it, carry):
        items = [(u, b, c) for u in range(HU) for b in range(NB) for c in range(NC)]
        tiles = [(u, b, c, t) for u, b, c in items for t in range(NT[c])]
        first = [n // NC * T0[NC] + T0[c] for n, (u, b, c) in enumerate(items)] + [len(tiles)]
        outs = [(n, q, r) for n, (u, b, c) in enumerate(items) for r in reversed(range(NV[c] // 8)) for q in range(NQ)]
        ties = {}
        for o, key in enumerate(outs):
            ties.setdefault(max((o * len(tiles)) // len(outs) + TSH, OFF), []).append(key)
        tiles += tiles[:OFF] if not DBG & 1 else [(HU - 1, 0) + t[2:] for t in tiles[:OFF]]
        head = lambda u: it * HU + u
        later = lambda u: jnp.minimum(it + 1, H // HU - 1) * HU + u
        always = z_v[...] >= 0.0
        sv, st = {}, {}

        def vpu_scores(n, q, r):
            if (n, q, r) not in sv:
                u, b, c = items[n]
                acc = None
                for d in range(DH):
                    t = kb[u][d, pl.ds(V0[c] + r * 8, 8), :] * qb[u, b, d, :, pl.ds(q * 128, 128)]
                    acc = t if acc is None else acc + t
                sv[n, q, r] = jnp.exp2(acc) if VEXP else acc
            return sv[n, q, r]

        def key_tile(g, moved=False):
            u, b, c, t = tiles[g]
            if moved:
                kt = kx[u][pl.ds((OFF - 1 - t) * 8, 8), :]
            else:
                kt = km[u][pl.ds((T0[c + 1] - 1 - t) * 8, 8), :]
            for key in ties.get(g, ()):
                kt = jnp.where(always, kt, pltpu.bitcast(vpu_scores(*key), u32))
            return kt

        def mxu_scores(g0, g1):
            if tiles[g0][:2] != tiles[g1 - 1][:2]:
                lhs = [jnp.where(lane < DH, key_tile(g), 0) for g in range(g0, g1 - OFF)]
                lhs += [key_tile(g, True) for g in range(g1 - OFF, g1)]
                w = query_weights(tiles[g0][:2], tiles[g1 - 1][:2])
            else:
                lhs = [key_tile(g) for g in range(g0, g1)]
                w = query_weights(tiles[g0][:2])
            s = _mm(pltpu.bitcast(jnp.concatenate(lhs, axis=0), bf16), w)
            for g in range(g0, g1):
                st[g] = s[(g - g0) * 16:(g - g0 + 1) * 16]

        def weights(n, l):
            c = items[n][2]
            rows = [st.pop(first[n + 1] - 1 - t) for t in range(NT[c])]
            more = [jnp.concatenate([vpu_scores(n, q, r) for q in range(NQ)], axis=1) for r in range(NV[c] // 8)]
            if VEXP:
                rows = [jnp.exp2(jnp.concatenate(rows, axis=0))]
                p = jnp.concatenate(more + rows if VPOS else rows + more, axis=0)
            else:
                p = jnp.exp2(jnp.concatenate(rows + more, axis=0))
            for r in reversed(range(CK // 8)):
                row = p[r * 8:(r + 1) * 8]
                l = row if l is None else l + row
            return p, l

        for g in range(OFF):
            st[g] = p0_v[pl.ds(g * 16, 16), :]
        l = acc = None
        for m in range(len(items) + 1):
            if m < len(items):
                mxu_scores(first[m] + OFF, first[m + 1] + OFF)
            if m == 0:
                finish_step(jnp.maximum(it - 1, 0), *carry)
                continue
            u, b, c = items[m - 1]
            if c == 0:
                l, acc = None, jnp.tile(z_v[...], (DH // 8, NQ))
            p, l = weights(m - 1, l)
            v = vw[u][0, :, pl.ds(c * CK, CK)]
            if m < len(items):
                acc = acc + _mm(pltpu.bitcast(v, bf16), p)
            else:
                late = jnp.tile(p[MOFF[c]:MOFF[c] + 8], (NV[c] // 8, 1))
                keep = jnp.tile(z_v[...], (NV[c] // 8, NQ)) >= 0.0
                pc_v[pl.ds(MOFF[c], CK - NV[c]), :] = p[MOFF[c]:MOFF[c] + CK - NV[c]]
                pc_v[pl.ds(VOFF[c], NV[c]), :] = jnp.where(keep, p[VOFF[c]:VOFF[c] + NV[c]], late)

            def after(x, src=l[:, 0:128]):
                return jnp.where(always, x, pltpu.bitcast(src, i32))

            def after2(x, src=p[MID * 8:MID * 8 + 8, 0:128]):
                return jnp.where(always, x, pltpu.bitcast(src, i32))
            h_fill = later(u - 1) if u > 0 else head(HU - 1)
            zero = jnp.minimum(it, 0) if u == 0 and DYN else 0
            span, n = (LSPAN, b * NC + c - LOFF) if u == HU - 1 else (KSPAN, b * NC + c)
            for part in range(KP):
                if part * span // KP == n:
                    stage_vpu_keys(h_fill, (u - 1) % HU, part, KP, after, zero)
            for part in range(MP):
                if part * span // MP == n:
                    stage_mxu_keys(h_fill, (u - 1) % HU, part, MP, after2, zero)
            if n == 0:
                stage_values(h_fill, (u - 1) % HU, zero)
            blk = u * NB + b
            if blk > 0:
                stage_query(later((blk - 1) // NB), (blk - 1) // NB, (blk - 1) % NB, c, after)
            if c == NC - 1:
                l_v[head(u), :, pl.ds(b * TQ, TQ)] = l
                if m < len(items):
                    ot_v[pl.ds(_mo(head(u) * DH, DH), DH), pl.ds(b * TQ, TQ)] = acc
        for g in range(OFF):
            p0_v[pl.ds(g * 16, 16), :] = st.pop(first[-1] + g)
        for d in range(DH):
            stage_query(later(HU - 1), HU - 1, NB - 1, d, after2)
        return acc, v

    one = jnp.ones((8, 128), f32)
    with jax.named_scope("phase2"):
        big = jnp.maximum(*peaks)
        if ONLY in (0, 2):
            lead = pltpu.bitcast(jnp.concatenate(
                [k_p[0, pl.ds(MOFF[0] // 2 + (NT[0] - 1 - t) * 8, 8), :] for t in range(OFF)], axis=0), bf16)
            p0_v[...] = _mm(lead, query_weights((0, 0)))
            pc_v[...] = jnp.zeros((CK, TQ), f32)
            carry = (jnp.zeros((DH, TQ), f32), jnp.zeros((DH // 2, CK), u32))
            carry = jax.lax.fori_loop(0, H // HU, fast_step, carry)
            finish_step(H // HU - 1, *carry)
        else:
            def dummy(i, c):
                z_v[...] = jnp.abs(z_v[...])
                l_v[i] = l_v[i] + 1.0
                if ONLY == 4:
                    for ref in (wo7, w17, w27, *kb, qb, qw, *vw, ko_v, k_p):
                        idx = (i % ref.shape[0],) + (0,) * (len(ref.shape) - 3) + (slice(0, 8), slice(0, 128))
                        z_v[...] = z_v[...] + ref[idx].astype(f32)
                    z_v[...] = z_v[...] + vt_p[pl.ds(_mo(i * 8, 8), 8), 0:128].astype(f32) + qt_v[pl.ds(_mo(i * 8, 8), 8), 0:128]
                return c
            jax.lax.fori_loop(0, 2, dummy, 0)
    if True:
        los, his = [one] * 4, [one] * 4
        for h in range(H):
            for n in range(S // 128):
                part = l_v[h, :, pl.ds(n * 128, 128)]
                los[n % 4] = jnp.minimum(los[n % 4], part)
                his[n % 4] = jnp.maximum(his[n % 4], part)
        lo = functools.reduce(jnp.minimum, los)
        hi = functools.reduce(jnp.maximum, his)
    if ALIVE:
        j = jnp.max(jnp.where(big > 0.0, 0, 1)).astype(i32)
        u = HU - 1
        keep = kb[u][j, pl.ds(_mo(j * 8, 8), 8), :] + pltpu.bitcast(km[u][pl.ds(_mo(j * 8, 8), 8), :] | kx[u][pl.ds(_mo(j * 8, 8), 8), :] | vw[u][j, :, 0:128], f32)
        big = jnp.where(z_v[...] >= 0.0, big, keep)
    safe = (lo >= L_MIN) & (hi <= L_MAX) & (big <= A_MAX)

    @pl.when(jnp.max(jnp.where(safe, float(FORCE_SAFE), 1.0)) > 0.0)
    def _():
        def safe_step(i, carry):
            h, b = i // (S // TS), i % (S // TS)
            cols = pl.ds(_mo(b * TS, TS), TS)
            q = qt_v[pl.ds(_mo(h * DH, DH), DH), cols]
            row_head = jax.lax.broadcasted_iota(i32, (128, TS), 0) // DH
            qm = jnp.where(row_head == h % 8, jnp.tile(q, (8, 1)), 0.0)
            s = _mm(pltpu.bitcast(k_p[h // 8], bf16), qm)
            p = jnp.exp2(s - jnp.max(s, axis=0, keepdims=True))
            v = pltpu.bitcast(vt_p[pl.ds(_mo(h * (DH // 2), DH // 2), DH // 2), :], bf16)
            ot_v[pl.ds(_mo(h * DH, DH), DH), cols] = _mm(v, p)
            l_v[h, :, cols] = jnp.sum(p.reshape(S // 8, 8, TS), axis=0)
            return carry
        jax.lax.fori_loop(0, H * (S // TS), safe_step, 0)

    b1 = b1_ref[...].astype(f32).reshape(1, F)
    b2 = b2_ref[...].astype(f32).reshape(1, D)
    RH, DQ, FH = R3 // 2, D // 2, F // 2

    def out_copy(i):
        rows = pl.ds(i * R3, R3)
        return pltpu.make_async_copy(out_v.at[rows], out_hbm.at[rows], out_sem.at[i])

    def quadrants(i):
        return [(pl.ds(i * R3 + r * RH, RH), pl.ds(c * DQ, DQ)) for r in range(2) for c in range(2)]

    def normalize(i, srcs=(None,)):
        rows = pl.ds(i * R3, R3)
        ot = []
        for h in range(H):
            lsum = jnp.sum(tie(l_v[h, :, rows], srcs[h * len(srcs) // H]), axis=0, keepdims=True)
            inv = pl.reciprocal(lsum, approx=True)
            ot.append(ot_v[pl.ds(h * DH, DH), rows] * (inv * (2.0 - lsum * inv)))
        o = jnp.concatenate(ot, axis=0).T
        if WO7:
            for j, op in enumerate(_lhs7(o[:RH, :DQ], o[:RH, DQ:], o[RH:, :DQ], o[RH:, DQ:])):
                o7[i % 4, j] = op
        else:
            for j, op in enumerate((o[:RH, :DQ], o[:RH, DQ:], o[RH:, :DQ], o[RH:, DQ:])):
                o7[i % 4, j] = op

    def out_proj(i):
        if WO7:
            ys = _join7([_mm(o7[i % 4, j], pltpu.bitcast(wo7[j], bf16)) for j in range(7)])
        else:
            o = jnp.concatenate([jnp.concatenate([o7[i % 4, 2 * r], o7[i % 4, 2 * r + 1]], axis=1) for r in range(2)], axis=0)
            y = _mm(o, wo_v[...])
            ys = (y[:RH, :DQ], y[:RH, DQ:], y[RH:, :DQ], y[RH:, DQ:])
        for q, y in zip(quadrants(i), ys):
            h_v[q] = x_v[q].astype(f32) + y

    def ln2(i, srcs=(None,)):
        step = RH // len(srcs)
        for n, src in enumerate(srcs):
            halves = []
            for r in range(2):
                hid = h_v[pl.ds(i * R3 + r * RH + n * step, step), :]
                hid = jnp.concatenate([tie(hid[:, 0:128], src), hid[:, 128:]], axis=1)
                halves.append(_ln(hid))
            top, bot = halves
            for j, op in enumerate(_lhs7(top[:, :DQ], top[:, DQ:], bot[:, :DQ], bot[:, DQ:])):
                hn7[i % 4, j, pl.ds(n * step, step), :] = op

    def ffn_up(i, f0):
        w = min(FC, FH - f0)
        ms = {j: _mm(hn7[i % 4, j], pltpu.bitcast(w17[j, :, pl.ds(f0, w)], bf16)) for j in ORD}
        bias = [b1[:, f0:f0 + w], b1[:, FH + f0:FH + f0 + w]] * 2
        act = [_gelu(a + bb) for a, bb in zip(_join7(ms), bias)]
        for j, op in enumerate(_lhs7(*act)):
            g7[i % 2, j, :, pl.ds(f0, w)] = _pack(op)

    def ffn_down(i, j):
        return _mm(g7[i % 2, j], pltpu.bitcast(w27[j], bf16))

    def finish(i, ms):
        for q, y, bb in zip(quadrants(i), _join7(ms), [b2[:, :DQ], b2[:, DQ:]] * 2):
            out_v[q] = (h_v[q] + y + bb).astype(out_v.dtype)
        out_copy(i).start()

    with jax.named_scope("phase3"):
        if ONLY in (0, 3):
            normalize(0)
            out_proj(0)
            normalize(1)
            out_proj(1)
            ln2(0)
            for i in range(n3):
                for f0 in range(0, FH, FC):
                    ffn_up(i, f0)
                if 0 < i < n3 - 1:
                    out_proj(i + 1)
                ms = [ffn_down(i, j) for j in range(7)]
                if i + 1 < n3:
                    ln2(i + 1, [None, ms[0], ms[1], ms[2]] if MIX & 1 else [ms[0], ms[1], ms[2], ms[3]])
                if i + 2 < n3:
                    normalize(i + 2, [ms[3], ms[4], ms[5], ms[6]] if MIX & 2 else [ms[2], ms[3], ms[4], ms[5]])
                finish(i, ms)
        else:
            for i in range(n3):
                out_copy(i).start()
    with jax.named_scope("tail"):
        for i in range(n3):
            out_copy(i).wait()


@jax.jit
def pallas_sequential_preLN__softmax_full_mha__dense_activation_gelu__prompt_kernel(
        A_x, A_wqkv, A_wo, B_x, B_w1, B_b1, B_w2, B_b2):
    del B_x
    any_spec = pl.BlockSpec(memory_space=pl.ANY)
    vmem_spec = pl.BlockSpec(memory_space=pltpu.VMEM)
    vm = pltpu.VMEM
    out = pl.pallas_call(
        _kernel,
        out_shape=jax.ShapeDtypeStruct((S, D), A_x.dtype),
        in_specs=[any_spec, any_spec, any_spec, any_spec, vmem_spec, any_spec, vmem_spec],
        out_specs=any_spec,
        scratch_shapes=[
            vm((S, D), bf16), vm((D, 3 * D), bf16), vm((D, D), bf16), vm((D, F), bf16), vm((F, D), bf16),
            vm((3, D // 2, D), u32), vm((2, D, D), bf16), vm((S, D), f32 if XF else bf16),
            vm((D // 128, S // 2, 128), u32), vm((D // 128, V0[NC], 128), f32),
            vm((D, S), f32), vm((D // 2, S), u32), vm((D, S), f32), vm((H, 8, S), f32),
            vm((HU, NB, DH, TQ), f32), vm((HU, NB, DH, 8, TQ), f32), vm((OFF * 16, TQ), f32), vm((CK, TQ), f32),
            vm((8, 128), f32),
            vm((7, D // 4, D // 2), u32), vm((7, D // 4, F // 2), u32), vm((7, F // 4, D // 2), u32),
            vm((4, 7, R3 // 2, D // 2), f32), vm((4, 7, R3 // 2, D // 2), f32), vm((2, 7, R3 // 2, F // 2), f32),
            vm((S, D), f32), vm((S, D), bf16),
            pltpu.SemaphoreType.DMA((9,)), pltpu.SemaphoreType.DMA((S // R3,)),
            *[vm((T0[NC] * 8, 128), u32)] * HU, *[vm((OFF * 8, 128), u32)] * HU,
            *[vm((DH, V0[NC], 128), f32)] * HU, *[vm((1, DH // 2, S), u32)] * HU,
        ],
        compiler_params=pltpu.CompilerParams(vmem_limit_bytes=100 * 1024 * 1024),
    )(A_x.reshape(S, D), A_wqkv, A_wo, B_w1, B_b1, B_w2, B_b2)
    return out.reshape(A_x.shape)
```

```python
import functools
import jax
import jax.numpy as jnp
import numpy as np
import jax.experimental.pallas as pl
import jax.experimental.pallas.tpu as pltpu

S, D, F, H, DH = 2048, 512, 1792, 32, 16
TQ = 512
NQ = TQ // 128
NB = S // TQ
CK = 128
NC = S // CK
PAT = [16,16,16,16,16,16,16,32]
NV = [PAT[c % len(PAT)] for c in range(NC)]
NT = [(CK - v) // 16 for v in NV]
V0 = [sum(NV[:c]) for c in range(NC + 1)]
T0 = [sum(NT[:c]) for c in range(NC + 1)]
HU = 4
OFF = 2
TSH = 9
KSP = 2
R1 = 256
R3 = 128
U1 = 1
FC = 256
ONLY = 0
FORCE_SAFE = 0
DMAP = 0
RCP = 1
MIX = 3
ORD = [range(7), (1, 3, 2, 4, 0, 5, 6), (0, 1, 3, 2, 4, 5, 6), (4, 2, 3, 1, 0, 6, 5)][0]
WO7 = 1
PR = 16
XF = 1
WP = 0
TORD = 0
NTM = 2
VB = 1
KQ = 2
KP = 16
MP = 16
KSPAN = 32
MID = 7
QA = 0
DYN = 1
ALIVE = 0
CHK = 2
LSPAN = 16
LOFF = 44
DBG = 0
VEXP = 1
VPOS = 1
MOFF = [v if VPOS else 0 for v in NV]
VOFF = [0 if VPOS else CK - v for v in NV]
FEN = 0
SCH = 0
FC2 = 1
KS = 0
QS = 0
LP = 16
LT = 3
PORD = 0
SR = 1
VB4 = 1024
KE = 5
TS = 128
EPS = 1e-5
L_MIN, L_MAX, A_MAX = 2.0 ** -40, 2.0 ** 40, 2.0 ** 80
bf16, f32, u32, i32 = jnp.bfloat16, jnp.float32, jnp.uint32, jnp.int32
Q_SCALE = float(DH ** -0.5 * np.log2(np.e))


def _mo(x, n):
    return x if isinstance(x, int) else pl.multiple_of(x, n)


def _mm(a, b):
    return jax.lax.dot_general(a, b, (((1,), (0,)), ((), ())), preferred_element_type=f32)


def _mm_nt(a, b):
    return jax.lax.dot_general(a, b, (((1,), (1,)), ((), ())), preferred_element_type=f32)


def _take(x, idx, axis):
    return jnp.take_along_axis(x, idx, axis=axis, mode="promise_in_bounds", wrap_negative_indices=False)


def _pack(x):
    return x


def _lhs7(a11, a12, a21, a22):
    return (a11 + a22, a21 + a22, a11, a22, a11 + a12, a21 - a11, a12 - a22)


def _rhs7(b11, b12, b21, b22):
    return (b11 + b22, b11, b12 - b22, b21 - b11, b22, b11 + b12, b21 + b22)


def _join7(m):
    return (m[0] + m[3] - m[4] + m[6], m[2] + m[4], m[1] + m[3], m[0] - m[1] + m[2] + m[5])


def _ln(x):
    m = jnp.mean(x, axis=-1, keepdims=True)
    xc = x - m
    v = jnp.mean(xc * xc, axis=-1, keepdims=True)
    return xc * jax.lax.rsqrt(v + EPS)


def _gelu(x):
    c = float(np.sqrt(2.0 / np.pi))
    return (0.5 * x) * (1.0 + jnp.tanh(x * (c + (c * 0.044715) * (x * x))))


def _kernel(x_hbm, wqkv_hbm, wo_hbm, w1_hbm, b1_hbm, w2_hbm, b2_hbm, out_hbm,
            x_v, wqkv_v, wo_v, w1_v, w2_v, wq7, wk7, wv7, wt_v, wtq_v, xn_v, xn7, k_p, ko_v, qt_v, vt_p, ot_v, l_v,
            ks_v, qw, qb, p0_v, pc_v, z_v, wo7, w17, w27, o7, hn7, g7, h_v, out_v, in_sem, out_sem, *slots):
    km, kx, kb, vw = (slots[i * HU:(i + 1) * HU] for i in range(4))
    b1_ref, b2_ref = slots[4 * HU:]
    n3 = S // R3
    wqk7 = (wq7, wk7)

    XA = 512

    def part(src, dst, rows, cols, i):
        return pltpu.make_async_copy(src.at[rows, cols], dst.at[rows, cols], in_sem.at[i])
    every = slice(None)
    cp_x = [part(x_hbm, x_v, pl.ds(r0, n), every, i) for i, (r0, n) in enumerate(((0, XA), (XA, XA), (2 * XA, S - 2 * XA)))]
    cp_q, cp_k, cp_v = [part(wqkv_hbm, wqkv_v, every, pl.ds(i * D, D), 3 + i) for i in range(3)]
    cp_w = [part(src, dst, every, every, 6 + i) for i, (src, dst) in enumerate(((wo_hbm, wo_v), (w1_hbm, w1_v), (w2_hbm, w2_v)))]
    cp_w += [pltpu.make_async_copy(src, dst, in_sem.at[9 + i]) for i, (src, dst) in enumerate(((b1_hbm, b1_ref), (b2_hbm, b2_ref)))]
    for c in (cp_x[0], cp_k, cp_q, cp_x[1], cp_v, cp_x[2], *cp_w):
        c.start()

    DQ, H1 = D // 2, R1 // 2

    def tie(x, src):
        if src is None:
            return x
        reps = (x.shape[0] // 8, x.shape[1] // 128)
        src = src[0:8, 0:128]
        src = src if x.dtype == src.dtype else pltpu.bitcast(src, x.dtype)
        return jnp.where(jnp.tile(z_v[...], reps) >= 0.0, x, jnp.tile(src, reps))

    def spread(results, n):
        if not results:
            return [None] * n
        tiles = [(y, r, c) for y in results for c in range(0, y.shape[1], 128) for r in range(0, y.shape[0], 8)]
        picks = [tiles[i * len(tiles) // n] for i in range(n)]
        return [y[r:r + 8, c:c + 128] for y, r, c in picks]

    def ln1(r0, r1, plain=False, results=()):
        pieces = [(i, r) for i in range(r0 // R1, r1 // R1) for r in range(0, H1, LP)]
        for (i, r), src in zip(pieces, spread(results, len(pieces))):
            halves = []
            for half in range(2):
                rows = pl.ds(i * R1 + half * H1 + r, LP)
                x = x_v[rows, :].astype(f32)
                halves.append(_ln(jnp.concatenate([tie(x[:, 0:128], src), x[:, 128:]], axis=1)))
                if plain:
                    xn_v[rows, :] = halves[-1]
            if plain:
                continue
            top, bot = halves
            for j, op in enumerate(_lhs7(top[:, :DQ], top[:, DQ:], bot[:, :DQ], bot[:, DQ:])):
                xn7[i, j, pl.ds(r, LP), :] = op

    def split_rows(r1, results):
        pieces = [(i, r) for i in range(r1 // R1) for r in range(0, H1, LP)]
        for (i, r), src in zip(pieces, spread(results, len(pieces))):
            top, bot = (tie(xn_v[pl.ds(i * R1 + half * H1 + r, LP), :], src) for half in range(2))
            for j, op in enumerate(_lhs7(top[:, :DQ], top[:, DQ:], bot[:, :DQ], bot[:, DQ:])):
                xn7[i, j, pl.ds(r, LP), :] = op

    def split_weights(jobs, results, order=(0, 1, 2, 3)):
        pieces = [(src, c0, n, dst, r, c) for src, c0, n, dst in jobs
                  for r in range(0, src.shape[0] // 2, 16) for c in range(0, n // 2, 128)]
        for (src, c0, n, dst, r, c), wait_for in zip(pieces, spread(results, len(pieces))):
            quad = []
            for i in range(2):
                for j in range(2):
                    w = pltpu.bitcast(src[pl.ds(r + i * src.shape[0] // 2, 16), pl.ds(c0 + j * n // 2 + c, 128)], u32)
                    quad.append(pltpu.bitcast(tie(w, wait_for), bf16).astype(f32))
            for i, op in enumerate(_rhs7(*[quad[o] for o in order])):
                dst[i, pl.ds(r // 2, 8), pl.ds(c, 128)] = pltpu.bitcast(op.astype(bf16), u32)

    def project(which, i, plain):
        if plain:
            y = _mm(xn_v[pl.ds(i * R1, R1), :], wqkv_v[:, pl.ds(which * D, D)])
            return y, [y]
        ms = [_mm(xn7[i, j], pltpu.bitcast(wqk7[which][j], bf16)) for j in range(7)]
        c11, c12, c21, c22 = _join7(ms)
        return jnp.concatenate([jnp.concatenate([c11, c12], axis=1), jnp.concatenate([c21, c22], axis=1)], axis=0), ms

    def project_t(w7, i):
        ms = [_mm_nt(pltpu.bitcast(w7[j], bf16), xn7[i, j]) for j in range(7)]
        c11, c12, c21, c22 = _join7(ms)
        return jnp.concatenate([jnp.concatenate([c11, c21], axis=1), jnp.concatenate([c12, c22], axis=1)], axis=0), ms

    def proj_q(r0, r1, plain=False):
        made = []
        for i in range(r0 // R1, r1 // R1):
            if plain:
                q, ms = project(0, i, plain)
                qt = q.T
            else:
                qt, ms = project_t(wq7, i)
            qt_v[:, pl.ds(i * R1, R1)] = qt * Q_SCALE
            made += ms
        return made

    def proj_k(r0, r1, plain=False):
        made = []
        for i in range(r0 // R1, r1 // R1):
            k, ms = project(1, i, plain)
            kp = pltpu.bitcast(k.astype(bf16), u32)
            for g in range(D // 128):
                lanes = slice(g * 128, (g + 1) * 128)
                k_p[g, pl.ds(i * R1 // 2, R1 // 2), :] = kp[:, lanes]
                for c in range(i * R1 // CK, (i + 1) * R1 // CK):
                    r = c * CK + VOFF[c] - i * R1
                    ko_v[g, pl.ds(V0[c], NV[c]), :] = k[r:r + NV[c], lanes]
            made += ms
        return made

    peaks = [jnp.zeros((8, 128), f32)] * 2

    def proj_v(r0, r1):
        made = []
        for i in range(r0 // R1, r1 // R1):
            vt, ms = project_t(wv7, i)
            vt_p[:, pl.ds(i * R1, R1)] = pltpu.bitcast(vt.astype(bf16), u32)
            for n in range(R1 // 128):
                for r in range(0, D, 8):
                    peaks[n % 2] = jnp.maximum(peaks[n % 2], jnp.abs(vt[r:r + 8, n * 128:(n + 1) * 128]))
            made += ms
        return made

    lane = jax.lax.broadcasted_iota(i32, (8, 128), 1)

    key_tiles = [(c, t) for c in range(NC) for t in range(NT[c])]

    def stage_mxu_keys(h, u, part, parts, after=lambda x: x, zero=0):
        mine = range(part * len(key_tiles) // parts, (part + 1) * len(key_tiles) // parts)
        idx = after((lane + (h % 8) * DH) & 127)
        for g in mine:
            c, t = key_tiles[g]
            kp = k_p[h // 8, pl.ds((c * CK + MOFF[c]) // 2 + t * 8, 8), :]
            km[u][pl.ds(_mo((g + zero) * 8, 8), 8), :] = _take(kp, idx, axis=1)
            if c == 0 and t >= NT[0] - OFF:
                moved = _take(kp, (idx + (128 - DH)) & 127, axis=1)
                kx[u][pl.ds(_mo((t - NT[0] + OFF + zero) * 8, 8), 8), :] = jnp.where((lane >= DH) & (lane < 2 * DH), moved, 0)

    def stage_values(h, u, zero=0):
        vw[u][zero] = vt_p[pl.ds(_mo(h * (DH // 2), DH // 2), DH // 2), :]

    def stage_vpu_keys(h, u, part, parts, after=lambda x: x, zero=0):
        d, sub = divmod(part, parts // DH)
        n = V0[NC] // 8
        r0, r1 = sub * n // (parts // DH), (sub + 1) * n // (parts // DH)
        idx = after(jnp.full((8, 128), (h % 8) * DH + d, i32))
        rows = pl.ds(r0 * 8, (r1 - r0) * 8)
        if KS:
            if d == 0:
                ks_v[u, rows, :] = ko_v[h // 8, rows, :]
            src = ks_v[u, rows, :]
        else:
            src = ko_v[h // 8, rows, :]
        kb[u][d + zero, rows, :] = _take(src, jnp.tile(idx, (r1 - r0, 1)), axis=1)

    def stage_query(h, u, b, d, after=lambda x: x):
        if d % 8 == 0 or not QS:
            q = qt_v[pl.ds(_mo(h * DH + d // 8 * 8, 8), 8), pl.ds(b * TQ, TQ)]
        else:
            q = qw[u, b, pl.ds(d // 8 * 8, 8), :]
        idx = after(jnp.full((8, 128), d % 8, i32))
        for n in range(NQ):
            qb[u, b, d, :, pl.ds(n * 128, 128)] = _take(q[:, n * 128:(n + 1) * 128], idx, axis=0)
        if d % 8 == 0:
            qw[u, b, pl.ds(d, 8), :] = q

    z_v[...] = jnp.zeros((8, 128), f32)
    def stage_keys(heads, results):
        marks = iter(spread(results, len(heads) * (NC + DH)))
        for u in heads:
            for c in range(NC):
                stage_mxu_keys(u, u, c, NC, functools.partial(tie, src=next(marks)))
            for d in range(DH):
                stage_vpu_keys(u, u, d, DH, functools.partial(tie, src=next(marks)))

    with jax.named_scope("wait0"):
        cp_x[0].wait()
        ln1(0, XA, plain=True)
        cp_k.wait()
    with jax.named_scope("phase1"):
        on = ONLY in (0, 1, 4)
        if on:
            made = proj_k(0, XA, plain=True)
            split_weights([(wqkv_v, D, D, wqk7[1])], made[:-1])
            if SR == 1:
                split_rows(XA, ())
        cp_q.wait()
        cp_x[1].wait()
        if on:
            made = proj_q(0, XA, plain=True)
            ln1(XA, 2 * XA, results=made[:1] if LT & 1 else ())
            if SR == 2:
                split_rows(XA, made[1:])
            made = proj_k(XA, 2 * XA)
            wtq_v[...] = wqkv_v[:, pl.ds(0, D)].T
            split_weights([(wtq_v, 0, D, wq7)], made[3:-4], order=(0, 2, 1, 3))
            if SR == 0:
                split_rows(XA, made[:-4])
        cp_v.wait()
        cp_x[2].wait()
        if on:
            wt_v[...] = wqkv_v[:, pl.ds(2 * D, D)].T
            made = proj_q(XA, 2 * XA)
            split_weights([(wt_v, 0, D, wv7)], made[3:-3], order=(0, 2, 1, 3))
            if SR == 3:
                split_rows(XA, made[:-4])
            if PORD == 0:
                made += proj_v(0, XA)
                ln1(2 * XA, S, results=made[:-7] if LT & 2 else ())
                proj_k(2 * XA, S)
            else:
                ln1(2 * XA, S, results=made[:7] if LT & 2 else ())
                proj_k(2 * XA, S)
                made = proj_v(0, XA)
                stage_keys(range(1), made[:-3])
        cp_w[0].wait()
        cp_w[1].wait()
        qs = proj_q(2 * XA, S) if on else []
        vs = proj_v(XA, VB4) if on else []
        stage_keys(range(KQ), qs + vs[:-KE])
        split_weights([(wo_v, 0, D, wo7), (w1_v, 0, F, w17)], qs + vs[:-KE])
        for c in cp_w[2:]:
            c.wait()
        vs = proj_v(VB4, S)[:-KE] if on else []
        stage_keys(range(KQ, HU - 1), vs)
        marks = iter(spread(vs, HU * NB * DH))
        for u in range(HU):
            for b in range(NB):
                for d in range(DH):
                    stage_query(u, u, b, d, functools.partial(tie, src=next(marks)))
        split_weights([(w2_v, 0, D, w27)], vs)
        for u in range(HU - 1 if SCH == 0 else 1):
            stage_values(u, u)

    def query_weights(*blocks):
        w = [qw[u, b] for u, b in blocks]
        return jnp.concatenate(w + [jnp.zeros((128 - DH * len(w), TQ), f32)], axis=0)

    def finish_step(it, acc, v):
        h = it * HU + HU - 1
        acc = acc + _mm(pltpu.bitcast(v, bf16), pc_v[...])
        ot_v[pl.ds(_mo(h * DH, DH), DH), pl.ds((NB - 1) * TQ, TQ)] = acc

    def fast_step(it, carry):
        items = [(u, b, c) for u in range(HU) for b in range(NB) for c in range(NC)]
        tiles = [(u, b, c, t) for u, b, c in items for t in range(NT[c])]
        first = [n // NC * T0[NC] + T0[c] for n, (u, b, c) in enumerate(items)] + [len(tiles)]
        outs = [(n, q, r) for n, (u, b, c) in enumerate(items) for r in reversed(range(NV[c] // 8)) for q in range(NQ)]
        ties = {}
        for o, key in enumerate(outs):
            ties.setdefault(max((o * len(tiles)) // len(outs) + TSH, OFF), []).append(key)
        tiles += tiles[:OFF]
        head = lambda u: it * HU + u
        later = lambda u: jnp.minimum(it + 1, H // HU - 1) * HU + u
        always = z_v[...] >= 0.0
        sv, st = {}, {}

        def vpu_scores(n, q, r):
            if (n, q, r) not in sv:
                u, b, c = items[n]
                acc = None
                for d in range(DH):
                    t = kb[u][d, pl.ds(V0[c] + r * 8, 8), :] * qb[u, b, d, :, pl.ds(q * 128, 128)]
                    acc = t if acc is None else acc + t
                sv[n, q, r] = jnp.exp2(acc) if VEXP else acc
            return sv[n, q, r]

        def key_tile(g, moved=False):
            u, b, c, t = tiles[g]
            if moved:
                kt = kx[u][pl.ds((OFF - 1 - t) * 8, 8), :]
            else:
                kt = km[u][pl.ds((T0[c + 1] - 1 - t) * 8, 8), :]
            for key in ties.get(g, ()):
                kt = jnp.where(always, kt, pltpu.bitcast(vpu_scores(*key), u32))
            return kt

        def mxu_scores(g0, g1):
            if tiles[g0][:2] != tiles[g1 - 1][:2]:
                lhs = [jnp.where(lane < DH, key_tile(g), 0) for g in range(g0, g1 - OFF)]
                lhs += [key_tile(g, True) for g in range(g1 - OFF, g1)]
                w = query_weights(tiles[g0][:2], tiles[g1 - 1][:2])
            else:
                lhs = [key_tile(g) for g in range(g0, g1)]
                w = query_weights(tiles[g0][:2])
            s = _mm(pltpu.bitcast(jnp.concatenate(lhs, axis=0), bf16), w)
            for g in range(g0, g1):
                st[g] = s[(g - g0) * 16:(g - g0 + 1) * 16]

        def weights(n, l):
            c = items[n][2]
            rows = [st.pop(first[n + 1] - 1 - t) for t in range(NT[c])]
            more = [jnp.concatenate([vpu_scores(n, q, r) for q in range(NQ)], axis=1) for r in range(NV[c] // 8)]
            if VEXP:
                rows = [jnp.exp2(jnp.concatenate(rows, axis=0))]
                p = jnp.concatenate(more + rows if VPOS else rows + more, axis=0)
            else:
                p = jnp.exp2(jnp.concatenate(rows + more, axis=0))
            for r in reversed(range(CK // 8)):
                row = p[r * 8:(r + 1) * 8]
                l = row if l is None else l + row
            return p, l

        for g in range(OFF):
            st[g] = p0_v[pl.ds(g * 16, 16), :]
        l = acc = None
        for m in range(len(items) + 1):
            if m < len(items):
                mxu_scores(first[m] + OFF, first[m + 1] + OFF)
            if m == 0:
                finish_step(jnp.maximum(it - 1, 0), *carry)
                continue
            u, b, c = items[m - 1]
            if c == 0:
                l, acc = None, jnp.tile(z_v[...], (DH // 8, NQ))
            p, l = weights(m - 1, l)
            v = vw[u][0, :, pl.ds(c * CK, CK)]
            if m < len(items):
                acc = acc + _mm(pltpu.bitcast(v, bf16), p)
            else:
                late = jnp.tile(p[MOFF[c]:MOFF[c] + 8], (NV[c] // 8, 1))
                keep = jnp.tile(z_v[...], (NV[c] // 8, NQ)) >= 0.0
                pc_v[pl.ds(MOFF[c], CK - NV[c]), :] = p[MOFF[c]:MOFF[c] + CK - NV[c]]
                pc_v[pl.ds(VOFF[c], NV[c]), :] = jnp.where(keep, p[VOFF[c]:VOFF[c] + NV[c]], late)

            def after(x, src=l[:, 0:128]):
                return jnp.where(always, x, pltpu.bitcast(src, i32))

            def after2(x, src=p[MID * 8:MID * 8 + 8, 0:128]):
                return jnp.where(always, x, pltpu.bitcast(src, i32))
            if SCH == 0:
                h_fill, slot = (later(u - 1) if u > 0 else head(HU - 1)), (u - 1) % HU
                zero = jnp.minimum(it, 0) if u == 0 and DYN else 0
            else:
                h_fill, slot = (head(u + 1) if u < HU - 1 else later(0)), (u + 1) % HU
                zero = jnp.minimum(it, 0) if u < HU - 1 or DYN == 2 else 0
            span, n = (LSPAN, b * NC + c - LOFF) if u == HU - 1 else (KSPAN, b * NC + c)
            for part in range(KP):
                if part * span // KP == n:
                    stage_vpu_keys(h_fill, slot, part, KP, after, zero)
            for part in range(MP):
                if part * span // MP == n:
                    stage_mxu_keys(h_fill, slot, part, MP, after2, zero)
            if n == 0:
                stage_values(h_fill, slot, zero)
            blk = u * NB + b
            if blk > 0:
                stage_query(later((blk - 1) // NB), (blk - 1) // NB, (blk - 1) % NB, c, after)
            if c == NC - 1:
                l_v[head(u), :, pl.ds(b * TQ, TQ)] = l
                if m < len(items):
                    ot_v[pl.ds(_mo(head(u) * DH, DH), DH), pl.ds(b * TQ, TQ)] = acc
        for g in range(OFF):
            p0_v[pl.ds(g * 16, 16), :] = st.pop(first[-1] + g)
        for d in range(DH):
            stage_query(later(HU - 1), HU - 1, NB - 1, d, after2)
        return acc, v

    one = jnp.ones((8, 128), f32)
    with jax.named_scope("phase2"):
        big = jnp.maximum(*peaks)
        if ONLY in (0, 2):
            lead = pltpu.bitcast(jnp.concatenate(
                [k_p[0, pl.ds(MOFF[0] // 2 + (NT[0] - 1 - t) * 8, 8), :] for t in range(OFF)], axis=0), bf16)
            p0_v[...] = _mm(lead, query_weights((0, 0)))
            pc_v[...] = jnp.zeros((CK, TQ), f32)
            carry = (jnp.zeros((DH, TQ), f32), jnp.zeros((DH // 2, CK), u32))
            carry = jax.lax.fori_loop(0, H // HU, fast_step, carry)
            finish_step(H // HU - 1, *carry)
        else:
            def dummy(i, c):
                z_v[...] = jnp.abs(z_v[...])
                l_v[i] = l_v[i] + 1.0
                if ONLY == 4:
                    for ref in (wo7, w17, w27, *kb, qb, qw, *vw, ko_v, k_p):
                        idx = (i % ref.shape[0],) + (0,) * (len(ref.shape) - 3) + (slice(0, 8), slice(0, 128))
                        z_v[...] = z_v[...] + ref[idx].astype(f32)
                    z_v[...] = z_v[...] + vt_p[pl.ds(_mo(i * 8, 8), 8), 0:128].astype(f32) + qt_v[pl.ds(_mo(i * 8, 8), 8), 0:128]
                return c
            jax.lax.fori_loop(0, 2, dummy, 0)
    if True:
        los, his = [one] * 4, [one] * 4
        for h in range(H):
            for n in range(S // 128):
                part = l_v[h, :, pl.ds(n * 128, 128)]
                los[n % 4] = jnp.minimum(los[n % 4], part)
                his[n % 4] = jnp.maximum(his[n % 4], part)
        lo = functools.reduce(jnp.minimum, los)
        hi = functools.reduce(jnp.maximum, his)
    safe = (lo >= L_MIN) & (hi <= L_MAX) & (big <= A_MAX)

    @pl.when(jnp.max(jnp.where(safe, float(FORCE_SAFE), 1.0)) > 0.0)
    def _():
        def safe_step(i, carry):
            h, b = i // (S // TS), i % (S // TS)
            cols = pl.ds(_mo(b * TS, TS), TS)
            q = qt_v[pl.ds(_mo(h * DH, DH), DH), cols]
            row_head = jax.lax.broadcasted_iota(i32, (128, TS), 0) // DH
            qm = jnp.where(row_head == h % 8, jnp.tile(q, (8, 1)), 0.0)
            s = _mm(pltpu.bitcast(k_p[h // 8], bf16), qm)
            p = jnp.exp2(s - jnp.max(s, axis=0, keepdims=True))
            v = pltpu.bitcast(vt_p[pl.ds(_mo(h * (DH // 2), DH // 2), DH // 2), :], bf16)
            ot_v[pl.ds(_mo(h * DH, DH), DH), cols] = _mm(v, p)
            l_v[h, :, cols] = jnp.sum(p.reshape(S // 8, 8, TS), axis=0)
            return carry
        jax.lax.fori_loop(0, H * (S // TS), safe_step, 0)

    b1 = b1_ref[...].astype(f32).reshape(1, F)
    b2 = b2_ref[...].astype(f32).reshape(1, D)
    RH, FH = R3 // 2, F // 2

    def out_copy(i):
        rows = pl.ds(i * R3, R3)
        return pltpu.make_async_copy(out_v.at[rows], out_hbm.at[rows], out_sem.at[i])

    def quadrants(i):
        return [(pl.ds(i * R3 + r * RH, RH), pl.ds(c * DQ, DQ)) for r in range(2) for c in range(2)]

    def normalize(i, srcs=(None,)):
        rows = pl.ds(i * R3, R3)
        ot = []
        for h in range(H):
            lsum = jnp.sum(tie(l_v[h, :, rows], srcs[h * len(srcs) // H]), axis=0, keepdims=True)
            inv = pl.reciprocal(lsum, approx=True)
            ot.append(ot_v[pl.ds(h * DH, DH), rows] * (inv * (2.0 - lsum * inv)))
        o = jnp.concatenate(ot, axis=0).T
        if WO7:
            for j, op in enumerate(_lhs7(o[:RH, :DQ], o[:RH, DQ:], o[RH:, :DQ], o[RH:, DQ:])):
                o7[i % 4, j] = op
        else:
            for j, op in enumerate((o[:RH, :DQ], o[:RH, DQ:], o[RH:, :DQ], o[RH:, DQ:])):
                o7[i % 4, j] = op

    def out_proj(i):
        if WO7:
            ys = _join7([_mm(o7[i % 4, j], pltpu.bitcast(wo7[j], bf16)) for j in range(7)])
        else:
            o = jnp.concatenate([jnp.concatenate([o7[i % 4, 2 * r], o7[i % 4, 2 * r + 1]], axis=1) for r in range(2)], axis=0)
            y = _mm(o, wo_v[...])
            ys = (y[:RH, :DQ], y[:RH, DQ:], y[RH:, :DQ], y[RH:, DQ:])
        for q, y in zip(quadrants(i), ys):
            h_v[q] = x_v[q].astype(f32) + y

    def ln2(i, srcs=(None,)):
        step = RH // len(srcs)
        for n, src in enumerate(srcs):
            halves = []
            for r in range(2):
                hid = h_v[pl.ds(i * R3 + r * RH + n * step, step), :]
                hid = jnp.concatenate([tie(hid[:, 0:128], src), hid[:, 128:]], axis=1)
                halves.append(_ln(hid))
            top, bot = halves
            for j, op in enumerate(_lhs7(top[:, :DQ], top[:, DQ:], bot[:, :DQ], bot[:, DQ:])):
                hn7[i % 4, j, pl.ds(n * step, step), :] = op

    def ffn_up(i, f0):
        w = min(FC, FH - f0)
        ms = {j: _mm(hn7[i % 4, j], pltpu.bitcast(w17[j, :, pl.ds(f0, w)], bf16)) for j in ORD}
        bias = [b1[:, f0:f0 + w], b1[:, FH + f0:FH + f0 + w]] * 2
        act = [_gelu(a + bb) for a, bb in zip(_join7(ms), bias)]
        for j, op in enumerate(_lhs7(*act)):
            g7[i % 2, j, :, pl.ds(f0, w)] = _pack(op)

    def ffn_down(i, j):
        return _mm(g7[i % 2, j], pltpu.bitcast(w27[j], bf16))

    def finish(i, ms):
        for q, y, bb in zip(quadrants(i), _join7(ms), [b2[:, :DQ], b2[:, DQ:]] * 2):
            out_v[q] = (h_v[q] + y + bb).astype(out_v.dtype)
        out_copy(i).start()

    with jax.named_scope("phase3"):
        if ONLY in (0, 3):
            normalize(0)
            out_proj(0)
            normalize(1)
            out_proj(1)
            ln2(0)
            for i in range(n3):
                for f0 in range(0, FH, FC):
                    ffn_up(i, f0)
                if 0 < i < n3 - 1:
                    out_proj(i + 1)
                ms = [ffn_down(i, j) for j in range(7)]
                if i + 1 < n3:
                    ln2(i + 1, [None, ms[0], ms[1], ms[2]] if MIX & 1 else [ms[0], ms[1], ms[2], ms[3]])
                if i + 2 < n3:
                    normalize(i + 2, [ms[3], ms[4], ms[5], ms[6]] if MIX & 2 else [ms[2], ms[3], ms[4], ms[5]])
                finish(i, ms)
        else:
            for i in range(n3):
                out_copy(i).start()
    with jax.named_scope("tail"):
        for i in range(n3):
            out_copy(i).wait()


@jax.jit
def pallas_sequential_preLN__softmax_full_mha__dense_activation_gelu__prompt_kernel(
        A_x, A_wqkv, A_wo, B_x, B_w1, B_b1, B_w2, B_b2):
    del B_x
    any_spec = pl.BlockSpec(memory_space=pl.ANY)
    vmem_spec = pl.BlockSpec(memory_space=pltpu.VMEM)
    vm = pltpu.VMEM
    out = pl.pallas_call(
        _kernel,
        out_shape=jax.ShapeDtypeStruct((S, D), A_x.dtype),
        in_specs=[any_spec] * 7,
        out_specs=any_spec,
        scratch_shapes=[
            vm((S, D), bf16), vm((D, 3 * D), bf16), vm((D, D), bf16), vm((D, F), bf16), vm((F, D), bf16),
            *[vm((7, D // 4, D // 2), u32)] * 3, vm((D, D), bf16), vm((D, D), bf16), vm((512, D), f32),
            vm((S // R1, 7, R1 // 2, D // 2), f32),
            vm((D // 128, S // 2, 128), u32), vm((D // 128, V0[NC], 128), f32),
            vm((D, S), f32), vm((D // 2, S), u32), vm((D, S), f32), vm((H, 8, S), f32),
            vm((HU, V0[NC], 128), f32), vm((HU, NB, DH, TQ), f32), vm((HU, NB, DH, 8, TQ), f32), vm((OFF * 16, TQ), f32), vm((CK, TQ), f32),
            vm((8, 128), f32),
            vm((7, D // 4, D // 2), u32), vm((7, D // 4, F // 2), u32), vm((7, F // 4, D // 2), u32),
            vm((4, 7, R3 // 2, D // 2), f32), vm((4, 7, R3 // 2, D // 2), f32), vm((2, 7, R3 // 2, F // 2), f32),
            vm((S, D), f32), vm((S, D), bf16),
            pltpu.SemaphoreType.DMA((11,)), pltpu.SemaphoreType.DMA((S // R3,)),
            *[vm((T0[NC] * 8, 128), u32)] * HU, *[vm((OFF * 8, 128), u32)] * HU,
            *[vm((DH, V0[NC], 128), f32)] * HU, *[vm((1, DH // 2, S), u32)] * HU,
            vm((F,), bf16), vm((D,), bf16),
        ],
        compiler_params=pltpu.CompilerParams(vmem_limit_bytes=100 * 1024 * 1024),
    )(A_x.reshape(S, D), A_wqkv, A_wo, B_w1, B_b1, B_w2, B_b2)
    return out.reshape(A_x.shape)
```

```python
import functools
import jax
import jax.numpy as jnp
import numpy as np
import jax.experimental.pallas as pl
import jax.experimental.pallas.tpu as pltpu

S, D, F, H, DH = 2048, 512, 1792, 32, 16
TQ = 512
NQ = TQ // 128
NB = S // TQ
CK = 128
NC = S // CK
PAT = [16,16,16,16,16,16,16,32]
NV = [PAT[c % len(PAT)] for c in range(NC)]
KF = 0
TR = 8 if KF else 16
NT = [(CK - v) // TR for v in NV]
V0 = [sum(NV[:c]) for c in range(NC + 1)]
T0 = [sum(NT[:c]) for c in range(NC + 1)]
HU = 4
OFF = 2
TSH = 9
KSP = 2
R1 = 256
R3 = 128
U1 = 1
FC = 256
ONLY = 0
FORCE_SAFE = 0
DMAP = 0
RCP = 1
MIX = 0
ORD = [range(7), (1, 3, 2, 4, 0, 5, 6), (0, 1, 3, 2, 4, 5, 6), (4, 2, 3, 1, 0, 6, 5)][0]
WO7 = 1
PR = 16
XF = 1
WP = 0
TORD = 0
NTM = 2
VB = 1
KQ = 2
KP = 16
MP = 16
KSPAN = 16
MID = 7
QA = 0
DYN = 1
ALIVE = 0
CHK = 2
LSPAN = 16
LOFF = 44
DBG = 0
VEXP = 1
VPOS = 1
MOFF = [v if VPOS else 0 for v in NV]
VOFF = [0 if VPOS else CK - v for v in NV]
FEN = 0
SCH = 0
FC2 = 1
KS = 0
QS = 0
LP = 16
LT = 3
PORD = 0
SR = 1
VB4 = 1024
KE = 5
OORD = 1
TREE = 1
KA = 0
MA = 1
MSH = 0
LNE = 3
LNP = 8
NS = 3
NE = 7
NP = 32
TS = 128
EPS = 1e-5
L_MIN, L_MAX, A_MAX = 2.0 ** -40, 2.0 ** 40, 2.0 ** 80
bf16, f32, u32, i32 = jnp.bfloat16, jnp.float32, jnp.uint32, jnp.int32
Q_SCALE = float(DH ** -0.5 * np.log2(np.e))


def _mo(x, n):
    return x if isinstance(x, int) else pl.multiple_of(x, n)


def _mm(a, b):
    return jax.lax.dot_general(a, b, (((1,), (0,)), ((), ())), preferred_element_type=f32)


def _mm_nt(a, b):
    return jax.lax.dot_general(a, b, (((1,), (1,)), ((), ())), preferred_element_type=f32)


def _take(x, idx, axis):
    return jnp.take_along_axis(x, idx, axis=axis, mode="promise_in_bounds", wrap_negative_indices=False)


def _pack(x):
    return x


def _keys(x):
    return x if KF else pltpu.bitcast(x, bf16)


def _lhs7(a11, a12, a21, a22):
    return (a11 + a22, a21 + a22, a11, a22, a11 + a12, a21 - a11, a12 - a22)


def _rhs7(b11, b12, b21, b22):
    return (b11 + b22, b11, b12 - b22, b21 - b11, b22, b11 + b12, b21 + b22)


def _join7(m):
    return (m[0] + m[3] - m[4] + m[6], m[2] + m[4], m[1] + m[3], m[0] - m[1] + m[2] + m[5])


def _ln(x):
    m = jnp.mean(x, axis=-1, keepdims=True)
    xc = x - m
    v = jnp.mean(xc * xc, axis=-1, keepdims=True)
    return xc * jax.lax.rsqrt(v + EPS)


def _gelu(x):
    c = float(np.sqrt(2.0 / np.pi))
    return (0.5 * x) * (1.0 + jnp.tanh(x * (c + (c * 0.044715) * (x * x))))


def _kernel(x_hbm, wqkv_hbm, wo_hbm, w1_hbm, b1_hbm, w2_hbm, b2_hbm, out_hbm,
            x_v, wqkv_v, wo_v, w1_v, w2_v, wq7, wk7, wv7, wt_v, wtq_v, xn_v, xn7, k_p, ko_v, qt_v, vt_p, ot_v, l_v,
            ks_v, qw, qb, p0_v, pc_v, z_v, wo7, w17, w27, o7, hn7, g7, h_v, out_v, in_sem, out_sem, *slots):
    km, kx, kb, vw = (slots[i * HU:(i + 1) * HU] for i in range(4))
    b1_ref, b2_ref = slots[4 * HU:]
    n3 = S // R3
    wqk7 = (wq7, wk7)

    XA = 512

    def part(src, dst, rows, cols, i):
        return pltpu.make_async_copy(src.at[rows, cols], dst.at[rows, cols], in_sem.at[i])
    every = slice(None)
    cp_x = [part(x_hbm, x_v, pl.ds(r0, n), every, i) for i, (r0, n) in enumerate(((0, XA), (XA, XA), (2 * XA, S - 2 * XA)))]
    cp_q, cp_k, cp_v = [part(wqkv_hbm, wqkv_v, every, pl.ds(i * D, D), 3 + i) for i in range(3)]
    cp_w = [part(src, dst, every, every, 6 + i) for i, (src, dst) in enumerate(((wo_hbm, wo_v), (w1_hbm, w1_v), (w2_hbm, w2_v)))]
    cp_w += [pltpu.make_async_copy(src, dst, in_sem.at[9 + i]) for i, (src, dst) in enumerate(((b1_hbm, b1_ref), (b2_hbm, b2_ref)))]
    for c in (cp_x[0], cp_k, cp_q, cp_x[1], cp_v, cp_x[2], *cp_w):
        c.start()

    DQ, H1 = D // 2, R1 // 2

    def tie(x, src):
        if src is None:
            return x
        reps = (x.shape[0] // 8, x.shape[1] // 128)
        src = src[0:8, 0:128]
        src = src if x.dtype == src.dtype else pltpu.bitcast(src, x.dtype)
        return jnp.where(jnp.tile(z_v[...], reps) >= 0.0, x, jnp.tile(src, reps))

    def spread(results, n):
        if not results:
            return [None] * n
        tiles = [(y, r, c) for y in results for c in range(0, y.shape[1], 128) for r in range(0, y.shape[0], 8)]
        picks = [tiles[i * len(tiles) // n] for i in range(n)]
        return [y[r:r + 8, c:c + 128] for y, r, c in picks]

    def ln1(r0, r1, plain=False, results=()):
        pieces = [(i, r) for i in range(r0 // R1, r1 // R1) for r in range(0, H1, LP)]
        for (i, r), src in zip(pieces, spread(results, len(pieces))):
            halves = []
            for half in range(2):
                rows = pl.ds(i * R1 + half * H1 + r, LP)
                x = x_v[rows, :].astype(f32)
                halves.append(_ln(jnp.concatenate([tie(x[:, 0:128], src), x[:, 128:]], axis=1)))
                if plain:
                    xn_v[rows, :] = halves[-1]
            if plain:
                continue
            top, bot = halves
            for j, op in enumerate(_lhs7(top[:, :DQ], top[:, DQ:], bot[:, :DQ], bot[:, DQ:])):
                xn7[i, j, pl.ds(r, LP), :] = op

    def split_rows(r1, results):
        pieces = [(i, r) for i in range(r1 // R1) for r in range(0, H1, LP)]
        for (i, r), src in zip(pieces, spread(results, len(pieces))):
            top, bot = (tie(xn_v[pl.ds(i * R1 + half * H1 + r, LP), :], src) for half in range(2))
            for j, op in enumerate(_lhs7(top[:, :DQ], top[:, DQ:], bot[:, :DQ], bot[:, DQ:])):
                xn7[i, j, pl.ds(r, LP), :] = op

    def split_weights(jobs, results, order=(0, 1, 2, 3)):
        pieces = [(src, c0, n, dst, r, c) for src, c0, n, dst in jobs
                  for r in range(0, src.shape[0] // 2, 16) for c in range(0, n // 2, 128)]
        for (src, c0, n, dst, r, c), wait_for in zip(pieces, spread(results, len(pieces))):
            quad = []
            for i in range(2):
                for j in range(2):
                    w = pltpu.bitcast(src[pl.ds(r + i * src.shape[0] // 2, 16), pl.ds(c0 + j * n // 2 + c, 128)], u32)
                    quad.append(pltpu.bitcast(tie(w, wait_for), bf16).astype(f32))
            for i, op in enumerate(_rhs7(*[quad[o] for o in order])):
                dst[i, pl.ds(r // 2, 8), pl.ds(c, 128)] = pltpu.bitcast(op.astype(bf16), u32)

    def project(which, i, plain):
        if plain:
            y = _mm(xn_v[pl.ds(i * R1, R1), :], wqkv_v[:, pl.ds(which * D, D)])
            return y, [y]
        ms = [_mm(xn7[i, j], pltpu.bitcast(wqk7[which][j], bf16)) for j in range(7)]
        c11, c12, c21, c22 = _join7(ms)
        return jnp.concatenate([jnp.concatenate([c11, c12], axis=1), jnp.concatenate([c21, c22], axis=1)], axis=0), ms

    def project_t(w7, i):
        ms = [_mm_nt(pltpu.bitcast(w7[j], bf16), xn7[i, j]) for j in range(7)]
        c11, c12, c21, c22 = _join7(ms)
        return jnp.concatenate([jnp.concatenate([c11, c21], axis=1), jnp.concatenate([c12, c22], axis=1)], axis=0), ms

    def proj_q(r0, r1, plain=False):
        made = []
        for i in range(r0 // R1, r1 // R1):
            if plain:
                q, ms = project(0, i, plain)
                qt = q.T
            else:
                qt, ms = project_t(wq7, i)
            qt_v[:, pl.ds(i * R1, R1)] = qt * Q_SCALE
            made += ms
        return made

    def proj_k(r0, r1, plain=False):
        made = []
        for i in range(r0 // R1, r1 // R1):
            k, ms = project(1, i, plain)
            kp = k if KF else pltpu.bitcast(k.astype(bf16), u32)
            for g in range(D // 128):
                lanes = slice(g * 128, (g + 1) * 128)
                k_p[g, pl.ds(i * R1 * 8 // TR, R1 * 8 // TR), :] = kp[:, lanes]
                for c in range(i * R1 // CK, (i + 1) * R1 // CK):
                    r = c * CK + VOFF[c] - i * R1
                    ko_v[g, pl.ds(V0[c], NV[c]), :] = k[r:r + NV[c], lanes]
            made += ms
        return made

    peaks = [jnp.zeros((8, 128), f32)] * 2

    def proj_v(r0, r1):
        made = []
        for i in range(r0 // R1, r1 // R1):
            vt, ms = project_t(wv7, i)
            vt_p[:, pl.ds(i * R1, R1)] = pltpu.bitcast(vt.astype(bf16), u32)
            for n in range(R1 // 128):
                for r in range(0, D, 8):
                    peaks[n % 2] = jnp.maximum(peaks[n % 2], jnp.abs(vt[r:r + 8, n * 128:(n + 1) * 128]))
            made += ms
        return made

    lane = jax.lax.broadcasted_iota(i32, (8, 128), 1)

    key_tiles = [(c, t) for c in range(NC) for t in range(NT[c])]

    def stage_mxu_keys(h, u, part, parts, after=lambda x: x, zero=0):
        mine = range(part * len(key_tiles) // parts, (part + 1) * len(key_tiles) // parts)
        idx = after((lane + (h % 8) * DH) & 127)
        for g in mine:
            c, t = key_tiles[g]
            kp = k_p[h // 8, pl.ds((c * CK + MOFF[c]) * 8 // TR + t * 8, 8), :]
            km[u][pl.ds(_mo((g + zero) * 8, 8), 8), :] = _take(kp, idx, axis=1)
            if c == 0 and t >= NT[0] - OFF:
                moved = _take(kp, (idx + (128 - DH)) & 127, axis=1)
                kx[u][pl.ds(_mo((t - NT[0] + OFF + zero) * 8, 8), 8), :] = jnp.where((lane >= DH) & (lane < 2 * DH), moved, jnp.zeros_like(moved))

    def stage_values(h, u, zero=0):
        vw[u][zero] = vt_p[pl.ds(_mo(h * (DH // 2), DH // 2), DH // 2), :]

    def stage_vpu_keys(h, u, part, parts, after=lambda x: x, zero=0):
        d, sub = divmod(part, parts // DH)
        n = V0[NC] // 8
        r0, r1 = sub * n // (parts // DH), (sub + 1) * n // (parts // DH)
        idx = after(jnp.full((8, 128), (h % 8) * DH + d, i32))
        rows = pl.ds(r0 * 8, (r1 - r0) * 8)
        if KS:
            if d == 0:
                ks_v[u, rows, :] = ko_v[h // 8, rows, :]
            src = ks_v[u, rows, :]
        else:
            src = ko_v[h // 8, rows, :]
        kb[u][d + zero, rows, :] = _take(src, jnp.tile(idx, (r1 - r0, 1)), axis=1)

    def stage_query(h, u, b, d, after=lambda x: x):
        if d % 8 == 0 or not QS:
            q = qt_v[pl.ds(_mo(h * DH + d // 8 * 8, 8), 8), pl.ds(b * TQ, TQ)]
        else:
            q = qw[u, b, pl.ds(d // 8 * 8, 8), :]
        idx = after(jnp.full((8, 128), d % 8, i32))
        for n in range(NQ):
            qb[u, b, d, :, pl.ds(n * 128, 128)] = _take(q[:, n * 128:(n + 1) * 128], idx, axis=0)
        if d % 8 == 0:
            qw[u, b, pl.ds(d, 8), :] = q

    z_v[...] = jnp.zeros((8, 128), f32)
    def stage_keys(heads, results):
        marks = iter(spread(results, len(heads) * (NC + DH)))
        for u in heads:
            for c in range(NC):
                stage_mxu_keys(u, u, c, NC, functools.partial(tie, src=next(marks)))
            for d in range(DH):
                stage_vpu_keys(u, u, d, DH, functools.partial(tie, src=next(marks)))

    with jax.named_scope("wait0"):
        cp_x[0].wait()
        ln1(0, XA, plain=True)
        cp_k.wait()
    with jax.named_scope("phase1"):
        on = ONLY in (0, 1, 4)
        if on:
            made = proj_k(0, XA, plain=True)
            split_weights([(wqkv_v, D, D, wqk7[1])], made[:-1])
            if SR == 1:
                split_rows(XA, ())
        cp_q.wait()
        cp_x[1].wait()
        if on:
            made = proj_q(0, XA, plain=True)
            ln1(XA, 2 * XA, results=made[:1] if LT & 1 else ())
            if SR == 2:
                split_rows(XA, made[1:])
            made = proj_k(XA, 2 * XA)
            wtq_v[...] = wqkv_v[:, pl.ds(0, D)].T
            split_weights([(wtq_v, 0, D, wq7)], made[3:-4], order=(0, 2, 1, 3))
            if SR == 0:
                split_rows(XA, made[:-4])
        cp_v.wait()
        cp_x[2].wait()
        if on:
            wt_v[...] = wqkv_v[:, pl.ds(2 * D, D)].T
            made = proj_q(XA, 2 * XA)
            split_weights([(wt_v, 0, D, wv7)], made[3:-3], order=(0, 2, 1, 3))
            if SR == 3:
                split_rows(XA, made[:-4])
            if PORD == 0:
                made += proj_v(0, XA)
                ln1(2 * XA, S, results=made[:-7] if LT & 2 else ())
                proj_k(2 * XA, S)
            else:
                ln1(2 * XA, S, results=made[:7] if LT & 2 else ())
                proj_k(2 * XA, S)
                made = proj_v(0, XA)
                stage_keys(range(1), made[:-3])
        cp_w[0].wait()
        cp_w[1].wait()
        qs = proj_q(2 * XA, S) if on else []
        vs = proj_v(XA, VB4) if on else []
        stage_keys(range(KQ), qs + vs[:-KE])
        split_weights([(wo_v, 0, D, wo7), (w1_v, 0, F, w17)], qs + vs[:-KE])
        for c in cp_w[2:]:
            c.wait()
        vs = proj_v(VB4, S)[:-KE] if on else []
        stage_keys(range(KQ, HU - 1), vs)
        marks = iter(spread(vs, HU * NB * DH))
        for u in range(HU):
            for b in range(NB):
                for d in range(DH):
                    stage_query(u, u, b, d, functools.partial(tie, src=next(marks)))
        split_weights([(w2_v, 0, D, w27)], vs)
        for u in range(HU - 1 if SCH == 0 else 1):
            stage_values(u, u)

    def query_weights(*blocks):
        w = [qw[u, b] for u, b in blocks]
        return jnp.concatenate(w + [jnp.zeros((128 - DH * len(w), TQ), f32)], axis=0)

    def finish_step(acc, v):
        return acc + _mm(pltpu.bitcast(v, bf16), pc_v[...])

    def store_block(it, acc):
        ot_v[pl.ds(_mo((it * HU + HU - 1) * DH, DH), DH), pl.ds((NB - 1) * TQ, TQ)] = acc

    def fast_step(it, carry):
        items = [(u, b, c) for u in range(HU) for b in range(NB) for c in range(NC)]
        tiles = [(u, b, c, t) for u, b, c in items for t in range(NT[c])]
        first = [n // NC * T0[NC] + T0[c] for n, (u, b, c) in enumerate(items)] + [len(tiles)]
        outs = [(n, q, r) for n, (u, b, c) in enumerate(items) for r in reversed(range(NV[c] // 8)) for q in range(NQ)]
        if OORD == 1:
            outs = [(n, q, r) for n, (u, b, c) in enumerate(items) for q in range(NQ) for r in reversed(range(NV[c] // 8))]
        if OORD == 2:
            outs = [(n, q, r0 + r) for n, (u, b, c) in enumerate(items) for r0 in reversed(range(0, NV[c] // 8, 2))
                    for q in range(NQ) for r in (1, 0)]
        ties = {}
        for o, key in enumerate(outs):
            ties.setdefault(max((o * len(tiles)) // len(outs) + TSH, OFF), []).append(key)
        tiles += tiles[:OFF]
        head = lambda u: it * HU + u
        later = lambda u: jnp.minimum(it + 1, H // HU - 1) * HU + u
        always = z_v[...] >= 0.0
        sv, st = {}, {}

        def vpu_scores(n, q, r):
            if (n, q, r) not in sv:
                u, b, c = items[n]
                accs = [None] * TREE
                for d in range(DH):
                    t = kb[u][d, pl.ds(V0[c] + r * 8, 8), :] * qb[u, b, d, :, pl.ds(q * 128, 128)]
                    accs[d % TREE] = t if accs[d % TREE] is None else accs[d % TREE] + t
                acc = functools.reduce(jnp.add, accs)
                sv[n, q, r] = jnp.exp2(acc) if VEXP else acc
            return sv[n, q, r]

        def key_tile(g, moved=False):
            u, b, c, t = tiles[g]
            if moved:
                kt = kx[u][pl.ds((OFF - 1 - t) * 8, 8), :]
            else:
                kt = km[u][pl.ds((T0[c + 1] - 1 - t) * 8, 8), :]
            for key in ties.get(g, ()):
                kt = jnp.where(always, kt, vpu_scores(*key) if KF else pltpu.bitcast(vpu_scores(*key), u32))
            return kt

        def mxu_scores(g0, g1):
            if tiles[g0][:2] != tiles[g1 - 1][:2]:
                lhs = [jnp.where(lane < DH, key_tile(g), 0.0 if KF else 0) for g in range(g0, g1 - OFF)]
                lhs += [key_tile(g, True) for g in range(g1 - OFF, g1)]
                w = query_weights(tiles[g0][:2], tiles[g1 - 1][:2])
            else:
                lhs = [key_tile(g) for g in range(g0, g1)]
                w = query_weights(tiles[g0][:2])
            s = _mm(_keys(jnp.concatenate(lhs, axis=0)), w)
            for g in range(g0, g1):
                st[g] = s[(g - g0) * TR:(g - g0 + 1) * TR]

        def weights(n, l):
            c = items[n][2]
            rows = [st.pop(first[n + 1] - 1 - t) for t in range(NT[c])]
            more = [jnp.concatenate([vpu_scores(n, q, r) for q in range(NQ)], axis=1) for r in range(NV[c] // 8)]
            if VEXP:
                rows = [jnp.exp2(jnp.concatenate(rows, axis=0))]
                p = jnp.concatenate(more + rows if VPOS else rows + more, axis=0)
            else:
                p = jnp.exp2(jnp.concatenate(rows + more, axis=0))
            for r in reversed(range(CK // 8)):
                row = p[r * 8:(r + 1) * 8]
                l = row if l is None else l + row
            return p, l

        for g in range(OFF):
            st[g] = p0_v[pl.ds(g * TR, TR), :]
        l = acc = None
        for m in range(len(items) + 1):
            if m < len(items):
                mxu_scores(first[m] + OFF, first[m + 1] + OFF)
            if m == 0:
                store_block(jnp.maximum(it - 1, 0), finish_step(*carry[:2]))
                continue
            u, b, c = items[m - 1]
            if c == 0:
                l, acc = None, jnp.tile(z_v[...], (DH // 8, NQ))
            p, l = weights(m - 1, l)
            v = vw[u][0, :, pl.ds(c * CK, CK)]
            if m < len(items):
                acc = acc + _mm(pltpu.bitcast(v, bf16), p)
            else:
                late = jnp.tile(p[MOFF[c]:MOFF[c] + 8], (NV[c] // 8, 1))
                keep = jnp.tile(z_v[...], (NV[c] // 8, NQ)) >= 0.0
                pc_v[pl.ds(MOFF[c], CK - NV[c]), :] = p[MOFF[c]:MOFF[c] + CK - NV[c]]
                pc_v[pl.ds(VOFF[c], NV[c]), :] = jnp.where(keep, p[VOFF[c]:VOFF[c] + NV[c]], late)

            def after(x, src=l[:, 0:128]):
                return jnp.where(always, x, pltpu.bitcast(src, i32))

            def after2(x, src=p[MID * 8:MID * 8 + 8, 0:128]):
                return jnp.where(always, x, pltpu.bitcast(src, i32))
            if SCH == 0:
                h_fill, slot = (later(u - 1) if u > 0 else head(HU - 1)), (u - 1) % HU
                zero = jnp.minimum(it, 0) if u == 0 and DYN else 0
            else:
                h_fill, slot = (head(u + 1) if u < HU - 1 else later(0)), (u + 1) % HU
                zero = jnp.minimum(it, 0) if u < HU - 1 or DYN == 2 else 0
            span, n = (LSPAN, b * NC + c - LOFF) if u == HU - 1 else (KSPAN, b * NC + c)
            for part in range(KP):
                if part * span // KP == n:
                    stage_vpu_keys(h_fill, slot, part, KP, after2 if KA else after, zero)
            for part in range(MP):
                if part * span // MP + MSH == n:
                    stage_mxu_keys(h_fill, slot, part, MP, after2 if MA else after, zero)
            if n == 0:
                stage_values(h_fill, slot, zero)
            blk = u * NB + b
            if blk > 0:
                stage_query(later((blk - 1) // NB), (blk - 1) // NB, (blk - 1) % NB, c, after2 if QA else after)
            if c == NC - 1:
                l_v[head(u), :, pl.ds(b * TQ, TQ)] = l
                if m < len(items):
                    ot_v[pl.ds(_mo(head(u) * DH, DH), DH), pl.ds(b * TQ, TQ)] = acc
        for g in range(OFF):
            p0_v[pl.ds(g * TR, TR), :] = st.pop(first[-1] + g)
        for d in range(DH):
            stage_query(later(HU - 1), HU - 1, NB - 1, d, after2)
        return acc, v

    one = jnp.ones((8, 128), f32)
    with jax.named_scope("phase2"):
        big = jnp.maximum(*peaks)
        if ONLY in (0, 2):
            lead = _keys(jnp.concatenate(
                [k_p[0, pl.ds(MOFF[0] * 8 // TR + (NT[0] - 1 - t) * 8, 8), :] for t in range(OFF)], axis=0))
            p0_v[...] = _mm(lead, query_weights((0, 0)))
            pc_v[...] = jnp.zeros((CK, TQ), f32)
            carry = (jnp.zeros((DH, TQ), f32), jnp.zeros((DH // 2, CK), u32))
            carry = jax.lax.fori_loop(0, H // HU, fast_step, carry)
        else:
            def dummy(i, c):
                z_v[...] = jnp.abs(z_v[...])
                l_v[i] = l_v[i] + 1.0
                if ONLY == 4:
                    for ref in (wo7, w17, w27, *kb, qb, qw, *vw, ko_v, k_p):
                        idx = (i % ref.shape[0],) + (0,) * (len(ref.shape) - 3) + (slice(0, 8), slice(0, 128))
                        z_v[...] = z_v[...] + ref[idx].astype(f32)
                    z_v[...] = z_v[...] + vt_p[pl.ds(_mo(i * 8, 8), 8), 0:128].astype(f32) + qt_v[pl.ds(_mo(i * 8, 8), 8), 0:128]
                return c
            jax.lax.fori_loop(0, 2, dummy, 0)
            carry = (jnp.zeros((DH, TQ), f32), jnp.zeros((DH // 2, CK), u32))
    los, his = [one] * 8, [one] * 8
    for h in range(H):
        for n in range(S // 128):
            part = l_v[h, :, pl.ds(n * 128, 128)]
            los[n % 8] = jnp.minimum(los[n % 8], part)
            his[n % 8] = jnp.maximum(his[n % 8], part)
    while len(los) > 1:
        los = [jnp.minimum(a, b) for a, b in zip(los[::2], los[1::2])]
        his = [jnp.maximum(a, b) for a, b in zip(his[::2], his[1::2])]
    lo, hi = los[0], his[0]
    safe = (lo >= L_MIN) & (hi <= L_MAX) & (big <= A_MAX)
    redo = jnp.max(jnp.where(safe, float(FORCE_SAFE), 1.0)) > 0.0

    @pl.when(redo)
    def _():
        def safe_step(i, carry):
            h, b = i // (S // TS), i % (S // TS)
            cols = pl.ds(_mo(b * TS, TS), TS)
            q = qt_v[pl.ds(_mo(h * DH, DH), DH), cols]
            row_head = jax.lax.broadcasted_iota(i32, (128, TS), 0) // DH
            qm = jnp.where(row_head == h % 8, jnp.tile(q, (8, 1)), 0.0)
            s = _mm(_keys(k_p[h // 8]), qm)
            p = jnp.exp2(s - jnp.max(s, axis=0, keepdims=True))
            v = pltpu.bitcast(vt_p[pl.ds(_mo(h * (DH // 2), DH // 2), DH // 2), :], bf16)
            ot_v[pl.ds(_mo(h * DH, DH), DH), cols] = _mm(v, p)
            l_v[h, :, cols] = jnp.sum(p.reshape(S // 8, 8, TS), axis=0)
            return carry
        jax.lax.fori_loop(0, H * (S // TS), safe_step, 0)

    b1 = b1_ref[...].astype(f32).reshape(1, F)
    b2 = b2_ref[...].astype(f32).reshape(1, D)
    RH, FH = R3 // 2, F // 2

    def out_copy(i):
        rows = pl.ds(i * R3, R3)
        return pltpu.make_async_copy(out_v.at[rows], out_hbm.at[rows], out_sem.at[i])

    def quadrants(i):
        return [(pl.ds(i * R3 + r * RH, RH), pl.ds(c * DQ, DQ)) for r in range(2) for c in range(2)]

    def normalize(i, srcs=(None,)):
        rows = pl.ds(i * R3, R3)
        ot = []
        for h in range(H):
            lsum = jnp.sum(tie(l_v[h, :, rows], srcs[h * len(srcs) // H]), axis=0, keepdims=True)
            inv = pl.reciprocal(lsum, approx=True)
            ot.append(ot_v[pl.ds(h * DH, DH), rows] * (inv * (2.0 - lsum * inv)))
        o = jnp.concatenate(ot, axis=0).T
        if WO7:
            for j, op in enumerate(_lhs7(o[:RH, :DQ], o[:RH, DQ:], o[RH:, :DQ], o[RH:, DQ:])):
                o7[i % 4, j] = op
        else:
            for j, op in enumerate((o[:RH, :DQ], o[:RH, DQ:], o[RH:, :DQ], o[RH:, DQ:])):
                o7[i % 4, j] = op

    def out_proj(i):
        if WO7:
            ys = _join7([_mm(o7[i % 4, j], pltpu.bitcast(wo7[j], bf16)) for j in range(7)])
        else:
            o = jnp.concatenate([jnp.concatenate([o7[i % 4, 2 * r], o7[i % 4, 2 * r + 1]], axis=1) for r in range(2)], axis=0)
            y = _mm(o, wo_v[...])
            ys = (y[:RH, :DQ], y[:RH, DQ:], y[RH:, :DQ], y[RH:, DQ:])
        for q, y in zip(quadrants(i), ys):
            h_v[q] = x_v[q].astype(f32) + y

    def ln2(i, srcs=(None,)):
        step = RH // len(srcs)
        for n, src in enumerate(srcs):
            halves = []
            for r in range(2):
                hid = h_v[pl.ds(i * R3 + r * RH + n * step, step), :]
                hid = jnp.concatenate([tie(hid[:, 0:128], src), hid[:, 128:]], axis=1)
                halves.append(_ln(hid))
            top, bot = halves
            for j, op in enumerate(_lhs7(top[:, :DQ], top[:, DQ:], bot[:, :DQ], bot[:, DQ:])):
                hn7[i % 4, j, pl.ds(n * step, step), :] = op

    def ffn_up(i, f0):
        w = min(FC, FH - f0)
        ms = {j: _mm(hn7[i % 4, j], pltpu.bitcast(w17[j, :, pl.ds(f0, w)], bf16)) for j in ORD}
        bias = [b1[:, f0:f0 + w], b1[:, FH + f0:FH + f0 + w]] * 2
        act = [_gelu(a + bb) for a, bb in zip(_join7(ms), bias)]
        for j, op in enumerate(_lhs7(*act)):
            g7[i % 2, j, :, pl.ds(f0, w)] = _pack(op)

    def ffn_down(i, j):
        return _mm(g7[i % 2, j], pltpu.bitcast(w27[j], bf16))

    def finish(i, ms):
        for q, y, bb in zip(quadrants(i), _join7(ms), [b2[:, :DQ], b2[:, DQ:]] * 2):
            out_v[q] = (h_v[q] + y + bb).astype(out_v.dtype)
        out_copy(i).start()

    with jax.named_scope("phase3"):
        last = ot_v[pl.ds((H - 1) * DH, DH), pl.ds((NB - 1) * TQ, TQ)]
        store_block(H // HU - 1, jnp.where(redo, last, finish_step(*carry[:2])))
        if ONLY in (0, 3):
            normalize(0)
            out_proj(0)
            normalize(1)
            out_proj(1)
            ln2(0)
            for i in range(n3):
                for f0 in range(0, FH, FC):
                    ffn_up(i, f0)
                if 0 < i < n3 - 1:
                    out_proj(i + 1)
                ms = [ffn_down(i, j) for j in range(7)]
                if i + 1 < n3:
                    ln2(i + 1, [None, ms[0], ms[1], ms[2]] if MIX & 1 else spread(ms[:LNE], LNP))
                if i + 2 < n3:
                    normalize(i + 2, [ms[3], ms[4], ms[5], ms[6]] if MIX & 2 else spread(ms[NS:NE], NP))
                finish(i, ms)
        else:
            for i in range(n3):
                out_copy(i).start()
    with jax.named_scope("tail"):
        for i in range(n3):
            out_copy(i).wait()


@jax.jit
def pallas_sequential_preLN__softmax_full_mha__dense_activation_gelu__prompt_kernel(
        A_x, A_wqkv, A_wo, B_x, B_w1, B_b1, B_w2, B_b2):
    del B_x
    any_spec = pl.BlockSpec(memory_space=pl.ANY)
    vmem_spec = pl.BlockSpec(memory_space=pltpu.VMEM)
    vm = pltpu.VMEM
    out = pl.pallas_call(
        _kernel,
        out_shape=jax.ShapeDtypeStruct((S, D), A_x.dtype),
        in_specs=[any_spec] * 7,
        out_specs=any_spec,
        scratch_shapes=[
            vm((S, D), bf16), vm((D, 3 * D), bf16), vm((D, D), bf16), vm((D, F), bf16), vm((F, D), bf16),
            *[vm((7, D // 4, D // 2), u32)] * 3, vm((D, D), bf16), vm((D, D), bf16), vm((512, D), f32),
            vm((S // R1, 7, R1 // 2, D // 2), f32),
            vm((D // 128, S * 8 // TR, 128), f32 if KF else u32), vm((D // 128, V0[NC], 128), f32),
            vm((D, S), f32), vm((D // 2, S), u32), vm((D, S), f32), vm((H, 8, S), f32),
            vm((HU, V0[NC], 128), f32), vm((HU, NB, DH, TQ), f32), vm((HU, NB, DH, 8, TQ), f32), vm((OFF * TR, TQ), f32), vm((CK, TQ), f32),
            vm((8, 128), f32),
            vm((7, D // 4, D // 2), u32), vm((7, D // 4, F // 2), u32), vm((7, F // 4, D // 2), u32),
            vm((4, 7, R3 // 2, D // 2), f32), vm((4, 7, R3 // 2, D // 2), f32), vm((2, 7, R3 // 2, F // 2), f32),
            vm((S, D), f32), vm((S, D), bf16),
            pltpu.SemaphoreType.DMA((11,)), pltpu.SemaphoreType.DMA((S // R3,)),
            *[vm((T0[NC] * 8, 128), f32 if KF else u32)] * HU, *[vm((OFF * 8, 128), f32 if KF else u32)] * HU,
            *[vm((DH, V0[NC], 128), f32)] * HU, *[vm((1, DH // 2, S), u32)] * HU,
            vm((F,), bf16), vm((D,), bf16),
        ],
        compiler_params=pltpu.CompilerParams(vmem_limit_bytes=100 * 1024 * 1024),
    )(A_x.reshape(S, D), A_wqkv, A_wo, B_w1, B_b1, B_w2, B_b2)
    return out.reshape(A_x.shape)
```

```python
import functools
import jax
import jax.numpy as jnp
import numpy as np
import jax.experimental.pallas as pl
import jax.experimental.pallas.tpu as pltpu

S, D, F, H, DH = 2048, 512, 1792, 32, 16
TQ = 512
NQ = TQ // 128
NB = S // TQ
CK = 128
NC = S // CK
PAT = [16,16,32,16]
NVB = [[PAT[c % len(PAT)] for c in range(NC)]] * NB
KF = 0
TR = 8 if KF else 16
NTB = [[(CK - v) // TR for v in nv] for nv in NVB]
NV = [max(v) for v in zip(*NVB)]
NT = [max(v) for v in zip(*NTB)]
V0 = [sum(NV[:c]) for c in range(NC + 1)]
T0 = [sum(NT[:c]) for c in range(NC + 1)]
HU = 4
OFF = 2
TSH = 8
KSP = 2
R1 = 256
R3 = 128
U1 = 1
FC = 256
ONLY = 0
FORCE_SAFE = 0
DMAP = 0
RCP = 1
MIX = 0
ORD = [range(7), (1, 3, 2, 4, 0, 5, 6), (0, 1, 3, 2, 4, 5, 6), (4, 2, 3, 1, 0, 6, 5)][0]
WO7 = 1
PR = 16
XF = 1
WP = 0
TORD = 0
NTM = 2
VB = 1
KQ = 2
KP = 16
MP = 16
KSPAN = 32
MID = 9
QA = 0
DYN = 1
ALIVE = 0
CHK = 2
LSPAN = 56
LOFF = 4
DBG = 0
VEXP = 1
VPOS = 1
assert VPOS
MOFF = [CK - t * TR for t in NT]
VOFF = [0] * NC
FEN = 0
SCH = 0
SCHK, SCHM, SCHV = SCH, SCH, SCH
READY = lambda sch: (HU - 1, 1, HU - 2)[sch]
FC2 = 1
KS = 0
QS = 0
LP = 16
LT = 3
PORD = 0
SR = 1
VB4 = 1024
KE = 5
OORD = 1
TREE = 2
KA = 0
MA = 1
MSH = 0
LNE = 3
LNP = 8
NS = 3
NE = 7
NP = 32
TMA = 1023
TML = 10
KOFF = 2
KOFF0 = KOFF
MSPAN = 16
MOFFS = 35
LMSPAN = 16
LMOFF = LOFF
PRE = 0
QSH = 1
QS2 = 1
qslot = lambda q, d: d // 4 * 4 + (d + QSH + QS2 * q) % 4
TS = 128
EPS = 1e-5
L_MIN, L_MAX, A_MAX = 2.0 ** -40, 2.0 ** 40, 2.0 ** 80
bf16, f32, u32, i32 = jnp.bfloat16, jnp.float32, jnp.uint32, jnp.int32
Q_SCALE = float(DH ** -0.5 * np.log2(np.e))


def _mo(x, n):
    return x if isinstance(x, int) else pl.multiple_of(x, n)


def _mm(a, b):
    return jax.lax.dot_general(a, b, (((1,), (0,)), ((), ())), preferred_element_type=f32)


def _mm_nt(a, b):
    return jax.lax.dot_general(a, b, (((1,), (1,)), ((), ())), preferred_element_type=f32)


def _take(x, idx, axis):
    return jnp.take_along_axis(x, idx, axis=axis, mode="promise_in_bounds", wrap_negative_indices=False)


def _pack(x):
    return x


def _keys(x):
    return x if KF else pltpu.bitcast(x, bf16)


def _lhs7(a11, a12, a21, a22):
    return (a11 + a22, a21 + a22, a11, a22, a11 + a12, a21 - a11, a12 - a22)


def _rhs7(b11, b12, b21, b22):
    return (b11 + b22, b11, b12 - b22, b21 - b11, b22, b11 + b12, b21 + b22)


def _join7(m):
    return (m[0] + m[3] - m[4] + m[6], m[2] + m[4], m[1] + m[3], m[0] - m[1] + m[2] + m[5])


def _ln(x):
    m = jnp.mean(x, axis=-1, keepdims=True)
    xc = x - m
    v = jnp.mean(xc * xc, axis=-1, keepdims=True)
    return xc * jax.lax.rsqrt(v + EPS)


def _gelu(x):
    c = float(np.sqrt(2.0 / np.pi))
    return (0.5 * x) * (1.0 + jnp.tanh(x * (c + (c * 0.044715) * (x * x))))


def _kernel(x_hbm, wqkv_hbm, wo_hbm, w1_hbm, b1_hbm, w2_hbm, b2_hbm, out_hbm,
            x_v, wqkv_v, wo_v, w1_v, w2_v, wq7, wk7, wv7, wt_v, wtq_v, xn_v, xn7, k_p, ko_v, qt_v, vt_p, ot_v, l_v,
            qw, qb, qwl, qbl, p0_v, pc_v, z_v, range_v, wo7, w17, w27, o7, hn7, g7, h_v, out_v, in_sem, out_sem, *slots):
    km, kx, kb, vw = (slots[i * HU:(i + 1) * HU] for i in range(4))
    b1_ref, b2_ref = slots[4 * HU:]
    n3 = S // R3
    wqk7 = (wq7, wk7)

    XA = 512

    def part(src, dst, rows, cols, i):
        return pltpu.make_async_copy(src.at[rows, cols], dst.at[rows, cols], in_sem.at[i])
    every = slice(None)
    cp_x = [part(x_hbm, x_v, pl.ds(r0, n), every, i) for i, (r0, n) in enumerate(((0, XA), (XA, XA), (2 * XA, S - 2 * XA)))]
    cp_q, cp_k, cp_v = [part(wqkv_hbm, wqkv_v, every, pl.ds(i * D, D), 3 + i) for i in range(3)]
    cp_w = [part(src, dst, every, every, 6 + i) for i, (src, dst) in enumerate(((wo_hbm, wo_v), (w1_hbm, w1_v), (w2_hbm, w2_v)))]
    cp_w += [pltpu.make_async_copy(src, dst, in_sem.at[9 + i]) for i, (src, dst) in enumerate(((b1_hbm, b1_ref), (b2_hbm, b2_ref)))]
    for c in (cp_x[0], cp_k, cp_q, cp_x[1], cp_v, cp_x[2], *cp_w):
        c.start()

    DQ, H1 = D // 2, R1 // 2

    def tie(x, src):
        if src is None:
            return x
        reps = (x.shape[0] // 8, x.shape[1] // 128)
        src = src[0:8, 0:128]
        src = src if x.dtype == src.dtype else pltpu.bitcast(src, x.dtype)
        return jnp.where(jnp.tile(z_v[...], reps) >= 0.0, x, jnp.tile(src, reps))

    def spread(results, n):
        if not results:
            return [None] * n
        tiles = [(y, r, c) for y in results for c in range(0, y.shape[1], 128) for r in range(0, y.shape[0], 8)]
        picks = [tiles[i * len(tiles) // n] for i in range(n)]
        return [y[r:r + 8, c:c + 128] for y, r, c in picks]

    def ln1(r0, r1, plain=False, results=()):
        pieces = [(i, r) for i in range(r0 // R1, r1 // R1) for r in range(0, H1, LP)]
        for (i, r), src in zip(pieces, spread(results, len(pieces))):
            halves = []
            for half in range(2):
                rows = pl.ds(i * R1 + half * H1 + r, LP)
                x = x_v[rows, :].astype(f32)
                halves.append(_ln(jnp.concatenate([tie(x[:, 0:128], src), x[:, 128:]], axis=1)))
                if plain:
                    xn_v[rows, :] = halves[-1]
            if plain:
                continue
            top, bot = halves
            for j, op in enumerate(_lhs7(top[:, :DQ], top[:, DQ:], bot[:, :DQ], bot[:, DQ:])):
                xn7[i, j, pl.ds(r, LP), :] = op

    def split_rows(r1, results):
        pieces = [(i, r) for i in range(r1 // R1) for r in range(0, H1, LP)]
        for (i, r), src in zip(pieces, spread(results, len(pieces))):
            top, bot = (tie(xn_v[pl.ds(i * R1 + half * H1 + r, LP), :], src) for half in range(2))
            for j, op in enumerate(_lhs7(top[:, :DQ], top[:, DQ:], bot[:, :DQ], bot[:, DQ:])):
                xn7[i, j, pl.ds(r, LP), :] = op

    def split_weights(jobs, results, order=(0, 1, 2, 3)):
        pieces = [(src, c0, n, dst, r, c) for src, c0, n, dst in jobs
                  for r in range(0, src.shape[0] // 2, 16) for c in range(0, n // 2, 128)]
        for (src, c0, n, dst, r, c), wait_for in zip(pieces, spread(results, len(pieces))):
            quad = []
            for i in range(2):
                for j in range(2):
                    w = pltpu.bitcast(src[pl.ds(r + i * src.shape[0] // 2, 16), pl.ds(c0 + j * n // 2 + c, 128)], u32)
                    quad.append(pltpu.bitcast(tie(w, wait_for), bf16).astype(f32))
            for i, op in enumerate(_rhs7(*[quad[o] for o in order])):
                dst[i, pl.ds(r // 2, 8), pl.ds(c, 128)] = pltpu.bitcast(op.astype(bf16), u32)

    def project(which, i, plain):
        if plain:
            y = _mm(xn_v[pl.ds(i * R1, R1), :], wqkv_v[:, pl.ds(which * D, D)])
            return y, [y]
        ms = [_mm(xn7[i, j], pltpu.bitcast(wqk7[which][j], bf16)) for j in range(7)]
        c11, c12, c21, c22 = _join7(ms)
        return jnp.concatenate([jnp.concatenate([c11, c12], axis=1), jnp.concatenate([c21, c22], axis=1)], axis=0), ms

    def project_t(w7, i):
        ms = [_mm_nt(pltpu.bitcast(w7[j], bf16), xn7[i, j]) for j in range(7)]
        c11, c12, c21, c22 = _join7(ms)
        return jnp.concatenate([jnp.concatenate([c11, c21], axis=1), jnp.concatenate([c12, c22], axis=1)], axis=0), ms

    def proj_q(r0, r1, plain=False):
        made = []
        for i in range(r0 // R1, r1 // R1):
            if plain:
                q, ms = project(0, i, plain)
                qt = q.T
            else:
                qt, ms = project_t(wq7, i)
            qt_v[:, pl.ds(i * R1, R1)] = qt * Q_SCALE
            made += ms
        return made

    def proj_k(r0, r1, plain=False):
        made = []
        for i in range(r0 // R1, r1 // R1):
            k, ms = project(1, i, plain)
            kp = k if KF else pltpu.bitcast(k.astype(bf16), u32)
            for g in range(D // 128):
                lanes = slice(g * 128, (g + 1) * 128)
                k_p[g, pl.ds(i * R1 * 8 // TR, R1 * 8 // TR), :] = kp[:, lanes]
                for c in range(i * R1 // CK, (i + 1) * R1 // CK):
                    r = c * CK + VOFF[c] - i * R1
                    ko_v[g, pl.ds(V0[c], NV[c]), :] = k[r:r + NV[c], lanes]
            made += ms
        return made

    peaks = [jnp.zeros((8, 128), f32)] * 2
    lane = jax.lax.broadcasted_iota(i32, (8, 128), 1)

    def proj_v(r0, r1):
        made = []
        for i in range(r0 // R1, r1 // R1):
            vt, ms = project_t(wv7, i)
            vt_p[:, pl.ds(i * R1, R1)] = pltpu.bitcast(vt.astype(bf16), u32)
            for n in range(R1 // 128):
                for r in range(0, D, 8):
                    peaks[n % 2] = jnp.maximum(peaks[n % 2], jnp.abs(vt[r:r + 8, n * 128:(n + 1) * 128]))
            made += ms
        return made


    key_tiles = [(c, t) for c in range(NC) for t in range(NT[c])]

    def stage_mxu_keys(h, u, part, parts, after=lambda x: x, zero=0):
        mine = range(part * len(key_tiles) // parts, (part + 1) * len(key_tiles) // parts)
        idx = after((lane + (h % 8) * DH) & 127)
        for g in mine:
            c, t = key_tiles[g]
            kp = k_p[h // 8, pl.ds((c * CK + MOFF[c]) * 8 // TR + t * 8, 8), :]
            km[u][pl.ds(_mo((g + zero) * 8, 8), 8), :] = _take(kp, idx, axis=1)
            if c == 0 and t >= NT[0] - OFF:
                moved = _take(kp, (idx + (128 - DH)) & 127, axis=1)
                kx[u][pl.ds(_mo((t - NT[0] + OFF + zero) * 8, 8), 8), :] = jnp.where((lane >= DH) & (lane < 2 * DH), moved, jnp.zeros_like(moved))

    def stage_values(h, u, zero=0):
        vw[u][zero] = vt_p[pl.ds(_mo(h * (DH // 2), DH // 2), DH // 2), :]

    def stage_vpu_keys(h, u, part, parts, after=lambda x: x, zero=0):
        d, sub = divmod(part, parts // DH)
        n = V0[NC] // 8
        r0, r1 = sub * n // (parts // DH), (sub + 1) * n // (parts // DH)
        idx = after(jnp.full((8, 128), (h % 8) * DH + d, i32))
        rows = pl.ds(r0 * 8, (r1 - r0) * 8)
        src = ko_v[h // 8, rows, :]
        for r in range(r0, r1):
            kb[u][r + zero, d] = _take(src[(r - r0) * 8:(r - r0 + 1) * 8], idx, axis=1)

    def query_slot(u, b):
        return (qwl, qbl, 0) if (u, b) == (HU - 1, NB - 1) else (qw, qb, u * NB + b)

    def stage_query(h, u, b, d, after=lambda x: x, zero=0):
        plain, spread_out, slot = query_slot(u, b)
        q = qt_v[pl.ds(_mo(h * DH + d // 8 * 8, 8), 8), pl.ds(b * TQ, TQ)]
        idx = after(jnp.full((8, 128), d % 8, i32))
        for n in range(NQ):
            spread_out[slot + zero, n, qslot(n, d)] = _take(q[:, n * 128:(n + 1) * 128], idx, axis=0)
        if d % 8 == 0:
            plain[slot + zero, pl.ds(d, 8), :] = q

    z_v[...] = jnp.zeros((8, 128), f32)
    def stage_keys(heads, results):
        jobs = []
        for u in heads:
            if u < READY(SCHM):
                jobs += [functools.partial(stage_mxu_keys, u, u, c, NC) for c in range(NC)]
            if u < READY(SCHK):
                jobs += [functools.partial(stage_vpu_keys, u, u, d, DH) for d in range(DH)]
        for job, src in zip(jobs, spread(results, len(jobs))):
            job(functools.partial(tie, src=src))

    with jax.named_scope("wait0"):
        cp_x[0].wait()
        ln1(0, XA, plain=True)
        cp_k.wait()
    with jax.named_scope("phase1"):
        on = ONLY in (0, 1, 4)
        if on:
            made = proj_k(0, XA, plain=True)
            split_weights([(wqkv_v, D, D, wqk7[1])], made[:-1])
            if SR == 1:
                split_rows(XA, ())
        cp_q.wait()
        cp_x[1].wait()
        if on:
            made = proj_q(0, XA, plain=True)
            ln1(XA, 2 * XA, results=made[:1] if LT & 1 else ())
            if SR == 2:
                split_rows(XA, made[1:])
            made = proj_k(XA, 2 * XA)
            wtq_v[...] = wqkv_v[:, pl.ds(0, D)].T
            split_weights([(wtq_v, 0, D, wq7)], made[3:-4], order=(0, 2, 1, 3))
            if SR == 0:
                split_rows(XA, made[:-4])
        cp_v.wait()
        cp_x[2].wait()
        if on:
            wt_v[...] = wqkv_v[:, pl.ds(2 * D, D)].T
            made = proj_q(XA, 2 * XA)
            split_weights([(wt_v, 0, D, wv7)], made[3:-3], order=(0, 2, 1, 3))
            if SR == 3:
                split_rows(XA, made[:-4])
            if PORD == 0:
                made += proj_v(0, XA)
                ln1(2 * XA, S, results=made[:-7] if LT & 2 else ())
                proj_k(2 * XA, S)
            else:
                ln1(2 * XA, S, results=made[:7] if LT & 2 else ())
                proj_k(2 * XA, S)
                made = proj_v(0, XA)
                stage_keys(range(1), made[:-3])
        cp_w[0].wait()
        cp_w[1].wait()
        qs = proj_q(2 * XA, S) if on else []
        vs = proj_v(XA, VB4) if on else []
        stage_keys(range(KQ), qs + vs[:-KE])
        split_weights([(wo_v, 0, D, wo7), (w1_v, 0, F, w17)], qs + vs[:-KE])
        for c in cp_w[2:]:
            c.wait()
        vs = proj_v(VB4, S)[:-KE] if on else []
        stage_keys(range(KQ, HU - 1), vs)
        blocks = [divmod(blk, NB) for blk in range(HU * NB - 1)]
        marks = iter(spread(vs, len(blocks) * DH))
        for u, b in blocks:
            for d in range(DH):
                stage_query(u, u, b, d, functools.partial(tie, src=next(marks)))
        split_weights([(w2_v, 0, D, w27)], vs)
        for u in range(READY(SCHV)):
            stage_values(u, u)

    def query_weights(*blocks):
        w = [plain[slot] for plain, _, slot in (query_slot(u, b) for u, b in blocks)]
        return jnp.concatenate(w + [jnp.zeros((128 - DH * len(w), TQ), f32)], axis=0)

    def finish_step(acc, v):
        return acc + _mm(pltpu.bitcast(v, bf16), pc_v[...])

    def store_block(it, acc):
        ot_v[pl.ds(_mo((it * HU + HU - 1) * DH, DH), DH), pl.ds((NB - 1) * TQ, TQ)] = acc

    def fast_step(it, carry):
        items = [(u, b, c) for u in range(HU) for b in range(NB) for c in range(NC)]
        tiles, first, ties = [], [], {}
        for u in range(HU):
            for b in range(NB):
                start, n0, outs = len(tiles), len(first), []
                for c in range(NC):
                    first.append(len(tiles))
                    tiles += [(u, b, c, t) for t in range(NTB[b][c])]
                    if OORD == 1:
                        outs += [(n0 + c, q, r) for q in range(NQ) for r in reversed(range(NVB[b][c] // 8))]
                    else:
                        outs += [(n0 + c, q, r) for r in reversed(range(NVB[b][c] // 8)) for q in range(NQ)]
                for o, key in enumerate(outs):
                    if (TMA >> o % TML) & 1:
                        ties.setdefault(max(start + o * (len(tiles) - start) // len(outs) + TSH, OFF), []).append(key)
        first.append(len(tiles))
        tiles += tiles[:OFF]
        head = lambda u: it * HU + u
        later = lambda u: jnp.minimum(it + 1, H // HU - 1) * HU + u
        always, also = z_v[...] >= 0.0, z_v[...] <= 0.0
        sv, st = {}, {}

        def vpu_scores(n, q, r):
            if (n, q, r) not in sv:
                u, b, c = items[n]
                _, spread_out, slot = query_slot(u, b)
                accs = [None] * TREE
                for d in range(DH):
                    t = kb[u][V0[c] // 8 + r, d] * spread_out[slot, q, qslot(q, d)]
                    accs[d % TREE] = t if accs[d % TREE] is None else accs[d % TREE] + t
                acc = functools.reduce(jnp.add, accs)
                sv[n, q, r] = jnp.exp2(acc) if VEXP else acc
            return sv[n, q, r]

        def key_tile(g, moved=False):
            u, b, c, t = tiles[g]
            if moved:
                kt = kx[u][pl.ds((OFF - 1 - t) * 8, 8), :]
            else:
                kt = km[u][pl.ds((T0[c + 1] - 1 - t) * 8, 8), :]
            for key, true in zip(ties.get(g, ()), (always, also) * 4):
                val = vpu_scores(*key)
                kt = jnp.where(true, kt, val if KF else pltpu.bitcast(val, u32))
            return kt

        def mxu_scores(g0, g1):
            if tiles[g0][:2] != tiles[g1 - 1][:2]:
                lhs = [jnp.where(lane < DH, key_tile(g), 0.0 if KF else 0) for g in range(g0, g1 - OFF)]
                lhs += [key_tile(g, True) for g in range(g1 - OFF, g1)]
                w = query_weights(tiles[g0][:2], tiles[g1 - 1][:2])
            else:
                lhs = [key_tile(g) for g in range(g0, g1)]
                w = query_weights(tiles[g0][:2])
            s = _mm(_keys(jnp.concatenate(lhs, axis=0)), w)
            for g in range(g0, g1):
                st[g] = s[(g - g0) * TR:(g - g0 + 1) * TR]

        def weights(n, l):
            u, b, c = items[n]
            rows = [st.pop(first[n + 1] - 1 - t) for t in range(NTB[b][c])]
            more = [jnp.concatenate([vpu_scores(n, q, r) for q in range(NQ)], axis=1) for r in range(NVB[b][c] // 8)]
            if VEXP:
                rows = [jnp.exp2(jnp.concatenate(rows, axis=0))]
                p = jnp.concatenate(more + rows if VPOS else rows + more, axis=0)
            else:
                p = jnp.exp2(jnp.concatenate(rows + more, axis=0))
            for r in reversed(range(CK // 8)):
                row = p[r * 8:(r + 1) * 8]
                l = row if l is None else l + row
            return p, l

        for g in range(OFF):
            st[g] = p0_v[pl.ds(g * TR, TR), :]
        l = acc = None
        for m in range(len(items) + 1):
            def early(lo, hi):
                for g in range(lo, hi):
                    for key in ties.get(g, ()):
                        vpu_scores(*key)
            if m < len(items):
                if PRE > 0:
                    early(first[m] + OFF, first[m + 1] + OFF + PRE)
                mxu_scores(first[m] + OFF, first[m + 1] + OFF)
                if PRE < 0:
                    early(first[m] + OFF, first[m + 1] + OFF - PRE)
            if m == 0:
                store_block(jnp.maximum(it - 1, 0), finish_step(*carry[:2]))
                continue
            u, b, c = items[m - 1]
            if c == 0:
                l, acc = None, jnp.tile(z_v[...], (DH // 8, NQ))
            p, l = weights(m - 1, l)
            v = vw[u][0, :, pl.ds(c * CK, CK)]
            if m < len(items):
                acc = acc + _mm(pltpu.bitcast(v, bf16), p)
            else:
                nv = NVB[b][c]
                late = jnp.tile(p[nv:nv + 8], (nv // 8, 1))
                keep = jnp.tile(z_v[...], (nv // 8, NQ)) >= 0.0
                pc_v[pl.ds(nv, CK - nv), :] = p[nv:]
                pc_v[pl.ds(0, nv), :] = jnp.where(keep, p[:nv], late)

            def after(x, src=l[:, 0:128]):
                return jnp.where(always, x, pltpu.bitcast(src, i32))

            def after2(x, src=p[MID * 8:MID * 8 + 8, 0:128]):
                return jnp.where(always, x, pltpu.bitcast(src, i32))
            def target(sch):
                if sch == 0:
                    return (later(u - 1) if u > 0 else head(HU - 1)), (u - 1) % HU, jnp.minimum(it, 0) if u == 0 or DYN == 2 else 0
                if sch == 2:
                    return (later(u - 2) if u > 1 else head(u + HU - 2)), (u - 2) % HU, jnp.minimum(it, 0) if u < 2 or DYN == 2 else 0
                return (head(u + 1) if u < HU - 1 else later(0)), (u + 1) % HU, jnp.minimum(it, 0) if u < HU - 1 or DYN == 2 else 0
            span, n = (LSPAN, b * NC + c - LOFF) if u == HU - 1 else (KSPAN, b * NC + c - (KOFF if u else KOFF0))
            mspan, mn = (LMSPAN, b * NC + c - LMOFF) if u == HU - 1 else (MSPAN, b * NC + c - MOFFS)
            for part in range(KP):
                if part * span // KP == n:
                    h_fill, slot, zero = target(SCHK)
                    stage_vpu_keys(h_fill, slot, part, KP, after2 if KA else after, zero)
            for part in range(MP):
                if part * mspan // MP == mn:
                    h_fill, slot, zero = target(SCHM)
                    stage_mxu_keys(h_fill, slot, part, MP, after2 if MA else after, zero)
            if n == 0:
                stage_values(*target(SCHV))
            blk = u * NB + b
            if blk > 0:
                stage_query(later((blk - 1) // NB), (blk - 1) // NB, (blk - 1) % NB, c, after2 if QA else after)
            else:
                stage_query(head(HU - 1), HU - 1, NB - 1, c, after2 if QA else after, jnp.minimum(it, 0))
            if c == NC - 1:
                l_v[head(u), :, pl.ds(b * TQ, TQ)] = l
                parts = [l[:, n * 128:(n + 1) * 128] for n in range(NQ)]
                range_v[0] = functools.reduce(jnp.minimum, parts, range_v[0])
                range_v[1] = functools.reduce(jnp.maximum, parts, range_v[1])
                if m < len(items):
                    ot_v[pl.ds(_mo(head(u) * DH, DH), DH), pl.ds(b * TQ, TQ)] = acc
        for g in range(OFF):
            p0_v[pl.ds(g * TR, TR), :] = st.pop(first[-1] + g)
        return acc, v

    one = jnp.ones((8, 128), f32)
    with jax.named_scope("phase2"):
        range_v[0] = one
        range_v[1] = one
        range_v[2] = jnp.maximum(*peaks)
        if ONLY in (0, 2):
            lead = _keys(jnp.concatenate(
                [k_p[0, pl.ds(MOFF[0] * 8 // TR + (NT[0] - 1 - t) * 8, 8), :] for t in range(OFF)], axis=0))
            p0_v[...] = _mm(lead, query_weights((0, 0)))
            pc_v[...] = jnp.zeros((CK, TQ), f32)
            carry = (jnp.zeros((DH, TQ), f32), jnp.zeros((DH // 2, CK), u32))
            carry = jax.lax.fori_loop(0, H // HU, fast_step, carry)
        else:
            def dummy(i, c):
                z_v[...] = jnp.abs(z_v[...])
                l_v[i] = l_v[i] + 1.0
                if ONLY == 4:
                    for ref in (wo7, w17, w27, *kb, qb, qw, qbl, qwl, *km, *kx, *vw, ko_v, k_p):
                        idx = (i % ref.shape[0],) + (0,) * (len(ref.shape) - 3) + (slice(0, 8), slice(0, 128))
                        z_v[...] = z_v[...] + ref[idx].astype(f32)
                    z_v[...] = z_v[...] + vt_p[pl.ds(_mo(i * 8, 8), 8), 0:128].astype(f32) + qt_v[pl.ds(_mo(i * 8, 8), 8), 0:128]
                return c
            jax.lax.fori_loop(0, 2, dummy, 0)
            carry = (jnp.zeros((DH, TQ), f32), jnp.zeros((DH // 2, CK), u32))
    safe = (range_v[0] >= L_MIN) & (range_v[1] <= L_MAX) & (range_v[2] <= A_MAX)
    redo = jnp.max(jnp.where(safe, float(FORCE_SAFE), 1.0)) > 0.0

    @pl.when(redo)
    def _():
        def safe_step(i, carry):
            h, b = i // (S // TS), i % (S // TS)
            cols = pl.ds(_mo(b * TS, TS), TS)
            q = qt_v[pl.ds(_mo(h * DH, DH), DH), cols]
            row_head = jax.lax.broadcasted_iota(i32, (128, TS), 0) // DH
            qm = jnp.where(row_head == h % 8, jnp.tile(q, (8, 1)), 0.0)
            s = _mm(_keys(k_p[h // 8]), qm)
            p = jnp.exp2(s - jnp.max(s, axis=0, keepdims=True))
            v = pltpu.bitcast(vt_p[pl.ds(_mo(h * (DH // 2), DH // 2), DH // 2), :], bf16)
            ot_v[pl.ds(_mo(h * DH, DH), DH), cols] = _mm(v, p)
            l_v[h, :, cols] = jnp.sum(p.reshape(S // 8, 8, TS), axis=0)
            return carry
        jax.lax.fori_loop(0, H * (S // TS), safe_step, 0)

    b1 = b1_ref[...].astype(f32).reshape(1, F)
    b2 = b2_ref[...].astype(f32).reshape(1, D)
    RH, FH = R3 // 2, F // 2

    def out_copy(i):
        rows = pl.ds(i * R3, R3)
        return pltpu.make_async_copy(out_v.at[rows], out_hbm.at[rows], out_sem.at[i])

    def quadrants(i):
        return [(pl.ds(i * R3 + r * RH, RH), pl.ds(c * DQ, DQ)) for r in range(2) for c in range(2)]

    def normalize(i, srcs=(None,)):
        rows = pl.ds(i * R3, R3)
        ot = []
        for h in range(H):
            lsum = jnp.sum(tie(l_v[h, :, rows], srcs[h * len(srcs) // H]), axis=0, keepdims=True)
            inv = pl.reciprocal(lsum, approx=True)
            ot.append(ot_v[pl.ds(h * DH, DH), rows] * (inv * (2.0 - lsum * inv)))
        o = jnp.concatenate(ot, axis=0).T
        if WO7:
            for j, op in enumerate(_lhs7(o[:RH, :DQ], o[:RH, DQ:], o[RH:, :DQ], o[RH:, DQ:])):
                o7[i % 4, j] = op
        else:
            for j, op in enumerate((o[:RH, :DQ], o[:RH, DQ:], o[RH:, :DQ], o[RH:, DQ:])):
                o7[i % 4, j] = op

    def out_proj(i):
        if WO7:
            ys = _join7([_mm(o7[i % 4, j], pltpu.bitcast(wo7[j], bf16)) for j in range(7)])
        else:
            o = jnp.concatenate([jnp.concatenate([o7[i % 4, 2 * r], o7[i % 4, 2 * r + 1]], axis=1) for r in range(2)], axis=0)
            y = _mm(o, wo_v[...])
            ys = (y[:RH, :DQ], y[:RH, DQ:], y[RH:, :DQ], y[RH:, DQ:])
        for q, y in zip(quadrants(i), ys):
            h_v[q] = x_v[q].astype(f32) + y

    def ln2(i, srcs=(None,)):
        step = RH // len(srcs)
        for n, src in enumerate(srcs):
            halves = []
            for r in range(2):
                hid = h_v[pl.ds(i * R3 + r * RH + n * step, step), :]
                hid = jnp.concatenate([tie(hid[:, 0:128], src), hid[:, 128:]], axis=1)
                halves.append(_ln(hid))
            top, bot = halves
            for j, op in enumerate(_lhs7(top[:, :DQ], top[:, DQ:], bot[:, :DQ], bot[:, DQ:])):
                hn7[i % 4, j, pl.ds(n * step, step), :] = op

    def ffn_up(i, f0):
        w = min(FC, FH - f0)
        ms = {j: _mm(hn7[i % 4, j], pltpu.bitcast(w17[j, :, pl.ds(f0, w)], bf16)) for j in ORD}
        bias = [b1[:, f0:f0 + w], b1[:, FH + f0:FH + f0 + w]] * 2
        act = [_gelu(a + bb) for a, bb in zip(_join7(ms), bias)]
        for j, op in enumerate(_lhs7(*act)):
            g7[i % 2, j, :, pl.ds(f0, w)] = _pack(op)

    def ffn_down(i, j):
        return _mm(g7[i % 2, j], pltpu.bitcast(w27[j], bf16))

    def finish(i, ms):
        for q, y, bb in zip(quadrants(i), _join7(ms), [b2[:, :DQ], b2[:, DQ:]] * 2):
            out_v[q] = (h_v[q] + y + bb).astype(out_v.dtype)
        out_copy(i).start()

    with jax.named_scope("phase3"):
        last = ot_v[pl.ds((H - 1) * DH, DH), pl.ds((NB - 1) * TQ, TQ)]
        store_block(H // HU - 1, jnp.where(redo, last, finish_step(*carry[:2])))
        if ONLY in (0, 3):
            normalize(0)
            out_proj(0)
            normalize(1)
            out_proj(1)
            ln2(0)
            for i in range(n3):
                for f0 in range(0, FH, FC):
                    ffn_up(i, f0)
                if 0 < i < n3 - 1:
                    out_proj(i + 1)
                ms = [ffn_down(i, j) for j in range(7)]
                if i + 1 < n3:
                    ln2(i + 1, [None, ms[0], ms[1], ms[2]] if MIX & 1 else spread(ms[:LNE], LNP))
                if i + 2 < n3:
                    normalize(i + 2, [ms[3], ms[4], ms[5], ms[6]] if MIX & 2 else spread(ms[NS:NE], NP))
                finish(i, ms)
        else:
            for i in range(n3):
                out_copy(i).start()
    with jax.named_scope("tail"):
        for i in range(n3):
            out_copy(i).wait()


@jax.jit
def pallas_sequential_preLN__softmax_full_mha__dense_activation_gelu__prompt_kernel(
        A_x, A_wqkv, A_wo, B_x, B_w1, B_b1, B_w2, B_b2):
    del B_x
    any_spec = pl.BlockSpec(memory_space=pl.ANY)
    vmem_spec = pl.BlockSpec(memory_space=pltpu.VMEM)
    vm = pltpu.VMEM
    out = pl.pallas_call(
        _kernel,
        out_shape=jax.ShapeDtypeStruct((S, D), A_x.dtype),
        in_specs=[any_spec] * 7,
        out_specs=any_spec,
        scratch_shapes=[
            vm((S, D), bf16), vm((D, 3 * D), bf16), vm((D, D), bf16), vm((D, F), bf16), vm((F, D), bf16),
            *[vm((7, D // 4, D // 2), u32)] * 3, vm((D, D), bf16), vm((D, D), bf16), vm((512, D), f32),
            vm((S // R1, 7, R1 // 2, D // 2), f32),
            vm((D // 128, S * 8 // TR, 128), f32 if KF else u32), vm((D // 128, V0[NC], 128), f32),
            vm((D, S), f32), vm((D // 2, S), u32), vm((D, S), f32), vm((H, 8, S), f32),
            vm((HU * NB - 1, DH, TQ), f32), vm((HU * NB - 1, NQ, DH, 8, 128), f32), vm((1, DH, TQ), f32), vm((1, NQ, DH, 8, 128), f32), vm((OFF * TR, TQ), f32), vm((CK, TQ), f32),
            vm((8, 128), f32), vm((3, 8, 128), f32),
            vm((7, D // 4, D // 2), u32), vm((7, D // 4, F // 2), u32), vm((7, F // 4, D // 2), u32),
            vm((4, 7, R3 // 2, D // 2), f32), vm((4, 7, R3 // 2, D // 2), f32), vm((2, 7, R3 // 2, F // 2), f32),
            vm((S, D), f32), vm((S, D), bf16),
            pltpu.SemaphoreType.DMA((11,)), pltpu.SemaphoreType.DMA((S // R3,)),
            *[vm((T0[NC] * 8, 128), f32 if KF else u32)] * HU, *[vm((OFF * 8, 128), f32 if KF else u32)] * HU,
            *[vm((V0[NC] // 8, DH, 8, 128), f32)] * HU, *[vm((1, DH // 2, S), u32)] * HU,
            vm((F,), bf16), vm((D,), bf16),
        ],
        compiler_params=pltpu.CompilerParams(vmem_limit_bytes=120 * 1024 * 1024),
    )(A_x.reshape(S, D), A_wqkv, A_wo, B_w1, B_b1, B_w2, B_b2)
    return out.reshape(A_x.shape)
```

```python
import functools

import jax
import jax.numpy as jnp
import numpy as np
import jax.experimental.pallas as pl
import jax.experimental.pallas.tpu as pltpu

S, D, F, H, DH = 2048, 512, 1792, 32, 16
EPS = 1e-5
bf16, f32, u32, i32 = jnp.bfloat16, jnp.float32, jnp.uint32, jnp.int32
Q_SCALE = float(DH ** -0.5 * np.log2(np.e))
L_MIN, L_MAX, W_MAX = 2.0 ** -40, 2.0 ** 40, 2.0 ** 70


def _order(digits):
    return [int(ch) - 1 for ch in str(digits)]


def _span(lo, hi):
    return lo, max(hi, lo + 10)


R1 = 256
XA = 512
K_ORDER, T_ORDER = _order(2435167), _order(2435167)
LN1_SPAN = _span(0, 75)
KEY_CUTS = (0, 6, 14, 16)
KEY_SPANS = (_span(30, 80), _span(10, 95), _span(0, 80))
QUERY_CUTS = (0, 2, 4)
QUERY_SPANS = (_span(40, 70), _span(20, 80))
WEIGHT_SPANS = (_span(50, 88), _span(5, 45), _span(45, 84))

TQ = 512
NQ, NB = TQ // 128, S // TQ
CK = 128
NC = S // CK
HU = 4
NV = [(16, 16, 32, 16)[c % 4] for c in range(NC)]
NT = [(CK - v) // 16 for v in NV]
V0 = [sum(NV[:c]) for c in range(NC + 1)]
T0 = [sum(NT[:c]) for c in range(NC + 1)]
AHEAD = 2
LAG = 8
VPU_REFILL, LAST_VPU_REFILL = (2, 32), (4, 56)
MXU_REFILL, LAST_MXU_REFILL = (35, 16), (4, 16)
MID = 9
TS = 128

R3 = 256
FQ = 384
F2 = 4 * FQ
UP_ORDER, REST_ORDER = _order(2435167), _order(2435167)
DOWN_ORDER, PROJ_ORDER = _order(4721536), _order(2435167)
UP_INNER, DOWN_INNER = _order(2413567), _order(2413567)
REST_SPAN, DOWN_SPAN = (20, 20 + 100), (10, 100 - 10)
PROJ_SPAN = (0, 0 + 10)
LN2_SPAN, NORM_SPAN = (max(30, PROJ_SPAN[1] + 1), 95), (30, 70)
LN2_PIECES = 8


def _aligned(x, n):
    return x if isinstance(x, int) else pl.multiple_of(x, n)


def _mm(a, b):
    return jax.lax.dot_general(a, b, (((1,), (0,)), ((), ())), preferred_element_type=f32)


def _mm_nt(a, b):
    return jax.lax.dot_general(a, b, (((1,), (1,)), ((), ())), preferred_element_type=f32)


def _take(x, idx, axis):
    return jnp.take_along_axis(x, idx, axis=axis, mode="promise_in_bounds", wrap_negative_indices=False)


def _words(ref, *idx):
    return ref.bitcast(u32)[idx]


def _tiles(ref, *idx):
    return jnp.concatenate([pltpu.bitcast(_words(ref, *idx, c), bf16) for c in range(ref.shape[len(idx)])], axis=1)


def _whole(c11, c12, c21, c22):
    return jnp.concatenate([jnp.concatenate([c11, c12], axis=1), jnp.concatenate([c21, c22], axis=1)], axis=0)


def _lhs7(a11, a12, a21, a22):
    return (a11 + a22, a21 + a22, a11, a22, a11 + a12, a21 - a11, a12 - a22)


def _rhs7(b11, b12, b21, b22):
    return (b11 + b22, b11, b12 - b22, b21 - b11, b22, b11 + b12, b21 + b22)


_TERMS = (((0, 3, 6), (4,)), ((2, 4), ()), ((1, 3), ()), ((0, 2, 5), (1,)))


def _join7(ms, quadrant):
    plus, minus = _TERMS[quadrant]
    terms = [j for j in ms if j in plus + minus]
    if terms[0] in minus:
        terms[:2] = terms[1::-1]
    acc = ms[terms[0]]
    for j in terms[1:]:
        acc = acc - ms[j] if j in minus else acc + ms[j]
    return acc


def _completed(ms, j):
    return [n for n, (plus, minus) in enumerate(_TERMS) if j in plus + minus and all(i in ms for i in plus + minus)]


def _ln(x):
    m = jnp.mean(x, axis=-1, keepdims=True)
    xc = x - m
    v = jnp.mean(xc * xc, axis=-1, keepdims=True)
    return xc * jax.lax.rsqrt(v + EPS)


def _gelu(x):
    c = float(np.sqrt(2.0 / np.pi))
    return (0.5 * x) * (1.0 + jnp.tanh(x * (c + (c * 0.044715) * (x * x))))


def _qslot(q, d):
    return d // 4 * 4 + (d + 1 + q) % 4


def _kernel(x_hbm, wqkv_hbm, wo_hbm, w1_hbm, b1_hbm, w2_hbm, b2_hbm, out_hbm,
            x_v, wqkv_v, wo_v, w1_v, w2_v, wq7, wk7, wv7, wvt_v, wqt_v, xn_v, xn7,
            k_v, kvpu_v, qt_v, vt_v, ot_v, l_v, s0_v, pc_v, z_v, range_v,
            wo7, w17, w27, w149, w249, h_v, out_v, in_sem, out_sem, *slots):
    km, kx, kb, vw = (slots[i * HU:(i + 1) * HU] for i in range(4))
    qw, qb = (slots[4 * HU + i * HU * NB:4 * HU + (i + 1) * HU * NB] for i in range(2))
    b1_v, b2_v = slots[-2:]

    def fetch(src, dst, i, rows=slice(None), cols=slice(None)):
        return pltpu.make_async_copy(src.at[rows, cols], dst.at[rows, cols], in_sem.at[i])

    cp_x = [fetch(x_hbm, x_v, i, rows=pl.ds(r0, n)) for i, (r0, n) in enumerate(((0, XA), (XA, XA), (2 * XA, S - 2 * XA)))]
    cp_q, cp_k, cp_v = [fetch(wqkv_hbm, wqkv_v, 3 + i, cols=pl.ds(i * D, D)) for i in range(3)]
    cp_w = [fetch(wo_hbm, wo_v, 6), fetch(w1_hbm, w1_v, 7), fetch(w2_hbm, w2_v, 8),
            pltpu.make_async_copy(b1_hbm, b1_v, in_sem.at[9]), pltpu.make_async_copy(b2_hbm, b2_v, in_sem.at[10])]
    for cp in (cp_x[0], cp_k, cp_q, cp_x[1], cp_v, cp_x[2], *cp_w):
        cp.start()

    lane = jax.lax.broadcasted_iota(i32, (8, 128), 1)
    z_v[...] = jnp.zeros((8, 128), f32)

    def tie(x, src):
        if src is None:
            return x
        reps = (x.shape[0] // 8, x.shape[1] // 128)
        src = src[0:8, 0:128]
        src = src if x.dtype == src.dtype else pltpu.bitcast(src, x.dtype)
        return jnp.where(jnp.tile(z_v[...], reps) >= 0.0, x, jnp.tile(src, reps))

    def spread(results, n, span=(0, 100)):
        results = results[len(results) * span[0] // 100:len(results) * span[1] // 100]
        if not results:
            return [None] * n
        tiles = [(y, r, c) for y in results for c in range(0, y.shape[1], 128) for r in range(0, y.shape[0], 8)]
        picks = [tiles[i * len(tiles) // n] for i in range(n)]
        return [y[r:r + 8, c:c + 128] for y, r, c in picks]

    def stage_mxu_keys(h, u, tiles, after, zero=0):
        idx = after((lane + (h % 8) * DH) & 127)
        for g in tiles:
            c = max(c for c in range(NC) if T0[c] <= g)
            t = g - T0[c]
            words = _words(k_v, h // 8, pl.ds((c * CK + NV[c]) // 2 + t * 8, 8))
            km[u][pl.ds(_aligned((g + zero) * 8, 8), 8), :] = _take(words, idx, axis=1)
            if c == 0 and t >= NT[0] - AHEAD:
                moved = _take(words, (idx + (128 - DH)) & 127, axis=1)
                moved = jnp.where((lane >= DH) & (lane < 2 * DH), moved, jnp.zeros_like(moved))
                kx[u][pl.ds(_aligned((t - NT[0] + AHEAD + zero) * 8, 8), 8), :] = moved

    def stage_vpu_keys(h, u, d, chunks, after, zero=0):
        r0, r1 = V0[chunks[0]] // 8, V0[chunks[1]] // 8
        idx = after(jnp.full((8, 128), (h % 8) * DH + d, i32))
        src = kvpu_v[h // 8, pl.ds(r0 * 8, (r1 - r0) * 8), :]
        for r in range(r0, r1):
            kb[u][r + zero, d] = _take(src[(r - r0) * 8:(r - r0 + 1) * 8], idx, axis=1)

    def stage_query(h, u, b, d, after, zero=0):
        q = qt_v[pl.ds(_aligned(h * DH + d // 8 * 8, 8), 8), pl.ds(b * TQ, TQ)]
        idx = after(jnp.full((8, 128), d % 8, i32))
        for n in range(NQ):
            qb[u * NB + b][zero, n, _qslot(n, d)] = _take(q[:, n * 128:(n + 1) * 128], idx, axis=0)
        if d % 8 == 0:
            qw[u * NB + b][zero, pl.ds(d, 8), :] = q

    def stage_values(h, u, zero=0):
        for c in range(NC):
            vw[u][zero, :, pl.ds(c * CK, CK)] = _words(vt_v, c, pl.ds(_aligned(h * (DH // 2), DH // 2), DH // 2))

    DQ, H1 = D // 2, R1 // 2

    def split_rows(i, r, top, bot):
        for j, op in enumerate(_lhs7(top[:, :DQ], top[:, DQ:], bot[:, :DQ], bot[:, DQ:])):
            xn7[i, j, pl.ds(r, 16), :] = op

    def ln1(r0, r1, results=(), span=(0, 100), plain=False):
        pieces = [(i, r) for i in range(r0 // R1, r1 // R1) for r in range(0, H1, 16)]
        for (i, r), src in zip(pieces, spread(results, len(pieces), span)):
            halves = []
            for half in range(2):
                rows = pl.ds(i * R1 + half * H1 + r, 16)
                x = x_v[rows, :].astype(f32)
                halves.append(_ln(jnp.concatenate([tie(x[:, 0:128], src), x[:, 128:]], axis=1)))
                if plain:
                    xn_v[rows, :] = halves[-1]
            if not plain:
                split_rows(i, r, *halves)

    def split_weights(jobs, results, span=(0, 100), transposed=False):
        peak = jnp.zeros((16, 128), f32)
        pieces = [(src, r0, rows, c0, cols, dst, r, c) for src, r0, rows, c0, cols, dst in jobs
                  for r in range(0, rows // 2, 16) for c in range(0, cols // 2, 128)]
        for (src, r0, rows, c0, cols, dst, r, c), wait_for in zip(pieces, spread(results, len(pieces), span)):
            quad = []
            for i in range(2):
                for j in range(2):
                    w = pltpu.bitcast(src[pl.ds(r0 + r + i * rows // 2, 16), pl.ds(c0 + j * cols // 2 + c, 128)], u32)
                    quad.append(pltpu.bitcast(tie(w, wait_for), bf16).astype(f32))
            for j, op in enumerate(_rhs7(*[quad[n] for n in ((0, 2, 1, 3) if transposed else (0, 1, 2, 3))])):
                dst[j, c // 128, pl.ds(r, 16), :] = op.astype(bf16)
            peak = jnp.maximum(peak, functools.reduce(jnp.maximum, map(jnp.abs, quad)))
        return jnp.maximum(peak[:8], peak[8:])

    def split_weights_twice(src, dst, results, span):
        pieces = [(t, r) for t in range(FQ // 128) for r in range(0, 128, 16)]
        for (t, r), wait_for in zip(pieces, spread(results, len(pieces), span)):
            def block(i, j):
                r0, c0 = (i * 128, j * FQ + t * 128) if src.shape[1] == F else (i * FQ + t * 128, j * 128)
                w = pltpu.bitcast(src[pl.ds(r0 + r, 16), pl.ds(c0, 128)], u32)
                return pltpu.bitcast(tie(w, wait_for if i == j == 0 else None), bf16).astype(f32)
            quad = [[block(i, j) for j in range(4)] for i in range(4)]
            outer = [_rhs7(quad[i][j], quad[i][2 + j], quad[2 + i][j], quad[2 + i][2 + j]) for i in range(2) for j in range(2)]
            for o in range(7):
                for p, op in enumerate(_rhs7(*[x[o] for x in outer])):
                    dst[o * 7 + p, pl.ds(t * 128 + r, 16), :] = op.astype(bf16)

    def project(i, plain, which):
        if plain:
            y = _mm(xn_v[pl.ds(i * R1, R1), :], wqkv_v[:, pl.ds(which * D, D)])
            return y, [y]
        ms = {j: _mm(xn7[i, j], _tiles(wk7, j)) for j in K_ORDER}
        return _whole(*[_join7(ms, n) for n in range(4)]), list(ms.values())

    def project_t(i, w7):
        ms = {j: _mm_nt(_tiles(w7, j), xn7[i, j]) for j in T_ORDER}
        c11, c12, c21, c22 = [_join7(ms, n) for n in range(4)]
        return _whole(c11, c21, c12, c22), list(ms.values())

    def proj_q(r0, r1, plain=False):
        made = []
        for i in range(r0 // R1, r1 // R1):
            if plain:
                q, ms = project(i, plain, 0)
                qt = q.T
            else:
                qt, ms = project_t(i, wq7)
            qt_v[:, pl.ds(i * R1, R1)] = qt * Q_SCALE
            made += ms
        return made

    def proj_k(r0, r1, plain=False):
        made = []
        for i in range(r0 // R1, r1 // R1):
            k, ms = project(i, plain, 1)
            for g in range(D // 128):
                lanes = slice(g * 128, (g + 1) * 128)
                k_v[g, pl.ds(i * R1, R1), :] = k[:, lanes].astype(bf16)
                for c in range(i * R1 // CK, (i + 1) * R1 // CK):
                    r = c * CK - i * R1
                    kvpu_v[g, pl.ds(V0[c], NV[c]), :] = k[r:r + NV[c], lanes]
            made += ms
        return made

    def proj_v(r0, r1):
        made = []
        for i in range(r0 // R1, r1 // R1):
            vt, ms = project_t(i, wv7)
            for n in range(R1 // CK):
                vt_v[i * R1 // CK + n] = vt[:, n * CK:(n + 1) * CK].astype(bf16)
            made += ms
        return made

    def first_keys(part, results):
        c0, c1 = KEY_CUTS[part:part + 2]
        jobs = []
        for u in range(HU - 1):
            jobs += [functools.partial(stage_mxu_keys, u, u, range(T0[c], T0[c + 1])) for c in range(c0, c1)]
            jobs += [functools.partial(stage_vpu_keys, u, u, d, (c0, c1)) for d in range(DH if c1 > c0 else 0)]
        for job, src in zip(jobs, spread(results, len(jobs), KEY_SPANS[part])):
            job(functools.partial(tie, src=src))

    def first_queries(part, results):
        jobs = [(u, b, d) for b in range(*QUERY_CUTS[part:part + 2]) for u in range(HU)
                if u * NB + b < HU * NB - 1 for d in range(DH)]
        for (u, b, d), src in zip(jobs, spread(results, len(jobs), QUERY_SPANS[part])):
            stage_query(u, u, b, d, functools.partial(tie, src=src))

    def phase1():
        cp_x[0].wait()
        ln1(0, XA, plain=True)
        cp_k.wait()
        made = proj_k(0, XA, plain=True)
        split_weights([(wqkv_v, 0, D, D, D, wk7)], made[:-1])
        for i in range(XA // R1):
            for r in range(0, H1, 16):
                split_rows(i, r, *(xn_v[pl.ds(i * R1 + half * H1 + r, 16), :] for half in range(2)))

        cp_q.wait()
        cp_x[1].wait()
        proj_q(0, XA, plain=True)
        ln1(XA, 2 * XA)
        ks = proj_k(XA, 2 * XA)
        wqt_v[...] = wqkv_v[:, pl.ds(0, D)].T
        split_weights([(wqt_v, 0, D, 0, D, wq7)], ks[3:-2], transposed=True)

        cp_v.wait()
        cp_x[2].wait()
        wvt_v[...] = wqkv_v[:, pl.ds(2 * D, D)].T
        qs = proj_q(XA, 2 * XA)
        range_v[2] = split_weights([(wvt_v, 0, D, 0, D, wv7)], qs[3:-3], transposed=True)
        vs = proj_v(0, XA)
        ln1(2 * XA, S, qs + vs, LN1_SPAN)
        ks = proj_k(2 * XA, S)
        qs = proj_q(2 * XA, S)
        first_keys(0, vs + ks)
        first_keys(1, ks[len(ks) // 2:] + qs)
        first_queries(0, vs + ks + qs)

        for cp in cp_w:
            cp.wait()
        vs = proj_v(XA, S)
        split_weights([(wo_v, 0, D, 0, D, wo7), (w1_v, 0, D, F2, F - F2, w17), (w2_v, F2, F - F2, 0, D, w27)],
                      vs, WEIGHT_SPANS[0])
        split_weights_twice(w1_v, w149, vs, WEIGHT_SPANS[1])
        split_weights_twice(w2_v, w249, vs, WEIGHT_SPANS[2])
        first_keys(2, vs)
        first_queries(1, vs)
        for u in range(HU - 1):
            stage_values(u, u)

    def query_weights(*blocks):
        w = [qw[u * NB + b][0] for u, b in blocks]
        return jnp.concatenate(w + [jnp.zeros((128 - DH * len(w), TQ), f32)], axis=0)

    def finish_step(acc, v):
        return acc + _mm(pltpu.bitcast(v, bf16), pc_v[...])

    def last_block(it):
        return pl.ds(_aligned((it * HU + HU - 1) * DH, DH), DH), pl.ds((NB - 1) * TQ, TQ)

    def fast_step(it, carry):
        items = [(u, b, c) for u in range(HU) for b in range(NB) for c in range(NC)]
        tiles, first, ties = [], [], {}
        for u in range(HU):
            for b in range(NB):
                start, n0, outs = len(tiles), len(first), []
                for c in range(NC):
                    first.append(len(tiles))
                    tiles += [(u, b, c, t) for t in range(NT[c])]
                    outs += [(n0 + c, q, r) for q in range(NQ) for r in reversed(range(NV[c] // 8))]
                for o, key in enumerate(outs):
                    ties.setdefault(max(start + o * (len(tiles) - start) // len(outs) + LAG, AHEAD), []).append(key)
        first.append(len(tiles))
        tiles += tiles[:AHEAD]
        head = lambda u: it * HU + u
        later = lambda u: jnp.minimum(it + 1, H // HU - 1) * HU + u
        always, also = z_v[...] >= 0.0, z_v[...] <= 0.0
        from_vpu, from_mxu = {}, {}

        def vpu_probs(n, q, r):
            if (n, q, r) not in from_vpu:
                u, b, c = items[n]
                accs = [None, None]
                for d in range(DH):
                    t = kb[u][V0[c] // 8 + r, d] * qb[u * NB + b][0, q, _qslot(q, d)]
                    accs[d % 2] = t if accs[d % 2] is None else accs[d % 2] + t
                from_vpu[n, q, r] = jnp.exp2(accs[0] + accs[1])
            return from_vpu[n, q, r]

        def key_tile(g, moved=False):
            u, b, c, t = tiles[g]
            kt = kx[u][pl.ds((AHEAD - 1 - t) * 8, 8), :] if moved else km[u][pl.ds((T0[c + 1] - 1 - t) * 8, 8), :]
            for key, true in zip(ties.get(g, ()), (always, also)):
                kt = jnp.where(true, kt, pltpu.bitcast(vpu_probs(*key), u32))
            return kt

        def mxu_scores(g0, g1):
            if tiles[g0][:2] != tiles[g1 - 1][:2]:
                lhs = [jnp.where(lane < DH, key_tile(g), 0) for g in range(g0, g1 - AHEAD)]
                lhs += [key_tile(g, True) for g in range(g1 - AHEAD, g1)]
                w = query_weights(tiles[g0][:2], tiles[g1 - 1][:2])
            else:
                lhs = [key_tile(g) for g in range(g0, g1)]
                w = query_weights(tiles[g0][:2])
            s = _mm(pltpu.bitcast(jnp.concatenate(lhs, axis=0), bf16), w)
            for g in range(g0, g1):
                from_mxu[g] = s[(g - g0) * 16:(g - g0 + 1) * 16]

        def probs(n, l):
            c = items[n][2]
            scores = [from_mxu.pop(first[n + 1] - 1 - t) for t in range(NT[c])]
            rows = [jnp.concatenate([vpu_probs(n, q, r) for q in range(NQ)], axis=1) for r in range(NV[c] // 8)]
            p = jnp.concatenate(rows + [jnp.exp2(jnp.concatenate(scores, axis=0))], axis=0)
            for r in reversed(range(CK // 8)):
                row = p[r * 8:(r + 1) * 8]
                l = row if l is None else l + row
            return p, l

        for g in range(AHEAD):
            from_mxu[g] = s0_v[pl.ds(g * 16, 16), :]
        l = acc = None
        for m in range(len(items) + 1):
            if m < len(items):
                mxu_scores(first[m] + AHEAD, first[m + 1] + AHEAD)
            if m == 0:
                ot_v[last_block(jnp.maximum(it - 1, 0))] = finish_step(*carry)
                continue
            u, b, c = items[m - 1]
            if c == 0:
                l, acc = None, jnp.tile(z_v[...], (DH // 8, NQ))
            p, l = probs(m - 1, l)
            v = vw[u][0, :, pl.ds(c * CK, CK)]
            if m < len(items):
                acc = acc + _mm(pltpu.bitcast(v, bf16), p)
            else:
                late = jnp.tile(p[NV[c]:NV[c] + 8], (NV[c] // 8, 1))
                keep = jnp.tile(z_v[...], (NV[c] // 8, NQ)) >= 0.0
                pc_v[pl.ds(NV[c], CK - NV[c]), :] = p[NV[c]:]
                pc_v[pl.ds(0, NV[c]), :] = jnp.where(keep, p[:NV[c]], late)

            after = functools.partial(lambda x, src: jnp.where(always, x, pltpu.bitcast(src, i32)), src=l[:, 0:128])
            midway = functools.partial(after, src=p[MID * 8:MID * 8 + 8, 0:128])
            target = (later(u - 1), u - 1) if u else (head(HU - 1), HU - 1)
            zero = 0 if u else jnp.minimum(it, 0)
            (v0, vn), (m0, mn) = (LAST_VPU_REFILL, LAST_MXU_REFILL) if u == HU - 1 else (VPU_REFILL, MXU_REFILL)
            for d in range(DH):
                if v0 + d * vn // DH == b * NC + c:
                    stage_vpu_keys(*target, d, (0, NC), after, zero)
            for part in range(NC):
                if m0 + part * mn // NC == b * NC + c:
                    stage_mxu_keys(*target, range(part * T0[NC] // NC, (part + 1) * T0[NC] // NC), midway, zero)
            if v0 == b * NC + c:
                stage_values(*target, zero)
            if u or b:
                u1, b1 = divmod(u * NB + b - 1, NB)
                stage_query(later(u1), u1, b1, c, after)
            else:
                stage_query(head(HU - 1), HU - 1, NB - 1, c, after, jnp.minimum(it, 0))
            if c == NC - 1:
                l_v[head(u), :, pl.ds(b * TQ, TQ)] = l
                parts = [l[:, n * 128:(n + 1) * 128] for n in range(NQ)]
                range_v[0] = functools.reduce(jnp.minimum, parts, range_v[0])
                range_v[1] = functools.reduce(jnp.maximum, parts, range_v[1])
                if m < len(items):
                    ot_v[pl.ds(_aligned(head(u) * DH, DH), DH), pl.ds(b * TQ, TQ)] = acc
        for g in range(AHEAD):
            s0_v[pl.ds(g * 16, 16), :] = from_mxu.pop(first[-1] + g)
        return acc, v

    def exact_step(i, carry):
        h, b = i // (S // TS), i % (S // TS)
        cols = pl.ds(_aligned(b * TS, TS), TS)
        q = qt_v[pl.ds(_aligned(h * DH, DH), DH), cols]
        row_head = jax.lax.broadcasted_iota(i32, (128, TS), 0) // DH
        s = _mm(k_v[h // 8], jnp.where(row_head == h % 8, jnp.tile(q, (8, 1)), 0.0))
        p = jnp.exp2(s - jnp.max(s, axis=0, keepdims=True))
        v = jnp.concatenate([vt_v[c, pl.ds(_aligned(h * DH, DH), DH), :] for c in range(NC)], axis=1)
        ot_v[pl.ds(_aligned(h * DH, DH), DH), cols] = _mm(v, p)
        l_v[h, :, cols] = jnp.sum(p.reshape(S // 8, 8, TS), axis=0)
        return carry

    def fast_attention():
        range_v[0] = jnp.ones((8, 128), f32)
        range_v[1] = jnp.ones((8, 128), f32)
        lead = [_words(k_v, 0, pl.ds(NV[0] // 2 + (NT[0] - 1 - t) * 8, 8)) for t in range(AHEAD)]
        s0_v[...] = _mm(pltpu.bitcast(jnp.concatenate(lead, axis=0), bf16), query_weights((0, 0)))
        pc_v[...] = jnp.zeros((CK, TQ), f32)
        ot_v[last_block(H // HU - 1)] = jnp.zeros((DH, TQ), f32)
        return jax.lax.fori_loop(0, H // HU, fast_step, (jnp.zeros((DH, TQ), f32), jnp.zeros((DH // 2, CK), u32)))

    def check_attention(carry):
        safe = (range_v[0] >= L_MIN) & (range_v[1] <= L_MAX) & (range_v[2] <= W_MAX)
        redo = jnp.max(jnp.where(safe, 0.0, 1.0)) > 0.0

        @pl.when(redo)
        def _():
            jax.lax.fori_loop(0, H * (S // TS), exact_step, 0)

        last = last_block(H // HU - 1)
        ot_v[last] = jnp.where(redo, ot_v[last], finish_step(*carry))

    RH, RQ = R3 // 2, R3 // 4

    def out_copy(n):
        rows = pl.ds(n * RH, RH)
        return pltpu.make_async_copy(out_v.at[rows], out_hbm.at[rows], out_sem.at[n])

    def normalize(i, h, src):
        rows = pl.ds(i * R3, R3)
        lsum = jnp.sum(tie(l_v[h, :, rows], src), axis=0, keepdims=True)
        inv = pl.reciprocal(lsum, approx=True)
        return ot_v[pl.ds(h * DH, DH), rows] * (inv * (2.0 - lsum * inv))

    def ln2(i, n, src):
        step = RQ // LN2_PIECES
        out = []
        for r in range(4):
            hid = h_v[pl.ds(i * R3 + r * RQ + n * step, step), :]
            out.append(_ln(jnp.concatenate([tie(hid[:, 0:128], src), hid[:, 128:]], axis=1)))
        return out

    def blocks(x):
        return [[x[r * RQ:(r + 1) * RQ, c * 128:(c + 1) * 128] for c in range(4)] for r in range(4)]

    def outer_lhs(a, o):
        return [_lhs7(a[i][j], a[i][2 + j], a[2 + i][j], a[2 + i][2 + j])[o] for i in range(2) for j in range(2)]

    def inner(ops, w49, o, rows, order):
        ms = {p: _mm(ops[p], pltpu.bitcast(_words(w49, o * 7 + p, rows), bf16)) for p in order}
        return [_join7(ms, n) for n in range(4)], list(ms.values())

    def phase3(steps):
        b1 = b1_v[...].astype(f32).reshape(1, F)
        b2 = b2_v[...].astype(f32).reshape(1, D)
        att = hn = act = act_rest = src = None
        for i in range(-2, steps + 1):
            def plan(kind, args, span):
                return [(span[0] + (n + 0.5) / len(args) * (span[1] - span[0]), kind, arg) for n, arg in enumerate(args)]

            jobs = []
            if 0 <= i < steps:
                jobs += plan("up", [(o, t) for o in UP_ORDER for t in range(FQ // 128)], (0, 100))
                jobs += plan("rest", REST_ORDER, REST_SPAN)
                outer_ops = [outer_lhs(hn, o) for o in range(7)]
                inner_ops = [_lhs7(*x) for x in outer_ops]
            if i > 0:
                jobs += plan("down", DOWN_ORDER, DOWN_SPAN)
            if 0 <= i + 1 < steps:
                jobs += plan("proj", PROJ_ORDER, PROJ_SPAN) + plan("ln", range(LN2_PIECES), LN2_SPAN)
            if i + 2 < steps:
                jobs += plan("norm", range(H), NORM_SPAN if i >= 0 else (100, 200))
            ups, rests, downs, projs = [{} for _ in range(FQ // 128)], {}, {}, {}
            lns, heads, done = [], [], []
            new_act, new_rest = [[[None] * (FQ // 128) for _ in range(4)] for _ in range(4)], [None] * 4
            for _, kind, arg in sorted(jobs, key=lambda job: job[0]):
                if kind == "up":
                    o, t = arg
                    ups[t][o], ms = inner(inner_ops[o], w149, o, pl.ds(t * 64, 64), UP_INNER)
                    for m in _completed(ups[t], o):
                        for n in range(4):
                            r, c = m // 2 * 2 + n // 2, m % 2 * 2 + n % 2
                            y = _join7({j: x[n] for j, x in ups[t].items()}, m)
                            new_act[r][c][t] = _gelu(y + b1[:, c * FQ + t * 128:c * FQ + (t + 1) * 128])
                elif kind == "rest":
                    rests[arg] = _mm(_whole(*outer_ops[arg]), _tiles(w17, arg))
                    ms = [rests[arg]]
                    for m in _completed(rests, arg):
                        new_rest[m] = _gelu(_join7(rests, m) + b1[:, F2 + m % 2 * 128:F2 + (m % 2 + 1) * 128])
                elif kind == "down":
                    ops = _lhs7(*outer_lhs(act, arg))
                    y = _mm(_lhs7(*act_rest)[arg], _tiles(w27, arg))
                    out, ms = inner(ops, w249, arg, slice(None), DOWN_INNER)
                    downs[arg] = [x + y[n // 2 * RQ:(n // 2 + 1) * RQ, n % 2 * 128:(n % 2 + 1) * 128] for n, x in enumerate(out)]
                    for m in _completed(downs, arg):
                        for n in range(4):
                            r, c = m // 2 * 2 + n // 2, m % 2 * 2 + n % 2
                            q = (pl.ds((i - 1) * R3 + r * RQ, RQ), pl.ds(c * 128, 128))
                            y = _join7({j: x[n] for j, x in downs.items()}, m)
                            out_v[q] = (h_v[q] + y + b2[:, c * 128:(c + 1) * 128]).astype(out_v.dtype)
                        done.append(m)
                        if m ^ 1 in done:
                            out_copy(2 * (i - 1) + m // 2).start()
                elif kind == "proj":
                    projs[arg] = _mm(_whole(*outer_lhs(att, arg)).astype(bf16), _tiles(wo7, arg))
                    ms = [projs[arg]]
                    for m in _completed(projs, arg):
                        q = (pl.ds((i + 1) * R3 + m // 2 * RH, RH), pl.ds(m % 2 * DQ, DQ))
                        h_v[q] = x_v[q].astype(f32) + _join7(projs, m)
                elif kind == "ln":
                    lns.append(ln2(i + 1, arg, src))
                    continue
                else:
                    heads.append(normalize(i + 2, arg, src))
                    continue
                src = ms[3 % len(ms)] if i >= 0 else None
            if 0 <= i < steps:
                act, act_rest = [[jnp.concatenate(x, axis=1) for x in row] for row in new_act], new_rest
            if lns:
                hn = blocks(jnp.concatenate([x[r] for r in range(4) for x in lns], axis=0))
            if heads:
                att = blocks(jnp.concatenate(heads, axis=0).T)

    phase1()
    check_attention(fast_attention())
    phase3(S // R3)
    for n in range(S // RH):
        out_copy(n).wait()


@jax.jit
def pallas_sequential_preLN__softmax_full_mha__dense_activation_gelu__prompt_kernel(
        A_x, A_wqkv, A_wo, B_x, B_w1, B_b1, B_w2, B_b2):
    del B_x
    any_spec = pl.BlockSpec(memory_space=pl.ANY)
    vm = pltpu.VMEM
    out = pl.pallas_call(
        _kernel,
        out_shape=jax.ShapeDtypeStruct((S, D), A_x.dtype),
        in_specs=[any_spec] * 7,
        out_specs=any_spec,
        scratch_shapes=[
            vm((S, D), bf16), vm((D, 3 * D), bf16), vm((D, D), bf16), vm((D, F), bf16), vm((F, D), bf16),
            *[vm((7, 2, D // 2, 128), bf16)] * 3, vm((D, D), bf16), vm((D, D), bf16),
            vm((XA, D), f32), vm((S // R1, 7, R1 // 2, D // 2), f32),
            vm((D // 128, S, 128), bf16), vm((D // 128, V0[NC], 128), f32),
            vm((D, S), f32), vm((NC, D, CK), bf16), vm((D, S), f32), vm((H, 8, S), f32),
            vm((AHEAD * 16, TQ), f32), vm((CK, TQ), f32), vm((8, 128), f32), vm((3, 8, 128), f32),
            vm((7, 2, D // 2, 128), bf16), vm((7, 1, D // 2, 128), bf16), vm((7, 2, (F - F2) // 2, 128), bf16),
            vm((49, FQ, 128), bf16), vm((49, FQ, 128), bf16), vm((S, D), f32), vm((S, D), bf16),
            pltpu.SemaphoreType.DMA((11,)), pltpu.SemaphoreType.DMA((2 * S // R3,)),
            *[vm((T0[NC] * 8, 128), u32)] * HU, *[vm((AHEAD * 8, 128), u32)] * HU,
            *[vm((V0[NC] // 8, DH, 8, 128), f32)] * HU, *[vm((1, DH // 2, S), u32)] * HU,
            *[vm((1, DH, TQ), f32)] * (HU * NB), *[vm((1, NQ, DH, 8, 128), f32)] * (HU * NB),
            vm((F,), bf16), vm((D,), bf16),
        ],
        compiler_params=pltpu.CompilerParams(vmem_limit_bytes=100 * 1024 * 1024),
    )(A_x.reshape(S, D), A_wqkv, A_wo, B_w1, B_b1, B_w2, B_b2)
    return out.reshape(A_x.shape)
```

```python
import functools

import jax
import jax.numpy as jnp
import numpy as np
import jax.experimental.pallas as pl
import jax.experimental.pallas.tpu as pltpu

S, D, F, H, DH = 2048, 512, 1792, 32, 16
EPS = 1e-5
bf16, f32, u32, i32 = jnp.bfloat16, jnp.float32, jnp.uint32, jnp.int32
Q_SCALE = float(DH ** -0.5 * np.log2(np.e))
L_MIN, L_MAX, W_MAX = 2.0 ** -60, 2.0 ** 100, 2.0 ** 14


def _order(digits):
    return [int(ch) - 1 for ch in str(digits)]


R1 = 256
XA = 512
K_ORDER, T_ORDER = _order(4235167), _order(4235167)
LN1_SPAN = (10, 75)
KEY_CUTS = (0, 6, 14, 16)
KEY_SPANS = ((20, 92), (10, 88), (5, 70))
QUERY_CUTS = (0, 1, 4)
QUERY_SPANS = ((60, 80), (20, 90))
WEIGHT_SPANS = ((50, 88), (5, 45), (45, 84))

TQ = 512
NQ, NB = TQ // 128, S // TQ
CK = 128
NC = S // CK
HU = 4
NV = [(16, 16, 32, 16)[c % 4] for c in range(NC)]
NT = [(CK - v) // 16 for v in NV]
V0 = [sum(NV[:c]) for c in range(NC + 1)]
T0 = [sum(NT[:c]) for c in range(NC + 1)]
AHEAD = 2
LAG = 8
VPU_REFILL, LAST_VPU_REFILL = (2, 32), (4, 56)
MXU_REFILL, LAST_MXU_REFILL = (35, 16), (4, 16)
MID = 9
TS = 128

R3 = 256
FQ = 384
F2 = 4 * FQ
UP_ORDER, REST_ORDER = _order(4235167), _order(2435167)
DOWN_ORDER, PROJ_ORDER = _order(4271356), _order(3524167)
FIRST_PROJ_ORDER = _order(4273516)
UP_INNER, DOWN_INNER = _order(2413576), _order(2413567)
REST_SPAN, DOWN_SPAN, PROJ_SPAN = (45, 105), (8, 102), (2, 7)
LN2_SPAN, NORM_SPAN = (50, 95), (50, 100)
LN2_PIECES = 8


def _aligned(x, n):
    return x if isinstance(x, int) else pl.multiple_of(x, n)


def _mm(a, b):
    return jax.lax.dot_general(a, b, (((1,), (0,)), ((), ())), preferred_element_type=f32)


def _mm_nt(a, b):
    return jax.lax.dot_general(a, b, (((1,), (1,)), ((), ())), preferred_element_type=f32)


def _take(x, idx, axis):
    return jnp.take_along_axis(x, idx, axis=axis, mode="promise_in_bounds", wrap_negative_indices=False)


def _halves(ref, *idx):
    return ref[idx] if ref.dtype == bf16 else pltpu.bitcast(ref[idx], bf16)


def _put(ref, idx, r0, x):
    if ref.dtype == bf16:
        ref[(*idx, pl.ds(r0, x.shape[0]))] = x.astype(bf16)
    else:
        ref[(*idx, pl.ds(r0 // 2, x.shape[0] // 2))] = pltpu.bitcast(x.astype(bf16), u32)


def _tiles(ref, *idx):
    return jnp.concatenate([_halves(ref, *idx, c) for c in range(ref.shape[len(idx)])], axis=1)


def _whole(c11, c12, c21, c22):
    return jnp.concatenate([jnp.concatenate([c11, c12], axis=1), jnp.concatenate([c21, c22], axis=1)], axis=0)


def _lhs7(a11, a12, a21, a22):
    return (a11 + a22, a21 + a22, a11, a22, a11 + a12, a21 - a11, a12 - a22)


def _rhs7(b11, b12, b21, b22):
    return (b11 + b22, b11, b12 - b22, b21 - b11, b22, b11 + b12, b21 + b22)


_TERMS = (((0, 3, 6), (4,)), ((2, 4), ()), ((1, 3), ()), ((0, 2, 5), (1,)))


def _join7(ms, quadrant):
    plus, minus = _TERMS[quadrant]
    terms = [j for j in ms if j in plus + minus]
    if terms[0] in minus:
        terms[:2] = terms[1::-1]
    acc = ms[terms[0]]
    for j in terms[1:]:
        acc = acc - ms[j] if j in minus else acc + ms[j]
    return acc


def _completed(ms, j):
    return [n for n, (plus, minus) in enumerate(_TERMS) if j in plus + minus and all(i in ms for i in plus + minus)]


def _ln(x):
    m = jnp.mean(x, axis=-1, keepdims=True)
    xc = x - m
    v = jnp.mean(xc * xc, axis=-1, keepdims=True)
    return xc * jax.lax.rsqrt(v + EPS)


def _gelu(x):
    c = float(np.sqrt(2.0 / np.pi))
    return (0.5 * x) * (1.0 + jnp.tanh(x * (c + (c * 0.044715) * (x * x))))


def _kernel(x_hbm, wqkv_hbm, wo_hbm, w1_hbm, b1_hbm, w2_hbm, b2_hbm, out_hbm,
            x_v, wqkv_v, wo_v, w1_v, w2_v, wq7, wk7, wv7, wvt_v, wqt_v, xn_v,
            k_v, kvpu_v, qt_v, vt_v, ot_v, l_v, s0_v, pc_v, z_v, range_v,
            wo7, w17, w27, w149, w249, h_v, out_v, in_sem, out_sem, *slots):
    km, kx, kb, vw = (slots[i * HU:(i + 1) * HU] for i in range(4))
    qw, qb = (slots[4 * HU + i * HU * NB:4 * HU + (i + 1) * HU * NB] for i in range(2))
    b1_v, b2_v = slots[-2:]

    def fetch(src, dst, i, rows=slice(None), cols=slice(None)):
        return pltpu.make_async_copy(src.at[rows, cols], dst.at[rows, cols], in_sem.at[i])

    groups = [
        [fetch(x_hbm, x_v, 0, rows=pl.ds(0, R1))],
        [fetch(wqkv_hbm, wqkv_v, 1, cols=pl.ds(D, D // 2))],
        [fetch(wqkv_hbm, wqkv_v, 2, cols=pl.ds(D + D // 2, D // 2))],
        [fetch(x_hbm, x_v, 3, rows=pl.ds(R1, XA - R1))],
        [fetch(wqkv_hbm, wqkv_v, 4, cols=pl.ds(0, D // 2))],
        [fetch(wqkv_hbm, wqkv_v, 5, cols=pl.ds(D // 2, D // 2)), fetch(x_hbm, x_v, 5, rows=pl.ds(XA, XA))],
        [fetch(wqkv_hbm, wqkv_v, 6, cols=pl.ds(2 * D, D)), fetch(x_hbm, x_v, 6, rows=pl.ds(2 * XA, S - 2 * XA))],
        [fetch(wo_hbm, wo_v, 7), fetch(w1_hbm, w1_v, 7), fetch(w2_hbm, w2_v, 7),
         pltpu.make_async_copy(b1_hbm, b1_v, in_sem.at[7]), pltpu.make_async_copy(b2_hbm, b2_v, in_sem.at[7])],
    ]
    for group in groups:
        for cp in group:
            cp.start()

    def arrived(n):
        for cp in groups[n]:
            cp.wait()

    lane = jax.lax.broadcasted_iota(i32, (8, 128), 1)
    z_v[...] = jnp.zeros((8, 128), f32)

    def tie(x, src):
        if src is None:
            return x
        reps = (x.shape[0] // 8, x.shape[1] // 128)
        src = src[0:8, 0:128]
        src = src if x.dtype == src.dtype else pltpu.bitcast(src, x.dtype)
        return jnp.where(jnp.tile(z_v[...], reps) >= 0.0, x, jnp.tile(src, reps))

    def spread(results, n, span=(0, 100)):
        results = results[len(results) * span[0] // 100:len(results) * span[1] // 100]
        if not results:
            return [None] * n
        tiles = [(y, r, c) for y in results for c in range(0, y.shape[1], 128) for r in range(0, y.shape[0], 8)]
        picks = [tiles[i * len(tiles) // n] for i in range(n)]
        return [y[r:r + 8, c:c + 128] for y, r, c in picks]

    def stage_mxu_keys(h, u, tiles, after, zero=0):
        idx = after((lane + (h & 7) * DH) & 127)
        for g in tiles:
            c = max(c for c in range(NC) if T0[c] <= g)
            t = g - T0[c]
            words = k_v[h >> 3, pl.ds((c * CK + NV[c]) // 2 + t * 8, 8)]
            km[u][pl.ds(_aligned((g + zero) * 8, 8), 8), :] = _take(words, idx, axis=1)
            if c == 0 and t >= NT[0] - AHEAD:
                moved = _take(words, (idx + (128 - DH)) & 127, axis=1)
                moved = jnp.where((lane >= DH) & (lane < 2 * DH), moved, jnp.zeros_like(moved))
                kx[u][pl.ds(_aligned((t - NT[0] + AHEAD + zero) * 8, 8), 8), :] = moved

    def stage_vpu_keys(h, u, d, chunks, after, zero=0):
        r0, r1 = V0[chunks[0]] // 8, V0[chunks[1]] // 8
        idx = after(jnp.full((8, 128), (h & 7) * DH + d, i32))
        src = kvpu_v[h >> 3, pl.ds(r0 * 8, (r1 - r0) * 8), :]
        wide = _take(src, jnp.tile(idx, (r1 - r0, 1)), axis=1)
        kb[u][pl.ds(r0 + zero, r1 - r0), pl.ds(d * 8, 8), :] = wide.reshape(r1 - r0, 8, 128)

    def stage_query(h, u, b, d, after, zero=0):
        q = qt_v[pl.ds(_aligned(h * DH + d // 8 * 8, 8), 8), pl.ds(b * TQ, TQ)]
        idx = after(jnp.full((8, 128), d % 8, i32))
        for n in range(NQ):
            qb[u * NB + b][zero, n, pl.ds((d + 1) * 8, 8), :] = _take(q[:, n * 128:(n + 1) * 128], idx, axis=0)
        if d % 8 == 0:
            qw[u * NB + b][zero, pl.ds(d, 8), :] = q

    def stage_values(h, u, zero=0):
        for c in range(NC):
            vw[u][zero, :, pl.ds(c * CK, CK)] = pltpu.bitcast(vt_v[c, pl.ds(_aligned(h * DH, DH), DH)], u32)

    DQ, H1 = D // 2, R1 // 2

    def ln1(r0, r1, results=(), span=(0, 100)):
        pieces = [i + r for i in range(r0, r1, R1) for r in range(0, H1, 16)]
        for r, src in zip(pieces, spread(results, len(pieces), span)):
            for half in range(2):
                rows = pl.ds(r + half * H1, 16)
                x = x_v[rows, :].astype(f32)
                xn_v[rows, :] = _ln(jnp.concatenate([tie(x[:, 0:128], src), x[:, 128:]], axis=1))

    def split_rows(i):
        return _lhs7(*[xn_v[pl.ds(i * R1 + n // 2 * H1, H1), pl.ds(n % 2 * DQ, DQ)] for n in range(4)])

    def split_weights(jobs, results, span=(0, 100), transposed=False):
        peak = jnp.zeros((16, 128), f32)
        pieces = [(src, r0, rows, c0, cols, dst, r, c) for src, r0, rows, c0, cols, dst in jobs
                  for r in range(0, rows // 2, 16) for c in range(0, cols // 2, 128)]
        for (src, r0, rows, c0, cols, dst, r, c), wait_for in zip(pieces, spread(results, len(pieces), span)):
            quad = []
            for i in range(2):
                for j in range(2):
                    w = pltpu.bitcast(src[pl.ds(r0 + r + i * rows // 2, 16), pl.ds(c0 + j * cols // 2 + c, 128)], u32)
                    quad.append(pltpu.bitcast(tie(w, wait_for), bf16).astype(f32))
            for j, op in enumerate(_rhs7(*[quad[n] for n in ((0, 2, 1, 3) if transposed else (0, 1, 2, 3))])):
                _put(dst, (j, c // 128), r, op)
            peak = jnp.maximum(peak, functools.reduce(jnp.maximum, map(jnp.abs, quad)))
        return jnp.maximum(peak[:8], peak[8:])

    def split_weights_twice(src, dst, results, span):
        pieces = [(t, r) for t in range(FQ // 128) for r in range(0, 128, 16)]
        for (t, r), wait_for in zip(pieces, spread(results, len(pieces), span)):
            def block(i, j):
                r0, c0 = (i * 128, j * FQ + t * 128) if src.shape[1] == F else (i * FQ + t * 128, j * 128)
                w = pltpu.bitcast(src[pl.ds(r0 + r, 16), pl.ds(c0, 128)], u32)
                return pltpu.bitcast(tie(w, wait_for if i == j == 0 else None), bf16).astype(f32)
            quad = [[block(i, j) for j in range(4)] for i in range(4)]
            outer = [_rhs7(quad[i][j], quad[i][2 + j], quad[2 + i][j], quad[2 + i][2 + j]) for i in range(2) for j in range(2)]
            for o in range(7):
                for p, op in enumerate(_rhs7(*[x[o] for x in outer])):
                    _put(dst, (o * 7 + p,), t * 128 + r, op)

    def project_t(i, w7):
        ops = split_rows(i)
        ms = {j: _mm_nt(_tiles(w7, j), ops[j]) for j in T_ORDER}
        c11, c12, c21, c22 = [_join7(ms, n) for n in range(4)]
        return _whole(c11, c21, c12, c22), list(ms.values())

    def proj_q(r0, r1):
        made = []
        for i in range(r0 // R1, r1 // R1):
            qt, ms = project_t(i, wq7)
            qt_v[:, pl.ds(i * R1, R1)] = qt * Q_SCALE
            made += ms
        return made

    def store_keys(i, g0, k):
        for g in range(k.shape[1] // 128):
            lanes = slice(g * 128, (g + 1) * 128)
            _put(k_v, (g0 + g,), i * R1, k[:, lanes])
            for c in range(i * R1 // CK, (i + 1) * R1 // CK):
                r = c * CK - i * R1
                kvpu_v[g0 + g, pl.ds(V0[c], NV[c]), :] = k[r:r + NV[c], lanes]

    def proj_k(r0, r1):
        made = []
        for i in range(r0 // R1, r1 // R1):
            ops = split_rows(i)
            ms = {j: _mm(ops[j], _tiles(wk7, j)) for j in K_ORDER}
            store_keys(i, 0, _whole(*[_join7(ms, n) for n in range(4)]))
            made += ms.values()
        return made

    def plain_k(i, n):
        k = _mm(xn_v[pl.ds(i * R1, R1), :], wqkv_v[:, pl.ds(D + n * DQ, DQ)])
        store_keys(i, n * DQ // 128, k)

    def plain_q(i, n):
        q = _mm(xn_v[pl.ds(i * R1, R1), :], wqkv_v[:, pl.ds(n * DQ, DQ)])
        qt_v[pl.ds(n * DQ, DQ), pl.ds(i * R1, R1)] = q.T * Q_SCALE

    def proj_v(r0, r1):
        made = []
        for i in range(r0 // R1, r1 // R1):
            vt, ms = project_t(i, wv7)
            for n in range(R1 // CK):
                vt_v[i * R1 // CK + n] = vt[:, n * CK:(n + 1) * CK].astype(bf16)
            made += ms
        return made

    def first_keys(part, results):
        c0, c1 = KEY_CUTS[part:part + 2]
        jobs = []
        for u in range(HU - 1):
            jobs += [functools.partial(stage_mxu_keys, u, u, range(T0[c], T0[c + 1])) for c in range(c0, c1)]
            jobs += [functools.partial(stage_vpu_keys, u, u, d, (c0, c1)) for d in range(DH if c1 > c0 else 0)]
        for job, src in zip(jobs, spread(results, len(jobs), KEY_SPANS[part])):
            job(functools.partial(tie, src=src))

    def first_queries(part, results):
        jobs = [(u, b, d) for b in range(*QUERY_CUTS[part:part + 2]) for u in range(HU)
                if u * NB + b < HU * NB - 1 for d in range(DH)]
        for (u, b, d), src in zip(jobs, spread(results, len(jobs), QUERY_SPANS[part])):
            stage_query(u, u, b, d, functools.partial(tie, src=src))

    def phase1():
        arrived(0)
        ln1(0, R1)
        arrived(1)
        plain_k(0, 0)
        arrived(2)
        plain_k(0, 1)
        arrived(3)
        ln1(R1, XA)
        arrived(4)
        split_weights([(wqkv_v, 0, D, D, D, wk7)], ())
        plain_q(0, 0)
        plain_q(1, 0)
        proj_k(R1, XA)

        arrived(5)
        plain_q(0, 1)
        plain_q(1, 1)
        ln1(XA, 2 * XA)
        ks = proj_k(XA, 2 * XA)
        wqt_v[...] = wqkv_v[:, pl.ds(0, D)].T
        split_weights([(wqt_v, 0, D, 0, D, wq7)], ks[3:-4], transposed=True)
        proj_q(XA, XA + R1)

        arrived(6)
        wvt_v[...] = wqkv_v[:, pl.ds(2 * D, D)].T
        qs = proj_q(XA + R1, 2 * XA)
        range_v[2] = split_weights([(wvt_v, 0, D, 0, D, wv7)], qs[3:-3], transposed=True)
        vs = proj_v(0, XA)
        ln1(2 * XA, S, qs + vs, LN1_SPAN)
        ks = proj_k(2 * XA, S)
        qs = proj_q(2 * XA, S)
        first_keys(0, vs + ks)
        first_keys(1, ks[len(ks) // 2:] + qs)
        first_queries(0, vs + ks + qs)

        arrived(7)
        vs = proj_v(XA, S)
        split_weights([(wo_v, 0, D, 0, D, wo7), (w1_v, 0, D, F2, F - F2, w17), (w2_v, F2, F - F2, 0, D, w27)],
                      vs, WEIGHT_SPANS[0])
        split_weights_twice(w1_v, w149, vs, WEIGHT_SPANS[1])
        split_weights_twice(w2_v, w249, vs, WEIGHT_SPANS[2])
        first_keys(2, vs)
        first_queries(1, vs)
        for u in range(HU - 1):
            stage_values(u, u)

    def query_weights(*blocks):
        w = [qw[u * NB + b][0] for u, b in blocks]
        return jnp.concatenate(w + [jnp.zeros((128 - DH * len(w), TQ), f32)], axis=0)

    def finish_step(acc, v):
        return acc + _mm(pltpu.bitcast(v, bf16), pc_v[...])

    def last_block(it):
        return pl.ds(_aligned((it * HU + HU - 1) * DH, DH), DH), pl.ds((NB - 1) * TQ, TQ)

    def fast_step(it, carry):
        items = [(u, b, c) for u in range(HU) for b in range(NB) for c in range(NC)]
        tiles, first, ties = [], [], {}
        for u in range(HU):
            for b in range(NB):
                start, n0, outs = len(tiles), len(first), []
                for c in range(NC):
                    first.append(len(tiles))
                    tiles += [(u, b, c, t) for t in range(NT[c])]
                    outs += [(n0 + c, q, r) for q in range(NQ) for r in reversed(range(NV[c] // 8))]
                for o, key in enumerate(outs):
                    ties.setdefault(max(start + o * (len(tiles) - start) // len(outs) + LAG, AHEAD), []).append(key)
        first.append(len(tiles))
        tiles += tiles[:AHEAD]
        head = lambda u: it * HU + u
        later = lambda u: jnp.minimum(it + 1, H // HU - 1) * HU + u
        always, also = z_v[...] >= 0.0, z_v[...] <= 0.0
        from_vpu, from_mxu = {}, {}

        def vpu_probs(n, q, r):
            if (n, q, r) not in from_vpu:
                u, b, c = items[n]
                accs = [None, None]
                for d in range(DH):
                    t = kb[u][V0[c] // 8 + r, pl.ds(d * 8, 8), :] * qb[u * NB + b][0, q, pl.ds((d + 1) * 8, 8), :]
                    accs[d % 2] = t if accs[d % 2] is None else accs[d % 2] + t
                from_vpu[n, q, r] = jnp.exp2(accs[0] + accs[1])
            return from_vpu[n, q, r]

        def key_tile(g, moved=False):
            u, b, c, t = tiles[g]
            kt = kx[u][pl.ds((AHEAD - 1 - t) * 8, 8), :] if moved else km[u][pl.ds((T0[c + 1] - 1 - t) * 8, 8), :]
            for key, true in zip(ties.get(g, ()), (always, also)):
                kt = jnp.where(true, kt, pltpu.bitcast(vpu_probs(*key), u32))
            return kt

        def mxu_scores(g0, g1):
            if tiles[g0][:2] != tiles[g1 - 1][:2]:
                lhs = [jnp.where(lane < DH, key_tile(g), 0) for g in range(g0, g1 - AHEAD)]
                lhs += [key_tile(g, True) for g in range(g1 - AHEAD, g1)]
                w = query_weights(tiles[g0][:2], tiles[g1 - 1][:2])
            else:
                lhs = [key_tile(g) for g in range(g0, g1)]
                w = query_weights(tiles[g0][:2])
            s = _mm(pltpu.bitcast(jnp.concatenate(lhs, axis=0), bf16), w)
            for g in range(g0, g1):
                from_mxu[g] = s[(g - g0) * 16:(g - g0 + 1) * 16]

        def probs(n, l):
            c = items[n][2]
            scores = [from_mxu.pop(first[n + 1] - 1 - t) for t in range(NT[c])]
            rows = [jnp.concatenate([vpu_probs(n, q, r) for q in range(NQ)], axis=1) for r in range(NV[c] // 8)]
            p = jnp.concatenate(rows + [jnp.exp2(jnp.concatenate(scores, axis=0))], axis=0)
            for r in reversed(range(CK // 8)):
                row = p[r * 8:(r + 1) * 8]
                l = row if l is None else l + row
            return p, l

        for g in range(AHEAD):
            from_mxu[g] = s0_v[pl.ds(g * 16, 16), :]
        l = acc = None
        for m in range(len(items) + 1):
            if m < len(items):
                mxu_scores(first[m] + AHEAD, first[m + 1] + AHEAD)
            if m == 0:
                ot_v[last_block(jnp.maximum(it - 1, 0))] = finish_step(*carry)
                continue
            u, b, c = items[m - 1]
            if c == 0:
                l, acc = None, jnp.tile(z_v[...], (DH // 8, NQ))
            p, l = probs(m - 1, l)
            v = vw[u][0, :, pl.ds(c * CK, CK)]
            if m < len(items):
                acc = acc + _mm(pltpu.bitcast(v, bf16), p)
            else:
                late = jnp.tile(p[NV[c]:NV[c] + 8], (NV[c] // 8, 1))
                keep = jnp.tile(z_v[...], (NV[c] // 8, NQ)) >= 0.0
                pc_v[pl.ds(NV[c], CK - NV[c]), :] = p[NV[c]:]
                pc_v[pl.ds(0, NV[c]), :] = jnp.where(keep, p[:NV[c]], late)

            after = functools.partial(lambda x, src: jnp.where(always, x, pltpu.bitcast(src, i32)), src=l[:, 0:128])
            midway = functools.partial(after, src=p[MID * 8:MID * 8 + 8, 0:128])
            target = (later(u - 1), u - 1) if u else (head(HU - 1), HU - 1)
            zero = 0 if u else jnp.minimum(it, 0)
            (v0, vn), (m0, mn) = (LAST_VPU_REFILL, LAST_MXU_REFILL) if u == HU - 1 else (VPU_REFILL, MXU_REFILL)
            for d in range(DH):
                if v0 + d * vn // DH == b * NC + c:
                    stage_vpu_keys(*target, d, (0, NC), after, zero)
            for part in range(NC):
                if m0 + part * mn // NC == b * NC + c:
                    stage_mxu_keys(*target, range(part * T0[NC] // NC, (part + 1) * T0[NC] // NC), midway, zero)
            if v0 == b * NC + c:
                stage_values(*target, zero)
            if u or b:
                u1, b1 = divmod(u * NB + b - 1, NB)
                stage_query(later(u1), u1, b1, c, after)
            else:
                stage_query(head(HU - 1), HU - 1, NB - 1, c, after, jnp.minimum(it, 0))
            if c == NC - 1:
                l_v[head(u), :, pl.ds(b * TQ, TQ)] = l
                parts = [l[:, n * 128:(n + 1) * 128] for n in range(NQ)]
                range_v[0] = functools.reduce(jnp.minimum, parts, range_v[0])
                range_v[1] = functools.reduce(jnp.maximum, parts, range_v[1])
                if m < len(items):
                    ot_v[pl.ds(_aligned(head(u) * DH, DH), DH), pl.ds(b * TQ, TQ)] = acc
        for g in range(AHEAD):
            s0_v[pl.ds(g * 16, 16), :] = from_mxu.pop(first[-1] + g)
        return acc, v

    def exact_step(i, carry):
        h, b = i // (S // TS), i % (S // TS)
        cols = pl.ds(_aligned(b * TS, TS), TS)
        q = qt_v[pl.ds(_aligned(h * DH, DH), DH), cols]
        row_head = jax.lax.broadcasted_iota(i32, (128, TS), 0) // DH
        s = _mm(_halves(k_v, h // 8), jnp.where(row_head == h % 8, jnp.tile(q, (8, 1)), 0.0))
        p = jnp.exp2(s - jnp.max(s, axis=0, keepdims=True))
        v = jnp.concatenate([vt_v[c, pl.ds(_aligned(h * DH, DH), DH), :] for c in range(NC)], axis=1)
        ot_v[pl.ds(_aligned(h * DH, DH), DH), cols] = _mm(v, p)
        l_v[h, :, cols] = jnp.sum(p.reshape(S // 8, 8, TS), axis=0)
        return carry

    def fast_attention():
        range_v[0] = jnp.ones((8, 128), f32)
        range_v[1] = jnp.ones((8, 128), f32)
        lead = [k_v[0, pl.ds(NV[0] // 2 + (NT[0] - 1 - t) * 8, 8)] for t in range(AHEAD)]
        s0_v[...] = _mm(pltpu.bitcast(jnp.concatenate(lead, axis=0), bf16), query_weights((0, 0)))
        pc_v[...] = jnp.zeros((CK, TQ), f32)
        carry = jax.lax.fori_loop(0, H // HU, fast_step, (jnp.zeros((DH, TQ), f32), jnp.zeros((DH // 2, CK), u32)))
        ot_v[last_block(H // HU - 1)] = finish_step(*carry)

    def check_attention():
        safe = (range_v[0] >= L_MIN) & (range_v[1] <= L_MAX) & (range_v[2] <= W_MAX)
        redo = jnp.max(jnp.where(safe, 0.0, 1.0)) > 0.0

        @pl.when(redo)
        def _():
            jax.lax.fori_loop(0, H * (S // TS), exact_step, 0)

    RH, RQ = R3 // 2, R3 // 4

    sent = []

    def send(*part):
        sent.append(pltpu.make_async_copy(out_v.at[part], out_hbm.at[part], out_sem))
        sent[-1].start()

    def normalize(i, h, src):
        rows = pl.ds(i * R3, R3)
        lsum = jnp.sum(tie(l_v[h, :, rows], src), axis=0, keepdims=True)
        inv = pl.reciprocal(lsum, approx=True)
        return ot_v[pl.ds(h * DH, DH), rows] * (inv * (2.0 - lsum * inv))

    def ln2(i, n, src):
        step = RQ // LN2_PIECES
        out = []
        for r in range(4):
            hid = h_v[pl.ds(i * R3 + r * RQ + n * step, step), :]
            out.append(_ln(jnp.concatenate([tie(hid[:, 0:128], src), hid[:, 128:]], axis=1)))
        return out

    def blocks(x):
        return [[x[r * RQ:(r + 1) * RQ, c * 128:(c + 1) * 128] for c in range(4)] for r in range(4)]

    def outer_lhs(a, o):
        return [_lhs7(a[i][j], a[i][2 + j], a[2 + i][j], a[2 + i][2 + j])[o] for i in range(2) for j in range(2)]

    loaded = {}

    def weights(key, load):
        if key not in loaded:
            loaded[key] = len(loaded) % 3
        if isinstance(loaded[key], int):
            if loaded[key]:
                loaded[key] -= 1
                return load()
            loaded[key] = pltpu.bitcast(load(), u32)
        return pltpu.bitcast(loaded[key], bf16)

    def inner(ops, w49, o, t, order):
        rows = slice(None) if t is None else pl.ds(t * 128, 128)
        ms = {p: _mm(ops[p], weights((t, o, p), lambda: w49[o * 7 + p, rows])) for p in order}
        return [_join7(ms, n) for n in range(4)], list(ms.values())

    def phase3(steps):
        b1 = b1_v[...].astype(f32).reshape(1, F)
        b2 = b2_v[...].astype(f32).reshape(1, D)
        att = hn = act = act_rest = src = None
        for i in range(-2, steps + 1):
            def plan(kind, args, span):
                return [(span[0] + (n + 0.5) / len(args) * (span[1] - span[0]), kind, arg) for n, arg in enumerate(args)]

            jobs = []
            if 0 <= i < steps:
                jobs += plan("up", [(o, t) for o in UP_ORDER for t in range(FQ // 128)], (0, 100))
                jobs += plan("rest", REST_ORDER, REST_SPAN)
                outer_ops = [outer_lhs(hn, o) for o in range(7)]
                inner_ops = [_lhs7(*x) for x in outer_ops]
            if i > 0:
                jobs += plan("down", DOWN_ORDER, DOWN_SPAN)
            if 0 <= i + 1 < steps:
                jobs += plan("proj", PROJ_ORDER if i >= 0 else FIRST_PROJ_ORDER, PROJ_SPAN if i else (-1, 0))
                jobs += plan("ln", range(LN2_PIECES), LN2_SPAN)
            if i + 2 < steps:
                jobs += plan("norm", range(H), NORM_SPAN if i >= 0 else (100, 200))
            ups, rests, downs, projs = [{} for _ in range(FQ // 128)], {}, {}, {}
            lns, heads, done = [], [], []
            new_act, new_rest = [[[None] * (FQ // 128) for _ in range(4)] for _ in range(4)], [None] * 4
            for _, kind, arg in sorted(jobs, key=lambda job: job[0]):
                if kind == "up":
                    o, t = arg
                    ups[t][o], ms = inner(inner_ops[o], w149, o, t, UP_INNER)
                    for m in _completed(ups[t], o):
                        for n in range(4):
                            r, c = m // 2 * 2 + n // 2, m % 2 * 2 + n % 2
                            y = _join7({j: x[n] for j, x in ups[t].items()}, m)
                            new_act[r][c][t] = _gelu(y + b1[:, c * FQ + t * 128:c * FQ + (t + 1) * 128])
                elif kind == "rest":
                    rests[arg] = _mm(_whole(*outer_ops[arg]), weights(("rest", arg), lambda: _tiles(w17, arg)))
                    ms = [rests[arg]]
                    for m in _completed(rests, arg):
                        new_rest[m] = _gelu(_join7(rests, m) + b1[:, F2 + m % 2 * 128:F2 + (m % 2 + 1) * 128])
                elif kind == "down":
                    ops = _lhs7(*outer_lhs(act, arg))
                    y = _mm(_lhs7(*act_rest)[arg], weights(("down", arg), lambda: _tiles(w27, arg)))
                    out, ms = inner(ops, w249, arg, None, DOWN_INNER)
                    downs[arg] = [x + y[n // 2 * RQ:(n // 2 + 1) * RQ, n % 2 * 128:(n % 2 + 1) * 128] for n, x in enumerate(out)]
                    for m in _completed(downs, arg):
                        for n in (1, 0, 3, 2):
                            r, c = m // 2 * 2 + n // 2, m % 2 * 2 + n % 2
                            q = (pl.ds((i - 1) * R3 + r * RQ, RQ), pl.ds(c * 128, 128))
                            y = _join7({j: x[n] for j, x in downs.items()}, m)
                            out_v[q] = (h_v[q] + y + b2[:, c * 128:(c + 1) * 128]).astype(out_v.dtype)
                        done.append(m)
                        if i == steps:
                            send(pl.ds((i - 1) * R3 + m // 2 * RH, RH), pl.ds(m % 2 * DQ, DQ))
                        elif len(done) == 4:
                            send(pl.ds((i - 1) * R3, R3))
                elif kind == "proj":
                    projs[arg] = _mm(_whole(*outer_lhs(att, arg)), weights(("proj", arg), lambda: _tiles(wo7, arg)))
                    ms = [projs[arg]]
                    for m in _completed(projs, arg):
                        q = (pl.ds((i + 1) * R3 + m // 2 * RH, RH), pl.ds(m % 2 * DQ, DQ))
                        h_v[q] = x_v[q].astype(f32) + _join7(projs, m)
                elif kind == "ln":
                    lns.append(ln2(i + 1, arg, src))
                    continue
                else:
                    heads.append(normalize(i + 2, arg, src))
                    continue
                src = ms[6 % len(ms)] if i >= 0 else None
            if 0 <= i < steps:
                act, act_rest = [[jnp.concatenate(x, axis=1) for x in row] for row in new_act], new_rest
            if lns:
                hn = blocks(jnp.concatenate([x[r] for r in range(4) for x in lns], axis=0))
            if heads:
                att = blocks(jnp.concatenate(heads, axis=0).T)

    phase1()
    fast_attention()
    check_attention()
    phase3(S // R3)
    for cp in sent:
        cp.wait()


@jax.jit
def pallas_sequential_preLN__softmax_full_mha__dense_activation_gelu__prompt_kernel(
        A_x, A_wqkv, A_wo, B_x, B_w1, B_b1, B_w2, B_b2):
    del B_x
    any_spec = pl.BlockSpec(memory_space=pl.ANY)
    vm = pltpu.VMEM
    out = pl.pallas_call(
        _kernel,
        out_shape=jax.ShapeDtypeStruct((S, D), A_x.dtype),
        in_specs=[any_spec] * 7,
        out_specs=any_spec,
        scratch_shapes=[
            vm((S, D), bf16), vm((D, 3 * D), bf16), vm((D, D), bf16), vm((D, F), bf16), vm((F, D), bf16),
            *[vm((7, 2, D // 4, 128), u32)] * 3, vm((D, D), bf16), vm((D, D), bf16),
            vm((S, D), f32),
            vm((D // 128, S // 2, 128), u32), vm((D // 128, V0[NC], 128), f32),
            vm((D, S), f32), vm((NC, D, CK), bf16), vm((D, S), f32), vm((H, 8, S), f32),
            vm((AHEAD * 16, TQ), f32), vm((CK, TQ), f32), vm((8, 128), f32), vm((3, 8, 128), f32),
            vm((7, 2, D // 2, 128), bf16), vm((7, 1, D // 2, 128), bf16), vm((7, 2, (F - F2) // 2, 128), bf16),
            vm((49, FQ, 128), bf16), vm((49, FQ, 128), bf16), vm((S, D), f32), vm((S, D), bf16),
            pltpu.SemaphoreType.DMA((8,)), pltpu.SemaphoreType.DMA,
            *[vm((T0[NC] * 8, 128), u32)] * HU, *[vm((AHEAD * 8, 128), u32)] * HU,
            *[vm((V0[NC] // 8, DH * 8, 128), f32)] * HU, *[vm((1, DH // 2, S), u32)] * HU,
            *[vm((1, DH, TQ), f32)] * (HU * NB), *[vm((1, NQ, (DH + 1) * 8, 128), f32)] * (HU * NB),
            vm((F,), bf16), vm((D,), bf16),
        ],
        compiler_params=pltpu.CompilerParams(
            vmem_limit_bytes=100 * 1024 * 1024,
        ),
    )(A_x.reshape(S, D), A_wqkv, A_wo, B_w1, B_b1, B_w2, B_b2)
    return out.reshape(A_x.shape)
```
